```python
import jax
import jax.numpy as jnp

def _softmax(x, axis=-1):
    return jax.nn.softmax(x, axis=axis)
def _gelu(x):
    return jax.nn.gelu(x, approximate=True)
def _silu(x):
    return jax.nn.silu(x)
def _sigmoid(x):
    return jax.nn.sigmoid(x)
def _layernorm(x, axis=-1, eps=1e-5):
    m = jnp.mean(x, axis=axis, keepdims=True)
    v = jnp.var(x, axis=axis, keepdims=True)
    return (x - m) / jnp.sqrt(v + eps)
def _scatter_add(tgt, idx, src, axis=0):
    return tgt.at[idx].add(src)
def _segment_sum(src, seg, n):
    return jax.ops.segment_sum(src, seg, n)
class _Rng:
    def __init__(self, key):
        self._k = key
    def _next(self):
        self._k, sub = jax.random.split(self._k)
        return sub
    def normal(self, shape):
        return jax.random.normal(self._next(), shape, dtype=jnp.bfloat16)
    def randint(self, lo, hi, shape):
        return jax.random.randint(self._next(), shape, lo, hi, dtype=jnp.int32)
    def uniform(self, shape, lo=0.0, hi=1.0):
        return jax.random.uniform(self._next(), shape, jnp.bfloat16, lo, hi)
    def permutation(self, n):
        return jax.random.permutation(self._next(), n)


kernel_name = 'concat_heads__gqa_block_cached__mha_block_cached__near_ridge'

def setup_inputs():
    _rng = _Rng(jax.random.key(int.from_bytes(__import__("os").urandom(4), "little")))
    _w = (lambda a: (lambda t: t.astype(jnp.bfloat16) if jnp.issubdtype(t.dtype, jnp.floating) else t)(jnp.asarray(a)))
    def _A_setup():
        B, Sq, D = 16, 160, 640
        Hq, Hkv, Sk, Dh = 32, 32, 512, 192
        assert Hq % Hkv == 0, (Hq, Hkv)
        return {
            "x": _w((lambda *s: _rng.normal(s) * 0.05)(B, Sq, D)),
            "k_cache": _w((lambda *s: _rng.normal(s) * 0.05)(B, Hkv, Sk, Dh)),
            "v_cache": _w((lambda *s: _rng.normal(s) * 0.05)(B, Hkv, Sk, Dh)),
            "wq": _w((lambda *s: _rng.normal(s) * 0.05)(D, Hq * Dh) * (D ** -0.5)),
            "wo": _w((lambda *s: _rng.normal(s) * 0.05)(Hq * Dh, D) * ((Hq * Dh) ** -0.5)),
        }
    _A_in = _A_setup()

    def _B_setup():
        B, Sq, D = 16, 160, 640
        H, Sk, Dh = 32, 512, 192
        return {
            "x": _w((lambda *s: _rng.normal(s) * 0.05)(B, Sq, D)),
            "k_cache": _w((lambda *s: _rng.normal(s) * 0.05)(B, H, Sk, Dh)),
            "v_cache": _w((lambda *s: _rng.normal(s) * 0.05)(B, H, Sk, Dh)),
            "wq": _w((lambda *s: _rng.normal(s) * 0.05)(D, H * Dh) * (D ** -0.5)),
            "wo": _w((lambda *s: _rng.normal(s) * 0.05)(H * Dh, D) * ((H * Dh) ** -0.5)),
        }
    _B_in = _B_setup()

    return {
        "A_x": _A_in["x"],
        "A_k_cache": _A_in["k_cache"],
        "A_v_cache": _A_in["v_cache"],
        "A_wq": _A_in["wq"],
        "A_wo": _A_in["wo"],
        "B_x": _B_in["x"],
        "B_k_cache": _B_in["k_cache"],
        "B_v_cache": _B_in["v_cache"],
        "B_wq": _B_in["wq"],
        "B_wo": _B_in["wo"],
    }

def reference(A_x, A_k_cache, A_v_cache, A_wq, A_wo, B_x, B_k_cache, B_v_cache, B_wq, B_wo):
    def _A_ref(x, k_cache, v_cache, wq, wo):
        B, Sq, D = x.shape
        Hq, Dh = 32, 192
        Hkv = k_cache.shape[1]
        rep = Hq // Hkv
        q = (lambda x, *d: x.transpose(*d))((x @ wq).reshape(B, Sq, Hq, Dh), 0, 2, 1, 3)
        k = jnp.repeat(k_cache, rep, axis=1)
        v = jnp.repeat(v_cache, rep, axis=1)
        scores = jnp.einsum("bhqd,bhkd->bhqk", q, k) * (Dh ** -0.5)
        p = _softmax(scores, axis=-1)
        o = jnp.einsum("bhqk,bhkd->bhqd", p, v)
        return (lambda x, *d: x.transpose(*d))(o, 0, 2, 1, 3).reshape(B, Sq, Hq * Dh) @ wo

    def _B_ref(x, k_cache, v_cache, wq, wo):
        B, Sq, D = x.shape
        H, Dh = 32, 192
        q = (lambda x, *d: x.transpose(*d))((x @ wq).reshape(B, Sq, H, Dh), 0, 2, 1, 3)
        scores = jnp.einsum("bhqd,bhkd->bhqk", q, k_cache) * (Dh ** -0.5)
        p = _softmax(scores, axis=-1)
        o = jnp.einsum("bhqk,bhkd->bhqd", p, v_cache)
        return (lambda x, *d: x.transpose(*d))(o, 0, 2, 1, 3).reshape(B, Sq, H * Dh) @ wo

    a = _A_ref(A_x, A_k_cache, A_v_cache, A_wq, A_wo)
    b = _B_ref(B_x, B_k_cache, B_v_cache, B_wq, B_wo)
    return jnp.concatenate([a, b], axis=-1)
```

```python
import functools
import jax, jax.numpy as jnp
from jax import lax
from jax.experimental import pallas as pl
from jax.experimental.pallas import tpu as pltpu

B, SQ, D, H, SK, DH = 16, 160, 640, 32, 512, 192
PW = 2 * DH
NP = H // 2
LOG2E = 1.4426950408889634
QSCALE = (DH ** -0.5) * LOG2E
NT = (((1,), (1,)), ((), ()))
f32 = jnp.float32
bf16 = jnp.bfloat16


def chunks(m):
    return [(r, min(r + m, SQ)) for r in range(0, SQ, m)]


def _build(nb=4, vmem=100, order=0, nodma=0, hyb=1, mq=80, mk=80, nk=256, mo=80, fold=1):
    nbg = B // nb
    M = nb * SQ

    def dot(a, b):
        return jnp.dot(a, b, preferred_element_type=f32)

    def dotnt(a, b):
        return lax.dot_general(a, b, NT, preferred_element_type=f32)

    def qproj(x, r0, wq):
        cols = []
        for j in range(3):
            parts = []
            for (a, b) in chunks(mq):
                xr = x[pl.ds(pl.multiple_of(r0 + a, 16), b - a), :]
                parts.append(dot(xr, wq[:, j * 128:(j + 1) * 128]) * QSCALE)
            cols.append(parts)
        out = []
        q0 = jnp.concatenate([p.astype(bf16) for p in cols[0]], axis=0)
        q2 = jnp.concatenate([p.astype(bf16) for p in cols[2]], axis=0)
        lo, hi = [], []
        for p in cols[1]:
            lane = lax.broadcasted_iota(jnp.int32, p.shape, 1)
            lo.append(jnp.where(lane < 64, p, 0.0).astype(bf16))
            hi.append(jnp.where(lane >= 64, p, 0.0).astype(bf16))
        qlo = jnp.concatenate(lo, axis=0)
        qhi = jnp.concatenate(hi, axis=0)
        return jnp.concatenate([q0, qlo], axis=1), jnp.concatenate([qhi, q2], axis=1)

    def qk(q, kt):
        res = []
        for h in range(2):
            l = q[h]
            rows = []
            for (a, b) in chunks(mk):
                cs = [dot(l[a:b], kt[h * 128:h * 128 + 256, c:c + nk]) for c in range(0, SK, nk)]
                rows.append(jnp.concatenate(cs, axis=1) if len(cs) > 1 else cs[0])
            res.append(rows)
        return res

    def soft(rows):
        ps, rs = [], []
        for s in rows:
            m = jnp.max(s, axis=-1, keepdims=True)
            p = jnp.exp2(s - m)
            l = jnp.sum(p, axis=-1, keepdims=True)
            ps.append(p.astype(bf16))
            rs.append(1.0 / l)
        return jnp.concatenate(ps, axis=0), jnp.concatenate(rs, axis=0)

    def pv_std(s, vt):
        p1, r1 = soft(s[0])
        p2, r2 = soft(s[1])
        oa = dotnt(p1, vt[0:128, :])
        om = dotnt(jnp.concatenate([p1, p2], axis=0), vt[128:256, :])
        oc = dotnt(p2, vt[256:384, :])
        lane = lax.broadcasted_iota(jnp.int32, (SQ, 128), 1)
        omid = jnp.where(lane < 64, om[:SQ] * r1, om[SQ:] * r2)
        return jnp.concatenate([oa * r1, omid, oc * r2], axis=1).astype(bf16)

    def pv_hyb(s, vt):
        p1, r1 = soft(s[0])
        p2, r2 = soft(s[1])
        T = 128
        R = SQ - T
        ot1 = dotnt(vt[0:192, :], p1[:T])
        oa = dotnt(p1[T:], vt[0:128, :])
        om = dotnt(jnp.concatenate([p1[T:], p2[T:]], axis=0), vt[128:256, :])
        ot2 = dotnt(vt[192:384, :], p2[:T])
        oc = dotnt(p2[T:], vt[256:384, :])
        lane = lax.broadcasted_iota(jnp.int32, (R, 128), 1)
        omr = jnp.where(lane < 64, om[:R], om[R:])
        ta = ot1[0:128].T
        tm = jnp.concatenate([ot1[128:192], ot2[0:64]], axis=0).T
        tc = ot2[64:192].T
        lane = lax.broadcasted_iota(jnp.int32, (SQ, 128), 1)
        rm = jnp.where(lane < 64, r1, r2)
        o0 = jnp.concatenate([ta, oa], axis=0) * r1
        o1 = jnp.concatenate([tm, omr], axis=0) * rm
        o2 = jnp.concatenate([tc, oc], axis=0) * r2
        return jnp.concatenate([o0, o1, o2], axis=1).astype(bf16)

    pv = pv_hyb if hyb else pv_std

    def kernel(xa, kta, vta, wqa, woa, xb, ktb, vtb, wqb, wob, o_ref, acc):
        hp = pl.program_id(0)
        bg = pl.program_id(1)
        row0 = pl.multiple_of(bg * M, M)

        if not fold:
            @pl.when(hp == 0)
            def _():
                acc[pl.ds(row0, M), :] = jnp.zeros((M, 2 * D), f32)

        probs = ((xa, kta, vta, wqa, woa), (xb, ktb, vtb, wqb, wob))
        items = [(p, b) for p in range(2) for b in range(nb)]
        n = len(items)
        Q, S, O = {}, {}, {}

        def do_qp(i):
            if i < n:
                p, b = items[i]
                Q[i] = qproj(probs[p][0], row0 + b * SQ, probs[p][3])

        def do_qk(i):
            if i < n:
                p, b = items[i]
                S[i] = qk(Q.pop(i), probs[p][1].at[b])

        def do_pv(i):
            p, b = items[i]
            O[i] = pv(S.pop(i), probs[p][2].at[b])

        def do_op(i):
            if 0 <= i < n:
                p, b = items[i]
                o = O.pop(i)
                wo = probs[p][4]
                for j in range(5):
                    for (a, e) in chunks(mo):
                        y = dot(o[a:e], wo[:, j * 128:(j + 1) * 128])
                        rs = pl.ds(pl.multiple_of(row0 + b * SQ + a, 16), e - a)
                        cs = slice(p * D + j * 128, p * D + (j + 1) * 128)
                        if fold:
                            t = jnp.where(hp == 0, 0.0, acc[rs, cs]) + y
                            acc[rs, cs] = t
                            o_ref[b * SQ + a:b * SQ + e, cs] = t.astype(bf16)
                        else:
                            acc[rs, cs] += y

        if order == 0:
            do_qp(0); do_qp(1); do_qk(0)
            for i in range(n):
                do_qp(i + 2); do_qk(i + 1); do_pv(i); do_op(i - 1)
            do_op(n - 1)
        elif order == 1:
            do_qp(0); do_qp(1); do_qk(0)
            for i in range(n):
                do_qk(i + 1); do_op(i - 1); do_pv(i); do_qp(i + 2)
            do_op(n - 1)
        elif order == 2:
            do_qp(0); do_qk(0)
            for i in range(n):
                do_qp(i + 1); do_op(i - 1); do_pv(i); do_qk(i + 1)
            do_op(n - 1)
        elif order == 3:
            do_qp(0); do_qk(0)
            for i in range(n):
                do_qp(i + 1); do_pv(i); do_qk(i + 1); do_op(i)

        if not fold:
            @pl.when(hp == NP - 1)
            def _():
                o_ref[...] = acc[pl.ds(row0, M), :].astype(o_ref.dtype)

    def fn(A_x, A_k, A_v, A_wq, A_wo, B_x, B_k, B_v, B_wq, B_wo):
        def prep(x, k, v):
            return (x.reshape(B * SQ, D),
                    jnp.swapaxes(k, 2, 3).reshape(B, H * DH, SK),
                    jnp.swapaxes(v, 2, 3).reshape(B, H * DH, SK))
        xa, kta, vta = prep(A_x, A_k, A_v)
        xb, ktb, vtb = prep(B_x, B_k, B_v)
        x_spec = pl.BlockSpec((B * SQ, D), lambda h, g: (0, 0))
        kv_spec = pl.BlockSpec((nb, PW, SK), (lambda h, g: (0, 0, 0)) if nodma else (lambda h, g: (g, h, 0)))
        wq_spec = pl.BlockSpec((D, PW), lambda h, g: (0, h))
        wo_spec = pl.BlockSpec((PW, D), lambda h, g: (h, 0))
        specs = [x_spec, kv_spec, kv_spec, wq_spec, wo_spec]
        out = pl.pallas_call(
            kernel,
            grid=(NP, nbg),
            in_specs=specs + specs,
            out_specs=pl.BlockSpec((M, 2 * D), lambda h, g: (jnp.where(h == NP - 1, g, 0), 0)),
            out_shape=jax.ShapeDtypeStruct((B * SQ, 2 * D), bf16),
            scratch_shapes=[pltpu.VMEM((B * SQ, 2 * D), f32)],
            compiler_params=pltpu.CompilerParams(
                dimension_semantics=("arbitrary", "arbitrary"),
                vmem_limit_bytes=vmem * 1024 * 1024),
        )(xa, kta, vta, A_wq, A_wo, xb, ktb, vtb, B_wq, B_wo)
        return out.reshape(B, SQ, 2 * D)
    return fn


@jax.jit
def pallas_concat_heads__gqa_block_cached__mha_block_cached__near_ridge_kernel(A_x, A_k_cache, A_v_cache, A_wq, A_wo, B_x, B_k_cache, B_v_cache, B_wq, B_wo):
    return _build()(A_x, A_k_cache, A_v_cache, A_wq, A_wo, B_x, B_k_cache, B_v_cache, B_wq, B_wo)
```

```python
import functools
import jax, jax.numpy as jnp
from jax import lax
from jax.experimental import pallas as pl
from jax.experimental.pallas import tpu as pltpu

B, SQ, D, H, SK, DH = 16, 160, 640, 32, 512, 192
PW = 2 * DH
GW = 2 * PW
LOG2E = 1.4426950408889634
QSCALE = (DH ** -0.5) * LOG2E
NT = (((1,), (1,)), ((), ()))
f32 = jnp.float32
bf16 = jnp.bfloat16
TT = 128
R = SQ - TT
HF = SQ // 2


def chunks(m, tot=SQ):
    return [(r, min(r + m, tot)) for r in range(0, tot, m)]


def dot(a, b):
    return jnp.dot(a, b, preferred_element_type=f32)


def dotnt(a, b):
    return lax.dot_general(a, b, NT, preferred_element_type=f32)


u32 = jnp.uint32


def pk(v):
    return pltpu.bitcast(v.astype(bf16), u32)


def unpk(v):
    return pltpu.bitcast(v, bf16)


def a_combos(a11, a12, a21, a22):
    return [a11 + a22, a21 + a22, a11, a22, a11 + a12, a21 - a11, a12 - a22]


def b_combos(b11, b12, b21, b22):
    return [b11 + b22, b11, b12 - b22, b21 - b11, b22, b11 + b12, b21 + b22]


def _build(NG=8, nb=2, vmem=110, mk=160, nk=256, ms=80, odd="Q0,Q1,Q2,K0,K1,P0,P1", even="K0,K1,P0,P1,O0,O1,O2",
          tail=2, koff=1, qk_="1", ok_="41", dpos=1):
    qcnt = {int(c): str(qk_).count(c) for c in str(qk_) if c != "x"}
    ocnt = {int(c): str(ok_).count(c) for c in str(ok_) if c != "x"}
    nbg = B // nb
    M = nb * SQ
    T = NG * nbg
    SLQ = 128 // nbg
    SQ2 = 2 * SLQ
    LG = nbg.bit_length() - 1
    SLO = PW // nbg

    def recip(l):
        r = pl.reciprocal(l, approx=True)
        return r * (2.0 - l * r)

    def soft(rows):
        ps = []
        for s in rows:
            m = jnp.max(s, axis=-1, keepdims=True)
            ps.append(jnp.exp2(s - m))
        p = jnp.concatenate(ps, axis=0)
        t = (p[:TT, 0:128] + p[:TT, 128:256]) + (p[:TT, 256:384] + p[:TT, 384:512])
        rrow = recip(jnp.sum(t.T, axis=0, keepdims=True))
        rrem = jnp.broadcast_to(recip(jnp.sum(p[TT:], axis=-1, keepdims=True)), (R, 128))
        return p, (rrow, rrem)

    units = [(p, b) for p in range(2) for b in range(nb)]
    U = len(units)
    n = 2 * U

    def kernel(xa, kta, vta, wqa, woa, xb, ktb, vtb, wqb, wob, o_hbm,
               acc, obuf, xraw, xsb, xtb, kvbuf, wqraw, woraw, wqsb, wqtb, wosb, wotb,
               kvsem, wsem, xsem, osem):
        xs, kvs, wqs, wos = (xa, xb), (kta, vta, ktb, vtb), (wqa, wqb), (woa, wob)

        def kv_start(sl, hg_, g_):
            for a in range(4):
                pltpu.make_async_copy(
                    kvs[a].at[pl.ds(g_ * nb, nb), pl.ds(pl.multiple_of(hg_ * GW, GW), GW), :],
                    kvbuf.at[sl, a], kvsem.at[sl]).start()

        def w_start(hg_, sl, par):
            cq = pl.ds(pl.multiple_of(hg_ * GW, GW), GW)
            for p in range(2):
                for (src0, dst0, nr) in ((sl * SQ2, 0, SQ2), (256 + sl * SQ2, SQ2, SQ2), (512 + sl * SLQ, 2 * SQ2, SLQ)):
                    pltpu.make_async_copy(wqs[p].at[pl.ds(pl.multiple_of(src0, 16), nr), cq],
                                          wqraw.at[sl, p, pl.ds(dst0, nr), :], wsem.at[par, 0]).start()
                pltpu.make_async_copy(wos[p].at[hg_, :, pl.ds(pl.multiple_of(sl * SLO, 16), SLO), :],
                                      woraw.at[sl, p], wsem.at[par, 1]).start()

        def w_wait(vq, vo, par):
            pltpu.make_async_copy(vq, vq, wsem.at[par, 0]).wait()
            pltpu.make_async_copy(vo, vo, wsem.at[par, 1]).wait()

        def x_start(g_):
            for p in range(2):
                pltpu.make_async_copy(xs[p].at[pl.ds(g_ * nb, nb)], xraw.at[g_ & 1, p], xsem.at[0]).start()

        def wq_piece(ws, sl, p, j, r0, nr):
            blk = [wqraw[sl, p, r * SQ2 + r0:r * SQ2 + r0 + nr, c * PW + j * 128:c * PW + (j + 1) * 128].astype(f32)
                   for r in range(2) for c in range(2)]
            for k, v in enumerate(b_combos(*blk)):
                wqsb[ws, p, k, j, pl.ds(pl.multiple_of(sl * SLQ + r0 // 2, 8), nr // 2), :] = pk(v)
            if r0 == 0:
                for c in (j, j + 3):
                    wqtb[ws, p, c, pl.ds(pl.multiple_of(sl * (SLQ // 2), 8), SLQ // 2), :] = pk(
                        wqraw[sl, p, 2 * SQ2:2 * SQ2 + SLQ, c * 128:(c + 1) * 128])

        def wo_piece(ws, sl, p, j, r0, nr):
            ho0 = pl.multiple_of(sl * (SLO // 2) + r0 // 2, 8)
            blk = [woraw[sl, p, r, r0:r0 + nr, c * 256 + j * 128:c * 256 + (j + 1) * 128].astype(f32)
                   for r in range(2) for c in range(2)]
            for k, v in enumerate(b_combos(*blk)):
                wosb[ws, p, k, j, pl.ds(ho0, nr // 2), :] = pk(v)
            wotb[ws, p, pl.ds(j * (PW // 2) + ho0, nr // 2), :] = pk(woraw[sl, p, j, r0:r0 + nr, 512:640])

        wq_pieces = [(p, j, r0, 16) for p in range(2) for j in range(3) for r0 in range(0, SQ2, 16)]
        wo_pieces = [(p, j, r0, 16) for p in range(2) for j in range(2) for r0 in range(0, SLO, 16)]

        def x_combos(g_):
            for p in range(2):
                for b in range(nb):
                    bb = g_ * nb + b
                    for kt in range(2):
                        blk = [xraw[g_ & 1, p, b, r * HF:(r + 1) * HF, (kt + 2 * c) * 128:(kt + 2 * c + 1) * 128].astype(f32)
                               for r in range(2) for c in range(2)]
                        for k, v in enumerate(a_combos(*blk)):
                            xsb[p, bb, k, kt] = pk(v)
                    xtb[p, bb] = pk(xraw[g_ & 1, p, b, :, 512:640])

        def step(t, carry):
            hg = lax.shift_right_logical(t, LG)
            g = t & (nbg - 1)
            slot = t & 1
            wslot = hg & 1
            row0 = pl.multiple_of(g * M, M)

            @pl.when(hg == 0)
            def _():
                pltpu.make_async_copy(xraw.at[g & 1], xraw.at[g & 1], xsem.at[0]).wait()

                @pl.when(g + 1 < nbg)
                def _():
                    x_start(g + 1)
                x_combos(g)

            @pl.when(hg + 1 < NG)
            def _():
                w_wait(wqraw.at[g], woraw.at[g], slot)

            pltpu.make_async_copy(kvbuf.at[slot], kvbuf.at[slot], kvsem.at[slot]).wait()

            def starts():
                t1 = t + 1
                hg1 = lax.shift_right_logical(t1, LG)
                g1 = t1 & (nbg - 1)

                @pl.when(t1 < T)
                def _():
                    kv_start(1 - slot, hg1, g1)

                t2 = t + 2

                @pl.when(t2 + nbg < T)
                def _():
                    w_start(lax.shift_right_logical(t2, LG) + 1, t2 & (nbg - 1), slot)

            st = [dict() for _ in range(n)]

            wq_todo, wo_todo = list(wq_pieces), list(wo_pieces)

            def emit(todo, fn, cnt):
                for _ in range(cnt):
                    if todo:
                        fn(1 - wslot, g, *todo.pop(0))

            def strassen(prod0, init, hook):
                def prod(k):
                    hook(k)
                    return prod0(k)
                m1 = prod(0)
                c11 = init(0, 0) + m1
                c22 = init(1, 1) + m1
                m4 = prod(3)
                c11 = c11 + m4
                c21 = init(1, 0) + m4
                m5 = prod(4)
                c11 = c11 - m5
                c12 = init(0, 1) + m5
                c11 = c11 + prod(6)
                m2 = prod(1)
                c21 = c21 + m2
                c22 = c22 - m2
                m3 = prod(2)
                c12 = c12 + m3
                c22 = c22 + m3
                c22 = c22 + prod(5)
                return c11, c12, c21, c22

            def task_q(u, j):
                p, b = units[u]
                bb = g * nb + b
                res = [[], [], [], []]
                for (a, e) in chunks(ms, HF):
                    def prod(k):
                        lhs = unpk(jnp.concatenate([xsb[p, bb, k, 0, a // 2:e // 2, :], xsb[p, bb, k, 1, a // 2:e // 2, :]], axis=1))
                        return dot(lhs, unpk(wqsb[wslot, p, k, j]))

                    def init(r, c):
                        return dot(unpk(xtb[p, bb, (r * HF + a) // 2:(r * HF + e) // 2, :]), unpk(wqtb[wslot, p, c * 3 + j]))
                    for lst, c in zip(res, strassen(prod, init, lambda k: emit(wq_todo, wq_piece, qcnt.get(k, 0)))):
                        lst.append(c * QSCALE)
                st[2 * u]["q%d" % j] = jnp.concatenate(res[0] + res[2], axis=0)
                st[2 * u + 1]["q%d" % j] = jnp.concatenate(res[1] + res[3], axis=0)

            def task_k(i, h):
                p, b = units[i // 2]
                k0 = (i % 2) * PW
                kt = kvbuf.at[slot, 2 * p, b]
                qm = st[i]["q1"]
                lane = lax.broadcasted_iota(jnp.int32, qm.shape, 1)
                if h == 0:
                    l = jnp.concatenate([st[i]["q0"], jnp.where(lane < 64, qm, 0.0)], axis=1)
                else:
                    l = jnp.concatenate([jnp.where(lane >= 64, qm, 0.0), st[i]["q2"]], axis=1)
                rows = []
                for (a, e) in chunks(mk):
                    lc = l[a:e].astype(bf16)
                    cs = [dot(lc, kt[k0 + h * 128:k0 + h * 128 + 256, c:c + nk]) for c in range(0, SK, nk)]
                    rows.append(jnp.concatenate(cs, axis=1) if len(cs) > 1 else cs[0])
                st[i]["s%d" % h] = rows

            def task_p(i, h):
                p, b = units[i // 2]
                k0 = (i % 2) * PW
                vt = kvbuf.at[slot, 2 * p + 1, b]
                d = st[i]
                pp, rr = soft(d["s%d" % h])
                d["p%d" % h], d["r%d" % h] = pp, rr
                if h == 0:
                    d["ot1"] = dotnt(vt[k0:k0 + 192, :], pp[:TT].astype(bf16))
                    d["oa"] = dotnt(pp[TT:].astype(bf16), vt[k0:k0 + 128, :])
                else:
                    p1, r1, p2, r2 = d["p0"], d["r0"], pp, rr
                    om = dotnt(jnp.concatenate([p1[TT:], p2[TT:]], axis=0).astype(bf16), vt[k0 + 128:k0 + 256, :])
                    ot2 = dotnt(vt[k0 + 192:k0 + 384, :], p2[:TT].astype(bf16))
                    oc = dotnt(p2[TT:].astype(bf16), vt[k0 + 256:k0 + 384, :])
                    ot1 = d["ot1"] * r1[0]
                    ot2 = ot2 * r2[0]
                    lane = lax.broadcasted_iota(jnp.int32, (R, 128), 1)
                    omr = jnp.where(lane < 64, om[:R] * r1[1], om[R:] * r2[1])
                    ta = ot1[0:128].T
                    tm = jnp.concatenate([ot1[128:192], ot2[0:64]], axis=0).T
                    tc = ot2[64:192].T
                    o0 = jnp.concatenate([ta, d["oa"] * r1[1]], axis=0)
                    o1 = jnp.concatenate([tm, omr], axis=0)
                    o2 = jnp.concatenate([tc, oc * r2[1]], axis=0)
                    d["o"] = jnp.concatenate([o0, o1, o2], axis=1)

            def task_o(u, j):
                p, b = units[u]
                d = st[2 * u]
                if "oc" not in d:
                    oa_, ob_ = st[2 * u]["o"], st[2 * u + 1]["o"]
                    cmb = a_combos(oa_[:HF], ob_[:HF], oa_[HF:], ob_[HF:])
                    d["oc"] = [[c[a:e].astype(bf16) for (a, e) in chunks(ms, HF)] for c in cmb]
                    d["of"] = [jnp.concatenate([oa_[a:e], ob_[a:e]], axis=1).astype(bf16) for (a, e) in chunks(HF)]

                def rows(a, e):
                    return pl.ds(pl.multiple_of(row0 + b * SQ + a, 16), e - a)

                def accv(rs, cs):
                    return jnp.where(hg == 0, 0.0, acc[rs, cs])

                def put(rs, cs, v):
                    acc[rs, cs] = v
                    obuf[rs, cs] = v.astype(bf16)
                if j < 2:
                    for ci, (a, e) in enumerate(chunks(ms, HF)):
                        def idx(r, c):
                            c0 = p * D + c * 256 + j * 128
                            return rows(r * HF + a, r * HF + e), slice(c0, c0 + 128)

                        def prod(k):
                            return dot(d["oc"][k][ci], unpk(wosb[wslot, p, k, j]))
                        c11, c12, c21, c22 = strassen(prod, lambda r, c: accv(*idx(r, c)), lambda k: emit(wo_todo, wo_piece, ocnt.get(k, 0)))
                        put(*idx(0, 0), c11); put(*idx(0, 1), c12); put(*idx(1, 0), c21); put(*idx(1, 1), c22)
                else:
                    cs = slice(p * D + 512, p * D + 640)
                    for ci, (a, e) in enumerate(chunks(HF)):
                        rs = rows(a, e)
                        put(rs, cs, accv(rs, cs) + dot(d["of"][ci], unpk(wotb[wslot, p])))

            seq = []
            for s in range(-3, n + 1):
                for tok in (odd if s % 2 else even).split(","):
                    k, j = tok[0], int(tok[1])
                    if k == "Q":
                        u = (s + 1) // 2 + koff
                        if 0 <= u < U: seq.append(("Q", u, j))
                    elif k == "O":
                        u = s // 2 - 1
                        if 0 <= u < U: seq.append(("O", u, j))
                    elif k == "K":
                        if 0 <= s + koff < n: seq.append(("K", s + koff, j))
                    else:
                        if 0 <= s < n: seq.append(("P", s, j))
            if tail:
                mv = [x for x in seq if x[0] == "O" and x[1] == U - 2][-tail:]
                seq = [x for x in seq if x not in mv]
                pos = seq.index(("P", n - 1, 1)) + 1
                seq = seq[:pos] + mv + seq[pos:]
            fns = {"Q": task_q, "K": task_k, "P": task_p, "O": task_o}
            for ti, tk in enumerate(seq):
                if ti == dpos:
                    starts()
                fns[tk[0]](tk[1], tk[2])
            emit(wq_todo, wq_piece, 100)
            emit(wo_todo, wo_piece, 100)

            @pl.when(hg == NG - 1)
            def _():
                rs = pl.ds(row0, M)
                pltpu.make_async_copy(obuf.at[rs, :], o_hbm.at[rs, :], osem.at[0]).start()
            return carry

        def pro0(sl, c):
            w_start(0, sl, 0)
            return c
        lax.fori_loop(0, nbg, pro0, 0)
        x_start(0)
        kv_start(0, 0, 0)
        w_wait(wqraw, woraw, 0)

        def pro(sl, c):
            for a in wq_pieces:
                wq_piece(0, sl, *a)
            for a in wo_pieces:
                wo_piece(0, sl, *a)
            return c
        lax.fori_loop(0, nbg, pro, 0)
        if NG > 1:
            w_start(1, 0, 0)
            w_start(1, 1, 1)
        lax.fori_loop(0, T, step, 0)
        pltpu.make_async_copy(obuf, o_hbm, osem.at[0]).wait()

    def fn(A_x, A_k, A_v, A_wq, A_wo, B_x, B_k, B_v, B_wq, B_wo):
        def kv(k):
            return jnp.swapaxes(k, 2, 3).reshape(B, H * DH, SK)

        def wq5(w):
            return w.reshape(5, 128, H * DH)

        def wo4(w):
            return w.reshape(8, 2, PW, D)
        anyspec = pl.BlockSpec(memory_space=pl.ANY)
        out = pl.pallas_call(
            kernel,
            in_specs=[anyspec] * 10,
            out_specs=anyspec,
            out_shape=jax.ShapeDtypeStruct((B * SQ, 2 * D), bf16),
            scratch_shapes=[pltpu.VMEM((B * SQ, 2 * D), f32),
                            pltpu.VMEM((B * SQ, 2 * D), bf16),
                            pltpu.VMEM((2, 2, nb, SQ, D), bf16),
                            pltpu.VMEM((2, B, 7, 2, HF // 2, 128), u32),
                            pltpu.VMEM((2, B, SQ // 2, 128), u32),
                            pltpu.VMEM((2, 4, nb, GW, SK), bf16),
                            pltpu.VMEM((nbg, 2, 5 * SLQ, GW), bf16),
                            pltpu.VMEM((nbg, 2, 2, SLO, D), bf16),
                            pltpu.VMEM((2, 2, 7, 3, 128, 128), u32),
                            pltpu.VMEM((2, 2, 6, 64, 128), u32),
                            pltpu.VMEM((2, 2, 7, 2, PW // 2, 128), u32),
                            pltpu.VMEM((2, 2, GW // 2, 128), u32),
                            pltpu.SemaphoreType.DMA((2,)),
                            pltpu.SemaphoreType.DMA((2, 2)),
                            pltpu.SemaphoreType.DMA((1,)),
                            pltpu.SemaphoreType.DMA((1,)),
                            ],
            compiler_params=pltpu.CompilerParams(
                vmem_limit_bytes=vmem * 1024 * 1024,
                disable_bounds_checks=True),
        )(A_x, kv(A_k), kv(A_v), A_wq, wo4(A_wo), B_x, kv(B_k), kv(B_v), B_wq, wo4(B_wo))
        return out.reshape(B, SQ, 2 * D)
    return fn


@jax.jit
def pallas_concat_heads__gqa_block_cached__mha_block_cached__near_ridge_kernel(A_x, A_k_cache, A_v_cache, A_wq, A_wo, B_x, B_k_cache, B_v_cache, B_wq, B_wo):
    return _build(ms=48)(A_x, A_k_cache, A_v_cache, A_wq, A_wo, B_x, B_k_cache, B_v_cache, B_wq, B_wo)
```

```python
import jax, jax.numpy as jnp
from jax import lax
from jax.experimental import pallas as pl
from jax.experimental.pallas import tpu as pltpu

B, SQ, D, H, SK, DH = 16, 160, 640, 32, 512, 192
PW = 2 * DH
GW = 2 * PW
LOG2E = 1.4426950408889634
QSCALE = (DH ** -0.5) * LOG2E
NT = (((1,), (1,)), ((), ()))
f32, bf16, u32 = jnp.float32, jnp.bfloat16, jnp.uint32
TT = 128
R = SQ - TT
HF = SQ // 2


def chunks(m, tot=SQ):
    return [(r, min(r + m, tot)) for r in range(0, tot, m)]


def dot(a, b):
    return jnp.dot(a, b, preferred_element_type=f32)


def dotnt(a, b):
    return lax.dot_general(a, b, NT, preferred_element_type=f32)


def unpk(v):
    return pltpu.bitcast(v, bf16)


def s_alpha(a11, a12, a21, a22):
    return [a11 + a22, a21 + a22, a11, a22, a11 + a12, a21 - a11, a12 - a22]


def s_gamma(b11, b12, b21, b22):
    return [b11 + b22, b11, b12 - b22, b21 - b11, b22, b11 + b12, b21 + b22]


S_BETA = {0: ((0, 0, 1), (1, 1, 1)), 3: ((0, 0, 1), (1, 0, 1)), 4: ((0, 0, -1), (0, 1, 1)), 6: ((0, 0, 1),),
          1: ((1, 0, 1), (1, 1, -1)), 2: ((0, 1, 1), (1, 1, 1)), 5: ((1, 1, 1),)}


def h_alpha(x0, x1, x2, y0, y1, y2):
    s0, s1, s2 = x0 + y0, x1 + y1, x2 + y2
    return [x0, s0, s1, y1, x2, y2, x0 + y1, x1 - x0, y0 - y1, s0 - y2, s2 - s0, y2 - y0, s1 - x2, s2 - s1, x2 - x1]


def h_gamma(w00, w01, w02, w10, w11, w12, w20, w21, w22):
    return [w00 - w02 + w10, w00 - w01 + w20, w11 - w10 + w21, w01 + w11 - w12, w12 - w20 + w22, w02 - w21 + w22,
            w01 + w10, w10, w01, w02 + w20, w20, w02, w12 + w21, w21, w12]


H_BETA = {2: ((0, 1, 1),), 3: ((0, 1, -1), (1, 1, 1)),
          6: ((0, 1, 1), (1, 0, 1)), 7: ((0, 0, 1), (0, 1, 1)), 8: ((1, 0, 1), (1, 1, 1)),
          0: ((0, 0, 1), (1, 0, -1)), 1: ((1, 0, 1),),
          9: ((0, 0, 1), (0, 2, 1), (1, 0, -1)), 10: ((0, 0, 1), (0, 2, 1)),
          11: ((0, 0, 1), (0, 2, 1), (1, 0, -1), (1, 2, -1)),
          4: ((0, 2, 1),), 5: ((1, 2, 1),),
          12: ((0, 1, -1), (1, 1, 1), (1, 2, 1)), 13: ((1, 1, 1), (1, 2, 1)),
          14: ((0, 1, -1), (0, 2, -1), (1, 1, 1), (1, 2, 1))}


def pcombos(blks, fn):
    us = [pltpu.bitcast(b, u32) for b in blks]
    lo_in = [pltpu.unpack_elementwise(u, index=0, packed_dtype=bf16, unpacked_dtype=f32) for u in us]
    hi_in = [pltpu.unpack_elementwise(u, index=1, packed_dtype=bf16, unpacked_dtype=f32) for u in us]
    out = []
    for lo, hi in zip(fn(*lo_in), fn(*hi_in)):
        triv = [k for k, v in enumerate(lo_in) if v is lo]
        out.append(us[triv[0]] if triv else pltpu.pack_elementwise([lo, hi], packed_dtype=bf16).astype(u32))
    return out


def bilinear(beta, order, prod, c, init=None):
    for r in order:
        m = prod(r)
        for (s, j, sg) in beta[r]:
            if (s, j) not in c and init is not None:
                c[(s, j)] = init(s, j)
            if (s, j) in c:
                c[(s, j)] = c[(s, j)] + m if sg > 0 else c[(s, j)] - m
            else:
                c[(s, j)] = m if sg > 0 else -m
    return c


def _build(NG=8, nb=2, vmem=110, mk=160, nk=256, mq=80, mo=80,
          odd="Q0,Q1,Q2,Q3,Q4,K0,K1,P0,P1", even="K0,K1,P0,P1,O0,O1,O2",
          tail=2, koff=1, dpos=1, sch=4, wq_every=4, wo_every=2):
    nbg = B // nb
    M = nb * SQ
    T = NG * nbg
    SL = 128 // nbg
    LG = nbg.bit_length() - 1

    def recip(l):
        r = pl.reciprocal(l, approx=True)
        return r * (2.0 - l * r)

    def soft(s, zvec):
        ps = []
        for r in range(SQ // 8):
            sb = s[r * 8:(r + 1) * 8]
            m = jnp.broadcast_to(jnp.max(sb, axis=-1, keepdims=True), (8, 128))
            if sch and r >= sch:
                link = pltpu.bitcast(ps[r - sch][:, 384:512], u32) & zvec
                m = pltpu.bitcast(pltpu.bitcast(m, u32) | link, f32)
            ps.append(jnp.exp2(sb - jnp.concatenate([m] * 4, axis=1)))
        p = jnp.concatenate(ps, axis=0)
        t = (p[:TT, 0:128] + p[:TT, 128:256]) + (p[:TT, 256:384] + p[:TT, 384:512])
        rrow = recip(jnp.sum(t.T, axis=0, keepdims=True))
        rrem = jnp.broadcast_to(recip(jnp.sum(p[TT:], axis=-1, keepdims=True)), (R, 128))
        return p, (rrow, rrem)

    units = [(p, b) for p in range(2) for b in range(nb)]
    U = len(units)
    n = 2 * U

    def kernel(xa, kta, vta, wqa, woa, xb, ktb, vtb, wqb, wob, o_hbm,
               acc, obuf, xraw, xsb, kvbuf, wqraw, woraw, wqc, woc, zv,
               kvsem, wsem, xsem, osem):
        xs, kvs, wqs, wos = (xa, xb), (kta, vta, ktb, vtb), (wqa, wqb), (woa, wob)

        def kv_start(sl, hg_, g_):
            for a in range(4):
                pltpu.make_async_copy(
                    kvs[a].at[pl.ds(g_ * nb, nb), pl.ds(pl.multiple_of(hg_ * GW, GW), GW), :],
                    kvbuf.at[sl, a], kvsem.at[sl]).start()

        def w_start(hg_, sl, par):
            cq = pl.ds(pl.multiple_of(hg_ * GW, GW), GW)
            for p in range(2):
                for kt in range(5):
                    pltpu.make_async_copy(wqs[p].at[pl.ds(pl.multiple_of(kt * 128 + sl * SL, SL), SL), cq],
                                          wqraw.at[sl, p, kt], wsem.at[par, 0]).start()
                pltpu.make_async_copy(wos[p].at[hg_, :, pl.ds(pl.multiple_of(sl * SL, SL), SL), :],
                                      woraw.at[sl, p], wsem.at[par, 1]).start()

        def w_wait(vq, vo, par):
            pltpu.make_async_copy(vq, vq, wsem.at[par, 0]).wait()
            pltpu.make_async_copy(vo, vo, wsem.at[par, 1]).wait()

        def x_start(g_):
            for p in range(2):
                pltpu.make_async_copy(xs[p].at[pl.ds(g_ * nb, nb)], xraw.at[g_ & 1, p], xsem.at[0]).start()

        def ct(c):
            return slice(c * 128, (c + 1) * 128)

        def wq_piece(ws, sl, p, kind, a):
            rs = pl.ds(pl.multiple_of(sl * (SL // 2), 8), SL // 2)
            if kind == 0:
                blk = [wqraw[sl, p, kt, :, ct(a + 3 * c)] for kt in range(2) for c in range(2)]
                for k, v in enumerate(pcombos(blk, s_gamma)):
                    wqc[ws, p, a * 7 + k, rs, :] = v
            else:
                blk = [wqraw[sl, p, 2 + i, :, ct(3 * a + j)] for i in range(3) for j in range(3)]
                for r, v in enumerate(pcombos(blk, h_gamma)):
                    wqc[ws, p, 21 + a * 15 + r, rs, :] = v

        def wo_piece(ws, sl, p, kind, a):
            rs = pl.ds(pl.multiple_of(sl * (SL // 2), 8), SL // 2)
            if kind == 0:
                blk = [woraw[sl, p, a + 3 * r, :, ct(c)] for r in range(2) for c in range(2)]
                for k, v in enumerate(pcombos(blk, s_gamma)):
                    woc[ws, p, k * 3 + a, rs, :] = v
            else:
                blk = [woraw[sl, p, 3 * a + i, :, ct(2 + j)] for i in range(3) for j in range(3)]
                for r, v in enumerate(pcombos(blk, h_gamma)):
                    woc[ws, p, 21 + r * 2 + a, rs, :] = v

        w_pieces = [(p, kind, a) for p in range(2) for kind in range(2) for a in range(3 - kind)]

        def x_combos(g_):
            for p in range(2):
                for b in range(nb):
                    bb = g_ * nb + b

                    def blk(r, kt):
                        return xraw[g_ & 1, p, b, r * HF:(r + 1) * HF, ct(kt)]
                    cs = pcombos([blk(r, kt) for r in range(2) for kt in range(2)], s_alpha)
                    cs += pcombos([blk(r, kt) for r in range(2) for kt in range(2, 5)], h_alpha)
                    for k, v in enumerate(cs):
                        xsb[p, bb, k] = v

        def step(t, carry):
            hg = lax.shift_right_logical(t, LG)
            g = t & (nbg - 1)
            slot = t & 1
            wslot = hg & 1
            row0 = pl.multiple_of(g * M, M)

            @pl.when(hg == 0)
            def _():
                pltpu.make_async_copy(xraw.at[g & 1], xraw.at[g & 1], xsem.at[0]).wait()

                @pl.when(g + 1 < nbg)
                def _():
                    x_start(g + 1)
                x_combos(g)

            @pl.when(hg + 1 < NG)
            def _():
                w_wait(wqraw.at[g], woraw.at[g], slot)

            pltpu.make_async_copy(kvbuf.at[slot], kvbuf.at[slot], kvsem.at[slot]).wait()

            def starts():
                t1 = t + 1

                @pl.when(t1 < T)
                def _():
                    kv_start(1 - slot, lax.shift_right_logical(t1, LG), t1 & (nbg - 1))

                t2 = t + 2

                @pl.when(t2 + nbg < T)
                def _():
                    w_start(lax.shift_right_logical(t2, LG) + 1, t2 & (nbg - 1), slot)

            st = [dict() for _ in range(n)]
            zvec = zv[...]
            todo = {"q": list(w_pieces), "o": list(w_pieces)}
            cnt = {"q": 0, "o": 0}

            def host(kind):
                cnt[kind] += 1
                every = wq_every if kind == "q" else wo_every
                if every and cnt[kind] % every == 0 and todo[kind]:
                    (wq_piece if kind == "q" else wo_piece)(1 - wslot, g, *todo[kind].pop(0))

            def task_q(u, j):
                p, b = units[u]
                bb = g * nb + b
                d = st[2 * u].setdefault("qc", {})
                for (a, e) in chunks(mq, HF):
                    c = d.setdefault(a, {})

                    def prod(xk, wk):
                        host("q")
                        return dot(unpk(xsb[p, bb, xk, a // 2:e // 2, :]), unpk(wqc[wslot, p, wk]))
                    if j < 2:
                        sub = bilinear(H_BETA, list(H_BETA), lambda r: prod(7 + r, 21 + j * 15 + r),
                                       {(s, jj): c[(s, 3 * j + jj)] for s in range(2) for jj in range(3) if (s, 3 * j + jj) in c})
                        for (s, jj), v in sub.items():
                            c[(s, 3 * j + jj)] = v
                    else:
                        jj = j - 2
                        sub = bilinear(S_BETA, list(S_BETA), lambda k: prod(k, jj * 7 + k),
                                       {(s, cc): c[(s, jj + 3 * cc)] for s in range(2) for cc in range(2) if (s, jj + 3 * cc) in c})
                        for (s, cc), v in sub.items():
                            c[(s, jj + 3 * cc)] = v

            def q_tile(i, j):
                d = st[2 * (i // 2)]["qc"]
                col = 3 * (i % 2) + j
                return jnp.concatenate([d[a][(s, col)] for s in range(2) for (a, e) in chunks(mq, HF)], axis=0) * QSCALE

            def task_k(i, h):
                p, b = units[i // 2]
                k0 = (i % 2) * PW
                kt = kvbuf.at[slot, 2 * p, b]
                d = st[i]
                if "qm" not in d:
                    d["qm"] = q_tile(i, 1)
                qm = d["qm"]
                lane = lax.broadcasted_iota(jnp.int32, qm.shape, 1)
                if h == 0:
                    l = jnp.concatenate([q_tile(i, 0), jnp.where(lane < 64, qm, 0.0)], axis=1)
                else:
                    l = jnp.concatenate([jnp.where(lane >= 64, qm, 0.0), q_tile(i, 2)], axis=1)
                rows = []
                for (a, e) in chunks(mk):
                    lc = l[a:e].astype(bf16)
                    cs = [dot(lc, kt[k0 + h * 128:k0 + h * 128 + 256, c:c + nk]) for c in range(0, SK, nk)]
                    rows.append(jnp.concatenate(cs, axis=1))
                pp, rr = soft(jnp.concatenate(rows, axis=0), zvec)
                d["p%d" % h], d["r%d" % h] = pp, rr

            def task_p(i, h):
                p, b = units[i // 2]
                k0 = (i % 2) * PW
                vt = kvbuf.at[slot, 2 * p + 1, b]
                d = st[i]
                if h == 0:
                    d["ot1"] = dotnt(vt[k0:k0 + 192, :], d["p0"][:TT].astype(bf16))
                    d["oa"] = dotnt(d["p0"][TT:].astype(bf16), vt[k0:k0 + 128, :])
                else:
                    p1, r1, p2, r2 = d["p0"], d["r0"], d["p1"], d["r1"]
                    om = dotnt(jnp.concatenate([p1[TT:], p2[TT:]], axis=0).astype(bf16), vt[k0 + 128:k0 + 256, :])
                    ot2 = dotnt(vt[k0 + 192:k0 + 384, :], p2[:TT].astype(bf16))
                    oc = dotnt(p2[TT:].astype(bf16), vt[k0 + 256:k0 + 384, :])
                    ot1 = d["ot1"] * r1[0]
                    ot2 = ot2 * r2[0]
                    lane = lax.broadcasted_iota(jnp.int32, (R, 128), 1)
                    omr = jnp.where(lane < 64, om[:R] * r1[1], om[R:] * r2[1])
                    ta = ot1[0:128].T
                    tm = jnp.concatenate([ot1[128:192], ot2[0:64]], axis=0).T
                    tc = ot2[64:192].T
                    d["o"] = [jnp.concatenate([ta, d["oa"] * r1[1]], axis=0),
                              jnp.concatenate([tm, omr], axis=0),
                              jnp.concatenate([tc, oc * r2[1]], axis=0)]

            H_SPLIT = [list(H_BETA)[:7], list(H_BETA)[7:]]

            def task_o(u, j):
                p, b = units[u]
                d = st[2 * u]
                if "os" not in d:
                    o1, o2 = st[2 * u]["o"], st[2 * u + 1]["o"]
                    f1, f2 = jnp.concatenate(o1, axis=1), jnp.concatenate(o2, axis=1)
                    d["os"] = s_alpha(f1[:HF], f2[:HF], f1[HF:], f2[HF:])
                    h1 = h_alpha(*([v[:HF] for v in o1] + [v[HF:] for v in o1]))
                    h2 = h_alpha(*([v[:HF] for v in o2] + [v[HF:] for v in o2]))
                    d["oh"] = [jnp.concatenate([v1, v2], axis=1) for v1, v2 in zip(h1, h2)]
                    d["hc"] = {}

                for (a, e) in chunks(mo, HF):
                    def idx(s, col):
                        c0 = p * D + col * 128
                        return pl.ds(pl.multiple_of(row0 + b * SQ + s * HF + a, 16), e - a), slice(c0, c0 + 128)

                    def accv(s, col):
                        return jnp.where(hg == 0, 0.0, acc[idx(s, col)])

                    def put(s, col, v):
                        acc[idx(s, col)] = v
                        obuf[idx(s, col)] = v.astype(bf16)

                    def prod(lhs, w0, nt):
                        host("o")
                        w = woc[wslot, p, w0:w0 + nt].reshape(nt * 64, 128)
                        return dot(lhs[a:e].astype(bf16), unpk(w))
                    if j == 0:
                        c = bilinear(S_BETA, list(S_BETA), lambda k: prod(d["os"][k], k * 3, 3), {}, accv)
                        for (s, col), v in c.items():
                            put(s, col, v)
                    else:
                        c = bilinear(H_BETA, H_SPLIT[j - 1], lambda r: prod(d["oh"][r], 21 + r * 2, 2),
                                     d["hc"].setdefault(a, {}), lambda s, col: accv(s, 2 + col))
                        if j == 2:
                            for (s, col), v in c.items():
                                put(s, 2 + col, v)

            seq = []
            for s in range(-3, n + 1):
                for tok in (odd if s % 2 else even).split(","):
                    k, j = tok[0], int(tok[1])
                    if k == "Q":
                        u = (s + 1) // 2 + koff
                        if 0 <= u < U: seq.append(("Q", u, j))
                    elif k == "O":
                        u = s // 2 - 1
                        if 0 <= u < U: seq.append(("O", u, j))
                    elif k == "K":
                        if 0 <= s + koff < n: seq.append(("K", s + koff, j))
                    else:
                        if 0 <= s < n: seq.append(("P", s, j))
            if tail:
                mv = [x for x in seq if x[0] == "O" and x[1] == U - 2][-tail:]
                seq = [x for x in seq if x not in mv]
                pos = seq.index(("P", n - 1, 1)) + 1
                seq = seq[:pos] + mv + seq[pos:]
            fns = {"Q": task_q, "K": task_k, "P": task_p, "O": task_o}
            for ti, tk in enumerate(seq):
                if ti == dpos:
                    starts()
                fns[tk[0]](tk[1], tk[2])
            for a in todo["q"]:
                wq_piece(1 - wslot, g, *a)
            for a in todo["o"]:
                wo_piece(1 - wslot, g, *a)

            @pl.when(hg == NG - 1)
            def _():
                rs = pl.ds(row0, M)
                pltpu.make_async_copy(obuf.at[rs, :], o_hbm.at[rs, :], osem.at[0]).start()
            return carry

        zv[...] = jnp.zeros((8, 128), u32)

        def pro0(sl, c):
            w_start(0, sl, 0)
            return c
        lax.fori_loop(0, nbg, pro0, 0)
        x_start(0)
        kv_start(0, 0, 0)
        w_wait(wqraw, woraw, 0)

        def pro(sl, c):
            for a in w_pieces:
                wq_piece(0, sl, *a)
                wo_piece(0, sl, *a)
            return c
        lax.fori_loop(0, nbg, pro, 0)
        if NG > 1:
            w_start(1, 0, 0)
            w_start(1, 1, 1)
        lax.fori_loop(0, T, step, 0)
        pltpu.make_async_copy(obuf, o_hbm, osem.at[0]).wait()

    def fn(A_x, A_k, A_v, A_wq, A_wo, B_x, B_k, B_v, B_wq, B_wo):
        def kv(k):
            return jnp.swapaxes(k, 2, 3).reshape(B, H * DH, SK)

        def wo4(w):
            return w.reshape(8, 6, 128, D)
        anyspec = pl.BlockSpec(memory_space=pl.ANY)
        out = pl.pallas_call(
            kernel,
            in_specs=[anyspec] * 10,
            out_specs=anyspec,
            out_shape=jax.ShapeDtypeStruct((B * SQ, 2 * D), bf16),
            scratch_shapes=[pltpu.VMEM((B * SQ, 2 * D), f32),
                            pltpu.VMEM((B * SQ, 2 * D), bf16),
                            pltpu.VMEM((2, 2, nb, SQ, D), bf16),
                            pltpu.VMEM((2, B, 22, HF // 2, 128), u32),
                            pltpu.VMEM((2, 4, nb, GW, SK), bf16),
                            pltpu.VMEM((nbg, 2, 5, SL, GW), bf16),
                            pltpu.VMEM((nbg, 2, 6, SL, D), bf16),
                            pltpu.VMEM((2, 2, 51, 64, 128), u32),
                            pltpu.VMEM((2, 2, 51, 64, 128), u32),
                            pltpu.VMEM((8, 128), u32),
                            pltpu.SemaphoreType.DMA((2,)),
                            pltpu.SemaphoreType.DMA((2, 2)),
                            pltpu.SemaphoreType.DMA((1,)),
                            pltpu.SemaphoreType.DMA((1,)),
                            ],
            compiler_params=pltpu.CompilerParams(
                vmem_limit_bytes=vmem * 1024 * 1024,
                disable_bounds_checks=True),
        )(A_x, kv(A_k), kv(A_v), A_wq, wo4(A_wo), B_x, kv(B_k), kv(B_v), B_wq, wo4(B_wo))
        return out.reshape(B, SQ, 2 * D)
    return fn


@jax.jit
def pallas_concat_heads__gqa_block_cached__mha_block_cached__near_ridge_kernel(A_x, A_k_cache, A_v_cache, A_wq, A_wo, B_x, B_k_cache, B_v_cache, B_wq, B_wo):
    return _build(mq=48)(A_x, A_k_cache, A_v_cache, A_wq, A_wo, B_x, B_k_cache, B_v_cache, B_wq, B_wo)
```

```python
import functools
import jax, jax.numpy as jnp
from jax import lax
from jax.experimental import pallas as pl
from jax.experimental.pallas import tpu as pltpu

B, SQ, D, H, SK, DH = 16, 160, 640, 32, 512, 192
PW = 2 * DH
GW = 2 * PW
LOG2E = 1.4426950408889634
QSCALE = (DH ** -0.5) * LOG2E
NT = (((1,), (1,)), ((), ()))
f32, bf16, u32 = jnp.float32, jnp.bfloat16, jnp.uint32
TT = 128
R = SQ - TT
HF = SQ // 2


def chunks(m, tot=SQ):
    return [(r, min(r + m, tot)) for r in range(0, tot, m)]


def dot(a, b):
    return jnp.dot(a, b, preferred_element_type=f32)


def dotnt(a, b):
    return lax.dot_general(a, b, NT, preferred_element_type=f32)


def unpk(v):
    return pltpu.bitcast(v, bf16)


def s_alpha(a11, a12, a21, a22):
    return [a11 + a22, a21 + a22, a11, a22, a11 + a12, a21 - a11, a12 - a22]


def s_gamma(b11, b12, b21, b22):
    return [b11 + b22, b11, b12 - b22, b21 - b11, b22, b11 + b12, b21 + b22]


S_BETA = {0: ((0, 0, 1), (1, 1, 1)), 3: ((0, 0, 1), (1, 0, 1)), 4: ((0, 0, -1), (0, 1, 1)), 6: ((0, 0, 1),),
          1: ((1, 0, 1), (1, 1, -1)), 2: ((0, 1, 1), (1, 1, 1)), 5: ((1, 1, 1),)}


def h_alpha(x0, x1, x2, y0, y1, y2):
    d0, d1, d2 = x0 - y0, x1 - y1, x2 - y2
    return [x0, d0, d1, y1, x2, y2, x0 - y1, x1 - x0, y1 - y0, d0 + y2, d2 - d0, y0 - y2, d1 - x2, d2 - d1, x2 - x1]


def h_gamma(w00, w01, w02, w10, w11, w12, w20, w21, w22):
    return [w00 - w02 + w10, w00 - w01 + w20, w11 - w10 + w21, w01 + w11 - w12, w12 - w20 + w22, w02 - w21 + w22,
            w01 + w10, w10, w01, w02 + w20, w20, w02, w12 + w21, w21, w12]


H_BETA = {2: ((0, 1, 1),),
          3: ((0, 1, 1), (1, 1, 1)),
          6: ((0, 1, 1), (1, 0, -1)),
          7: ((0, 0, 1), (0, 1, 1)),
          8: ((1, 0, -1), (1, 1, -1)),
          0: ((0, 0, 1), (1, 0, 1)),
          1: ((1, 0, -1),),
          9: ((0, 0, 1), (0, 2, 1), (1, 0, 1)),
          10: ((0, 0, 1), (0, 2, 1)),
          11: ((0, 0, 1), (0, 2, 1), (1, 0, 1), (1, 2, 1)),
          4: ((0, 2, 1),),
          5: ((1, 2, 1),),
          12: ((0, 1, -1), (1, 1, -1), (1, 2, -1)),
          13: ((1, 1, -1), (1, 2, -1)),
          14: ((0, 1, -1), (0, 2, -1), (1, 1, -1), (1, 2, -1))}


def pcombos(blks, fn):
    us = [pltpu.bitcast(b, u32) for b in blks]
    lo_in = [pltpu.unpack_elementwise(u, index=0, packed_dtype=bf16, unpacked_dtype=f32) for u in us]
    hi_in = [pltpu.unpack_elementwise(u, index=1, packed_dtype=bf16, unpacked_dtype=f32) for u in us]
    out = []
    for lo, hi in zip(fn(*lo_in), fn(*hi_in)):
        triv = [k for k, v in enumerate(lo_in) if v is lo]
        out.append(us[triv[0]] if triv else pltpu.pack_elementwise([lo, hi], packed_dtype=bf16).astype(u32))
    return out


def bilinear(beta, order, prod, c, init=None):
    for r in order:
        m = prod(r)
        for (s, j, sg) in beta[r]:
            if (s, j) not in c and init is not None:
                c[(s, j)] = init(s, j)
            if (s, j) in c:
                c[(s, j)] = c[(s, j)] + m if sg > 0 else c[(s, j)] - m
            else:
                c[(s, j)] = m if sg > 0 else -m
    return c


def _build(NG=8, nb=2, vmem=110, mk=160, nk=256, mq=80, mo=80,
          odd="Q0,Q1,Q2,Q3,Q4,K0,K1,P0,P1", even="K0,K1,P0,P1,O0,O1,O2",
          tail=2, qlag=2, mqq=80, dpos=1, sch=4, wq_every=4, wo_every=2, xq_every=3, head="", ltail=2):
    nbg = B // nb
    M = nb * SQ
    T = NG * nbg
    assert nbg == 8
    SL = 128 // nbg
    LG = nbg.bit_length() - 1

    def recip(l):
        r = pl.reciprocal(l, approx=True)
        return r * (2.0 - l * r)

    def soft(s, zvec):
        ps = []
        for r in range(SQ // 8):
            sb = s[r * 8:(r + 1) * 8]
            m = jnp.broadcast_to(jnp.max(sb, axis=-1, keepdims=True), (8, 128))
            if sch and r >= sch:
                link = pltpu.bitcast(ps[r - sch][:, 384:512], u32) & zvec
                m = pltpu.bitcast(pltpu.bitcast(m, u32) | link, f32)
            ps.append(jnp.exp2(sb - jnp.concatenate([m] * 4, axis=1)))
        p = jnp.concatenate(ps, axis=0)
        t = (p[:TT, 0:128] + p[:TT, 128:256]) + (p[:TT, 256:384] + p[:TT, 384:512])
        rrow = recip(jnp.sum(t.T, axis=0, keepdims=True))
        rrem = jnp.broadcast_to(recip(jnp.sum(p[TT:], axis=-1, keepdims=True)), (R, 128))
        return p, (rrow, rrem)

    units = [(p, b) for p in range(2) for b in range(nb)]
    U = len(units)
    n = 2 * U

    def kernel(xa, kta, vta, wqa, woa, xb, ktb, vtb, wqb, wob, o_hbm,
               acc, obuf, xraw, xsb, qbuf, kvbuf, wqraw, woraw, wqc, woc, zv,
               kvsem, wsem, xsem, osem):
        xs, kvs, wqs, wos = (xa, xb), (kta, vta, ktb, vtb), (wqa, wqb), (woa, wob)

        def kv_start(sl, hg_, g_):
            for a in range(4):
                pltpu.make_async_copy(
                    kvs[a].at[pl.ds(g_ * nb, nb), pl.ds(pl.multiple_of(hg_ * GW, GW), GW), :],
                    kvbuf.at[sl, a], kvsem.at[sl]).start()

        def wq_start(hg_, sl, par):
            cq = pl.ds(pl.multiple_of(hg_ * GW, GW), GW)
            for p in range(2):
                for kt in range(5):
                    pltpu.make_async_copy(wqs[p].at[pl.ds(pl.multiple_of(kt * 128 + sl * SL, SL), SL), cq],
                                          wqraw.at[sl, p, kt], wsem.at[par, 0]).start()

        def wo_start(hg_, sl, par):
            for p in range(2):
                pltpu.make_async_copy(wos[p].at[hg_, :, pl.ds(pl.multiple_of(sl * SL, SL), SL), :],
                                      woraw.at[sl, p], wsem.at[par, 1]).start()

        def wait_buf(v, sem):
            pltpu.make_async_copy(v, v, sem).wait()

        def x_start(g_):
            for p in range(2):
                pltpu.make_async_copy(xs[p].at[pl.ds(g_ * nb, nb)], xraw.at[g_ & 1, p], xsem.at[g_ & 1]).start()

        def ct(c):
            return slice(c * 128, (c + 1) * 128)

        def wq_piece(ws, sl, p, kind, a):
            rs = pl.ds(pl.multiple_of(sl * (SL // 2), 8), SL // 2)
            if kind == 0:
                blk = [wqraw[sl, p, kt, :, ct(a + 3 * c)] for kt in range(2) for c in range(2)]
                for k, v in enumerate(pcombos(blk, s_gamma)):
                    wqc[ws, p, a * 7 + k, rs, :] = v
            else:
                blk = [wqraw[sl, p, 2 + i, :, ct(3 * a + j)] for i in range(3) for j in range(3)]
                for r, v in enumerate(pcombos(blk, h_gamma)):
                    wqc[ws, p, 21 + a * 15 + r, rs, :] = v

        def wo_piece(ws, sl, p, kind, a):
            rs = pl.ds(pl.multiple_of(sl * (SL // 2), 8), SL // 2)
            if kind == 0:
                blk = [woraw[sl, p, a + 3 * r, :, ct(c)] for r in range(2) for c in range(2)]
                for k, v in enumerate(pcombos(blk, s_gamma)):
                    woc[ws, p, k * 3 + a, rs, :] = v
            else:
                blk = [woraw[sl, p, 3 * a + i, :, ct(2 + j)] for i in range(3) for j in range(3)]
                for r, v in enumerate(pcombos(blk, h_gamma)):
                    woc[ws, p, 21 + r * 2 + a, rs, :] = v

        w_pieces = [(p, kind, a) for p in range(2) for kind in range(2) for a in range(3 - kind)]

        def x_piece(g_, p, b, kind, r0):
            rs = slice(r0, r0 + 16)

            def blk(r, kt):
                return xraw[g_ & 1, p, b, r * HF + r0:r * HF + r0 + 16, ct(kt)]
            if kind == 0:
                cs = pcombos([blk(r, kt) for r in range(2) for kt in range(2)], s_alpha)
            else:
                cs = pcombos([blk(r, kt) for r in range(2) for kt in range(2, 5)], h_alpha)
            for k, v in enumerate(cs):
                xsb[p, g_ * nb + b, 7 * kind + k, r0 // 2:r0 // 2 + 8, :] = v

        x_pieces = [(p, b, kind, r0) for p in range(2) for b in range(nb) for r0 in range(0, HF, 16) for kind in range(2)]

        def body(mode, t):
            g = t & (nbg - 1)
            hg1 = lax.shift_right_logical(t, LG)
            hg = hg1 - 1
            par = t & 1
            slot = lax.rem(t + 1, 3)
            qslot = hg1 & 1
            wslot = 1 - qslot
            row0 = pl.multiple_of(g * M, M)

            def starts():
                t1, t2 = t + 1, t + 2
                if mode != "q":
                    @pl.when(t2 < T + nbg)
                    def _():
                        kv_start(lax.rem(t, 3), lax.shift_right_logical(t2, LG) - 1, t2 & (nbg - 1))
                if mode != "l":
                    hg2 = lax.shift_right_logical(t2, LG)

                    @pl.when(hg2 + 1 < NG)
                    def _():
                        wq_start(hg2 + 1, t2 & (nbg - 1), par)

                    @pl.when(hg2 < NG)
                    def _():
                        wo_start(hg2, t2 & (nbg - 1), par)

            if mode == "q":
                @pl.when(g + 2 < nbg)
                def _():
                    x_start(g + 2)
                for a in range(4):
                    for b in range(nb):
                        @pl.when(g == a * nb + b)
                        def _():
                            pltpu.make_async_copy(kvs[a].at[b, pl.ds(0, GW), :], kvbuf.at[0, a, b], kvsem.at[0]).start()

            if mode == "q":
                @pl.when(g + 1 < nbg)
                def _():
                    wait_buf(xraw.at[(g + 1) & 1], xsem.at[(g + 1) & 1])
            if mode != "l":
                @pl.when(hg1 + 1 < NG)
                def _():
                    wait_buf(wqraw.at[g], wsem.at[par, 0])
                wait_buf(woraw.at[g], wsem.at[par, 1])
            if mode != "q":
                wait_buf(kvbuf.at[slot], kvsem.at[slot])

            st = [dict() for _ in range(n)]
            mq_ = mqq if mode == "q" else mq
            zvec = zv[...]
            jq = [functools.partial(wq_piece, 1 - qslot, g, *a) for a in w_pieces]
            jo = [functools.partial(wo_piece, 1 - wslot, g, *a) for a in w_pieces]
            gx = jnp.minimum(g + 1, nbg - 1)
            jx = [functools.partial(x_piece, gx, *a) for a in x_pieces]
            todo = {"q": {"q": jq + jo, "o": [], "x": jx}, "m": {"q": jq, "o": jo, "x": []},
                    "l": {"q": [], "o": [], "x": []}}[mode]
            cnt = {"q": 0, "o": 0, "x": 0}
            every = {"q": wq_every, "o": wo_every, "x": xq_every}

            def host(kind):
                cnt[kind] += 1
                if every[kind] and cnt[kind] % every[kind] == 0 and todo[kind]:
                    todo[kind].pop(0)()

            def task_q(u, j):
                p, b = units[u]
                bb = g * nb + b
                d = st[2 * u].setdefault("qc", {})
                for (a, e) in chunks(mq_, HF):
                    c = d.setdefault(a, {})

                    def prod(xk, wk):
                        host("q")
                        host("x")
                        return dot(unpk(xsb[p, bb, xk, a // 2:e // 2, :]), unpk(wqc[qslot, p, wk]))
                    if j < 2:
                        sub = bilinear(H_BETA, list(H_BETA), lambda r: prod(7 + r, 21 + j * 15 + r),
                                       {(s, jj): c[(s, 3 * j + jj)] for s in range(2) for jj in range(3) if (s, 3 * j + jj) in c})
                        for (s, jj), v in sub.items():
                            c[(s, 3 * j + jj)] = v
                    else:
                        jj = j - 2
                        sub = bilinear(S_BETA, list(S_BETA), lambda k: prod(k, jj * 7 + k),
                                       {(s, cc): c[(s, jj + 3 * cc)] for s in range(2) for cc in range(2) if (s, jj + 3 * cc) in c})
                        for (s, cc), v in sub.items():
                            c[(s, jj + 3 * cc)] = v

                done = st[2 * u].setdefault("qdone", set())
                done.add(j)
                for col in range(6):
                    if {col // 3, 2 + col % 3} <= done and col + 10 not in done:
                        done.add(col + 10)
                        v = jnp.concatenate([d[a][(s, col)] for s in range(2) for (a, e) in chunks(mq_, HF)], axis=0)
                        qbuf[g, u, col] = pltpu.bitcast((v * QSCALE).astype(bf16), u32)

            def task_k(i, h):
                p, b = units[i // 2]
                k0 = (i % 2) * PW
                kt = kvbuf.at[slot, 2 * p, b]
                d = st[i]
                lane = lax.broadcasted_iota(jnp.int32, (HF, 128), 1)
                qm = qbuf[g, i // 2, 3 * (i % 2) + 1]
                if h == 0:
                    l = [qbuf[g, i // 2, 3 * (i % 2)], jnp.where(lane < 64, qm, jnp.uint32(0))]
                else:
                    l = [jnp.where(lane >= 64, qm, jnp.uint32(0)), qbuf[g, i // 2, 3 * (i % 2) + 2]]
                l = jnp.concatenate(l, axis=1)
                rows = []
                for (a, e) in chunks(mk):
                    lc = unpk(l[a // 2:e // 2])
                    cs = [dot(lc, kt[k0 + h * 128:k0 + h * 128 + 256, c:c + nk]) for c in range(0, SK, nk)]
                    rows.append(jnp.concatenate(cs, axis=1))
                pp, rr = soft(jnp.concatenate(rows, axis=0), zvec)
                d["p%d" % h], d["r%d" % h] = pp, rr

            def task_p(i, h):
                p, b = units[i // 2]
                k0 = (i % 2) * PW
                vt = kvbuf.at[slot, 2 * p + 1, b]
                d = st[i]
                if h == 0:
                    d["ot1"] = dotnt(vt[k0:k0 + 192, :], d["p0"][:TT].astype(bf16))
                    d["oa"] = dotnt(d["p0"][TT:].astype(bf16), vt[k0:k0 + 128, :])
                else:
                    p1, r1, p2, r2 = d["p0"], d["r0"], d["p1"], d["r1"]
                    om = dotnt(jnp.concatenate([p1[TT:], p2[TT:]], axis=0).astype(bf16), vt[k0 + 128:k0 + 256, :])
                    ot2 = dotnt(vt[k0 + 192:k0 + 384, :], p2[:TT].astype(bf16))
                    oc = dotnt(p2[TT:].astype(bf16), vt[k0 + 256:k0 + 384, :])
                    ot1 = d["ot1"] * r1[0]
                    ot2 = ot2 * r2[0]
                    lane = lax.broadcasted_iota(jnp.int32, (R, 128), 1)
                    omr = jnp.where(lane < 64, om[:R] * r1[1], om[R:] * r2[1])
                    ta = ot1[0:128].T
                    tm = jnp.concatenate([ot1[128:192], ot2[0:64]], axis=0).T
                    tc = ot2[64:192].T
                    d["o"] = [jnp.concatenate([ta, d["oa"] * r1[1]], axis=0),
                              jnp.concatenate([tm, omr], axis=0),
                              jnp.concatenate([tc, oc * r2[1]], axis=0)]

            H_SPLIT = [list(H_BETA)[:7], list(H_BETA)[7:]]

            def task_o(u, j):
                p, b = units[u]
                d = st[2 * u]
                if "os" not in d:
                    o1, o2 = st[2 * u]["o"], st[2 * u + 1]["o"]
                    f1, f2 = jnp.concatenate(o1, axis=1), jnp.concatenate(o2, axis=1)
                    d["os"] = s_alpha(f1[:HF], f2[:HF], f1[HF:], f2[HF:])
                    h1 = h_alpha(*([v[:HF] for v in o1] + [v[HF:] for v in o1]))
                    h2 = h_alpha(*([v[:HF] for v in o2] + [v[HF:] for v in o2]))
                    d["oh"] = [jnp.concatenate([v1, v2], axis=1) for v1, v2 in zip(h1, h2)]
                    d["hc"] = {}

                for (a, e) in chunks(mo, HF):
                    def idx(s, col):
                        c0 = p * D + col * 128
                        return pl.ds(pl.multiple_of(row0 + b * SQ + s * HF + a, 16), e - a), slice(c0, c0 + 128)

                    def accv(s, col):
                        return jnp.where(hg == 0, 0.0, acc[idx(s, col)]) if mode == "m" else acc[idx(s, col)]

                    def put(s, col, v):
                        if mode == "l":
                            obuf[idx(s, col)] = v.astype(bf16)
                        else:
                            acc[idx(s, col)] = v

                    def prod(lhs, w0, nt):
                        host("o")
                        w = woc[wslot, p, w0:w0 + nt].reshape(nt * 64, 128)
                        return dot(lhs[a:e].astype(bf16), unpk(w))
                    if j == 0:
                        c = bilinear(S_BETA, list(S_BETA), lambda k: prod(d["os"][k], k * 3, 3), {}, accv)
                        for (s, col), v in c.items():
                            put(s, col, v)
                    else:
                        c = bilinear(H_BETA, H_SPLIT[j - 1], lambda r: prod(d["oh"][r], 21 + r * 2, 2),
                                     d["hc"].setdefault(a, {}), lambda s, col: accv(s, 2 + col))
                        if j == 2:
                            for (s, col), v in c.items():
                                put(s, 2 + col, v)

            seq = []
            if mode == "q":
                seq = [("Q", u, j) for u in range(U) for j in range(5)]
            else:
                for s in range(-3, n + 1):
                    for tok in (odd if s % 2 else even).split(","):
                        k, j = tok[0], int(tok[1])
                        if k == "Q":
                            u = (s + 1) // 2 + 1 - qlag
                            if 0 <= u < U and mode == "m": seq.append(("Q", u, j))
                        elif k == "O":
                            u = s // 2 - 1
                            if 0 <= u < U: seq.append(("O", u, j))
                        elif k == "K":
                            if 0 <= s + 1 < n: seq.append(("K", s + 1, j))
                        else:
                            if 0 <= s < n: seq.append(("P", s, j))
                tl = tail if mode == "m" else ltail
                if tl:
                    mv = [x for x in seq if x[0] == "O" and x[1] == U - 2][-tl:]
                    seq = [x for x in seq if x not in mv]
                    pos = seq.index(("P", n - 1, 1)) + 1
                    seq = seq[:pos] + mv + seq[pos:]
            fns = {"Q": task_q, "K": task_k, "P": task_p, "O": task_o}
            for ti, tk in enumerate(seq):
                if ti == dpos:
                    starts()
                fns[tk[0]](tk[1], tk[2])
            for lst in todo.values():
                for job in lst:
                    job()
            if mode == "l":
                rs = pl.ds(row0, M)
                pltpu.make_async_copy(obuf.at[rs, :], o_hbm.at[rs, :], osem.at[0]).start()

        zv[...] = jnp.zeros((8, 128), u32)

        def loop(lo, hi, fn):
            def w(i, c):
                fn(i)
                return c
            lax.fori_loop(lo, hi, w, 0)

        loop(0, nbg, lambda sl: wq_start(0, sl, 0))
        x_start(0)
        x_start(1)
        wait_buf(wqraw, wsem.at[0, 0])

        def pro(sl):
            for a in w_pieces:
                wq_piece(0, sl, *a)
        loop(0, nbg, pro)
        for k in range(2):
            wq_start(1, k, k)
            wo_start(0, k, k)
        wait_buf(xraw.at[0], xsem.at[0])
        for a in x_pieces:
            x_piece(0, *a)
        loop(0, nbg, functools.partial(body, "q"))
        kv_start(1, 0, 1)
        loop(nbg, T, functools.partial(body, "m"))
        loop(T, T + nbg, functools.partial(body, "l"))
        pltpu.make_async_copy(obuf, o_hbm, osem.at[0]).wait()

    def fn(A_x, A_k, A_v, A_wq, A_wo, B_x, B_k, B_v, B_wq, B_wo):
        def kv(k):
            return jnp.swapaxes(k, 2, 3).reshape(B, H * DH, SK)

        def wo4(w):
            return w.reshape(8, 6, 128, D)
        anyspec = pl.BlockSpec(memory_space=pl.ANY)
        out = pl.pallas_call(
            kernel,
            in_specs=[anyspec] * 10,
            out_specs=anyspec,
            out_shape=jax.ShapeDtypeStruct((B * SQ, 2 * D), bf16),
            scratch_shapes=[pltpu.VMEM((B * SQ, 2 * D), f32),
                            pltpu.VMEM((B * SQ, 2 * D), bf16),
                            pltpu.VMEM((2, 2, nb, SQ, D), bf16),
                            pltpu.VMEM((2, B, 22, HF // 2, 128), u32),
                            pltpu.VMEM((nbg, U, 6, HF, 128), u32),
                            pltpu.VMEM((3, 4, nb, GW, SK), bf16),
                            pltpu.VMEM((nbg, 2, 5, SL, GW), bf16),
                            pltpu.VMEM((nbg, 2, 6, SL, D), bf16),
                            pltpu.VMEM((2, 2, 51, 64, 128), u32),
                            pltpu.VMEM((2, 2, 51, 64, 128), u32),
                            pltpu.VMEM((8, 128), u32),
                            pltpu.SemaphoreType.DMA((3,)),
                            pltpu.SemaphoreType.DMA((2, 2)),
                            pltpu.SemaphoreType.DMA((2,)),
                            pltpu.SemaphoreType.DMA((1,)),
                            ],
            compiler_params=pltpu.CompilerParams(
                vmem_limit_bytes=vmem * 1024 * 1024,
                disable_bounds_checks=True),
        )(A_x, kv(A_k), kv(A_v), A_wq, wo4(A_wo), B_x, kv(B_k), kv(B_v), B_wq, wo4(B_wo))
        return out.reshape(B, SQ, 2 * D)
    return fn


@jax.jit
def pallas_concat_heads__gqa_block_cached__mha_block_cached__near_ridge_kernel(A_x, A_k_cache, A_v_cache, A_wq, A_wo, B_x, B_k_cache, B_v_cache, B_wq, B_wo):
    return _build(mq=48, tail=1, ltail=1)(A_x, A_k_cache, A_v_cache, A_wq, A_wo, B_x, B_k_cache, B_v_cache, B_wq, B_wo)
```

```python
import functools
import jax, jax.numpy as jnp
from jax import lax
from jax.experimental import pallas as pl
from jax.experimental.pallas import tpu as pltpu

B, SQ, D, H, SK, DH = 16, 160, 640, 32, 512, 192
PW = 2 * DH
GW = 2 * PW
LOG2E = 1.4426950408889634
QSCALE = (DH ** -0.5) * LOG2E
NT = (((1,), (1,)), ((), ()))
f32, bf16, u32 = jnp.float32, jnp.bfloat16, jnp.uint32
TT = 128
R = SQ - TT
HF = SQ // 2


def chunks(m, tot=SQ):
    return [(r, min(r + m, tot)) for r in range(0, tot, m)]


def dot(a, b):
    return jnp.dot(a, b, preferred_element_type=f32)


def dotnt(a, b):
    return lax.dot_general(a, b, NT, preferred_element_type=f32)


def unpk(v):
    return pltpu.bitcast(v, bf16)


def s_alpha(a11, a12, a21, a22):
    return [a11 + a22, a21 + a22, a11, a22, a11 + a12, a21 - a11, a12 - a22]


def s_gamma(b11, b12, b21, b22):
    return [b11 + b22, b11, b12 - b22, b21 - b11, b22, b11 + b12, b21 + b22]


S_BETA = {0: ((0, 0, 1), (1, 1, 1)), 3: ((0, 0, 1), (1, 0, 1)), 4: ((0, 0, -1), (0, 1, 1)), 6: ((0, 0, 1),),
          1: ((1, 0, 1), (1, 1, -1)), 2: ((0, 1, 1), (1, 1, 1)), 5: ((1, 1, 1),)}


def h_alpha(x0, x1, x2, y0, y1, y2):
    d0, d1, d2 = x0 - y0, x1 - y1, x2 - y2
    return [x0, d0, d1, y1, x2, y2, x0 - y1, x1 - x0, y1 - y0, d0 + y2, d2 - d0, y0 - y2, d1 - x2, d2 - d1, x2 - x1]


def h_gamma(w00, w01, w02, w10, w11, w12, w20, w21, w22):
    return [w00 - w02 + w10, w00 - w01 + w20, w11 - w10 + w21, w01 + w11 - w12, w12 - w20 + w22, w02 - w21 + w22,
            w01 + w10, w10, w01, w02 + w20, w20, w02, w12 + w21, w21, w12]


H_BETA = {2: ((0, 1, 1),),
          3: ((0, 1, 1), (1, 1, 1)),
          6: ((0, 1, 1), (1, 0, -1)),
          7: ((0, 0, 1), (0, 1, 1)),
          8: ((1, 0, -1), (1, 1, -1)),
          0: ((0, 0, 1), (1, 0, 1)),
          1: ((1, 0, -1),),
          9: ((0, 0, 1), (0, 2, 1), (1, 0, 1)),
          10: ((0, 0, 1), (0, 2, 1)),
          11: ((0, 0, 1), (0, 2, 1), (1, 0, 1), (1, 2, 1)),
          4: ((0, 2, 1),),
          5: ((1, 2, 1),),
          12: ((0, 1, -1), (1, 1, -1), (1, 2, -1)),
          13: ((1, 1, -1), (1, 2, -1)),
          14: ((0, 1, -1), (0, 2, -1), (1, 1, -1), (1, 2, -1))}


def pcombos(blks, fn):
    us = [pltpu.bitcast(b, u32) for b in blks]
    lo_in = [pltpu.unpack_elementwise(u, index=0, packed_dtype=bf16, unpacked_dtype=f32) for u in us]
    hi_in = [pltpu.unpack_elementwise(u, index=1, packed_dtype=bf16, unpacked_dtype=f32) for u in us]
    out = []
    for lo, hi in zip(fn(*lo_in), fn(*hi_in)):
        triv = [k for k, v in enumerate(lo_in) if v is lo]
        out.append(us[triv[0]] if triv else pltpu.pack_elementwise([lo, hi], packed_dtype=bf16).astype(u32))
    return out


def bilinear(beta, order, prod, c, init=None):
    for r in order:
        m = prod(r)
        for (s, j, sg) in beta[r]:
            if (s, j) not in c and init is not None:
                c[(s, j)] = init(s, j)
            if (s, j) in c:
                c[(s, j)] = c[(s, j)] + m if sg > 0 else c[(s, j)] - m
            else:
                c[(s, j)] = m if sg > 0 else -m
    return c


def _build(NG=8, nb=2, vmem=110, mk=160, nk=256, mq=48, mo=80,
          odd="Q0,Q1,Q2,Q3,Q4,K0,K1,P0,P1", even="K0,K1,P0,P1,O0,O1,O2",
          tail=1, qlag=2, mqq=80, dpos=1, sch=4, wq_every=4, wo_every=2, xq_every=3, head="", ltail=1, only="qml", horder=0, osplit=7, och=0, pord=0):
    nbg = B // nb
    M = nb * SQ
    T = NG * nbg
    assert nbg == 8
    SL = 128 // nbg
    LG = nbg.bit_length() - 1

    def recip(l):
        r = pl.reciprocal(l, approx=True)
        return r * (2.0 - l * r)

    def soft(s, zvec):
        ps = []
        for r in range(SQ // 8):
            sb = s[r * 8:(r + 1) * 8]
            m = jnp.broadcast_to(jnp.max(sb, axis=-1, keepdims=True), (8, 128))
            if sch and r >= sch:
                link = pltpu.bitcast(ps[r - sch][:, 384:512], u32) & zvec
                m = pltpu.bitcast(pltpu.bitcast(m, u32) | link, f32)
            ps.append(jnp.exp2(sb - jnp.concatenate([m] * 4, axis=1)))
        p = jnp.concatenate(ps, axis=0)
        t = (p[:TT, 0:128] + p[:TT, 128:256]) + (p[:TT, 256:384] + p[:TT, 384:512])
        rrow = recip(jnp.sum(t.T, axis=0, keepdims=True))
        rrem = jnp.broadcast_to(recip(jnp.sum(p[TT:], axis=-1, keepdims=True)), (R, 128))
        return p, (rrow, rrem)

    HORD = [[2, 3, 6, 7, 8, 0, 1, 9, 10, 11, 4, 5, 12, 13, 14],
            [6, 7, 8, 2, 3, 12, 13, 14, 4, 5, 9, 10, 11, 0, 1],
            [0, 1, 7, 6, 8, 2, 3, 14, 12, 13, 4, 5, 10, 9, 11],
            [4, 5, 10, 9, 11, 0, 1, 7, 6, 8, 2, 3, 14, 12, 13]][horder]
    units = [(p, b) for p in range(2) for b in range(nb)]
    U = len(units)
    n = 2 * U

    def kernel(xa, kta, vta, wqa, woa, xb, ktb, vtb, wqb, wob, o_hbm,
               acc, obuf, xraw, xsb, qbuf, kvbuf, wqraw, woraw, wqc, woc, zv,
               kvsem, wsem, xsem, osem):
        xs, kvs, wqs, wos = (xa, xb), (kta, vta, ktb, vtb), (wqa, wqb), (woa, wob)

        def kv_start(sl, hg_, g_):
            for a in range(4):
                pltpu.make_async_copy(
                    kvs[a].at[pl.ds(g_ * nb, nb), pl.ds(pl.multiple_of(hg_ * GW, GW), GW), :],
                    kvbuf.at[sl, a], kvsem.at[sl]).start()

        def kv_piece(k):
            a, b = k // nb, k % nb
            pltpu.make_async_copy(kvs[a].at[b, pl.ds(0, GW), :], kvbuf.at[0, a, b], kvsem.at[0]).start()

        def wq_start(hg_, sl, par):
            cq = pl.ds(pl.multiple_of(hg_ * GW, GW), GW)
            for p in range(2):
                for kt in range(5):
                    pltpu.make_async_copy(wqs[p].at[pl.ds(pl.multiple_of(kt * 128 + sl * SL, SL), SL), cq],
                                          wqraw.at[sl, p, kt], wsem.at[par, 0]).start()

        def wo_start(hg_, sl, par):
            for p in range(2):
                pltpu.make_async_copy(wos[p].at[hg_, :, pl.ds(pl.multiple_of(sl * SL, SL), SL), :],
                                      woraw.at[sl, p], wsem.at[par, 1]).start()

        def wait_buf(v, sem):
            pltpu.make_async_copy(v, v, sem).wait()

        def x_start(g_):
            for p in range(2):
                pltpu.make_async_copy(xs[p].at[pl.ds(g_ * nb, nb)], xraw.at[g_ & 1, p], xsem.at[g_ & 1]).start()

        def ct(c):
            return slice(c * 128, (c + 1) * 128)

        def wq_piece(ws, sl, p, kind, a):
            rs = pl.ds(pl.multiple_of(sl * (SL // 2), 8), SL // 2)
            if kind == 0:
                blk = [wqraw[sl, p, kt, :, ct(a + 3 * c)] for kt in range(2) for c in range(2)]
                for k, v in enumerate(pcombos(blk, s_gamma)):
                    wqc[ws, p, a * 7 + k, rs, :] = v
            else:
                blk = [wqraw[sl, p, 2 + i, :, ct(3 * a + j)] for i in range(3) for j in range(3)]
                for r, v in enumerate(pcombos(blk, h_gamma)):
                    wqc[ws, p, 21 + a * 15 + r, rs, :] = v

        def wo_piece(ws, sl, p, kind, a):
            rs = pl.ds(pl.multiple_of(sl * (SL // 2), 8), SL // 2)
            if kind == 0:
                blk = [woraw[sl, p, a + 3 * r, :, ct(c)] for r in range(2) for c in range(2)]
                for k, v in enumerate(pcombos(blk, s_gamma)):
                    woc[ws, p, k * 3 + a, rs, :] = v
            else:
                blk = [woraw[sl, p, 3 * a + i, :, ct(2 + j)] for i in range(3) for j in range(3)]
                for r, v in enumerate(pcombos(blk, h_gamma)):
                    woc[ws, p, 21 + r * 2 + a, rs, :] = v

        w_pieces = [(p, kind, a) for p in range(2) for kind in range(2) for a in range(3 - kind)]

        def x_piece(g_, p, b, kind, r0):
            rs = slice(r0, r0 + 16)

            def blk(r, kt):
                return xraw[g_ & 1, p, b, r * HF + r0:r * HF + r0 + 16, ct(kt)]
            if kind == 0:
                cs = pcombos([blk(r, kt) for r in range(2) for kt in range(2)], s_alpha)
            else:
                cs = pcombos([blk(r, kt) for r in range(2) for kt in range(2, 5)], h_alpha)
            for k, v in enumerate(cs):
                xsb[p, g_ * nb + b, 7 * kind + k, r0 // 2:r0 // 2 + 8, :] = v

        x_pieces = [(p, b, kind, r0) for p in range(2) for b in range(nb) for r0 in range(0, HF, 16) for kind in range(2)]

        def body(mode, t, slot):
            g = t & (nbg - 1)
            hg1 = lax.shift_right_logical(t, LG)
            hg = hg1 - 1
            par = t & 1
            slot2 = jnp.where(slot == 0, 2, slot - 1)
            qslot = hg1 & 1
            wslot = 1 - qslot
            row0 = pl.multiple_of(g * M, M)

            def starts():
                t1, t2 = t + 1, t + 2
                if mode != "q":
                    @pl.when(t2 < T + nbg)
                    def _():
                        kv_start(slot2, lax.shift_right_logical(t2, LG) - 1, t2 & (nbg - 1))
                if mode == "q":
                    for k in range(1, nbg):
                        pl.when(g + 1 == k)(functools.partial(kv_piece, k))
                if mode != "l":
                    hg2 = lax.shift_right_logical(t2, LG)

                    @pl.when(hg2 + 1 < NG)
                    def _():
                        wq_start(hg2 + 1, t2 & (nbg - 1), par)

                    @pl.when(hg2 < NG)
                    def _():
                        wo_start(hg2, t2 & (nbg - 1), par)

            if mode == "q":
                @pl.when(g + 2 < nbg)
                def _():
                    x_start(g + 2)

            if mode == "q":
                @pl.when(g + 1 < nbg)
                def _():
                    wait_buf(xraw.at[(g + 1) & 1], xsem.at[(g + 1) & 1])
            if mode != "l":
                @pl.when(hg1 + 1 < NG)
                def _():
                    wait_buf(wqraw.at[g], wsem.at[par, 0])
                wait_buf(woraw.at[g], wsem.at[par, 1])
            if mode != "q":
                wait_buf(kvbuf.at[slot], kvsem.at[slot])

            st = [dict() for _ in range(n)]
            mq_ = mqq if mode == "q" else mq
            zvec = zv[...]
            jq = [functools.partial(wq_piece, 1 - qslot, g, *a) for a in w_pieces]
            jo = [functools.partial(wo_piece, 1 - wslot, g, *a) for a in w_pieces]
            gx = jnp.minimum(g + 1, nbg - 1)
            jx = [functools.partial(x_piece, gx, *a) for a in x_pieces]
            todo = {"q": {"q": jq + jo, "o": [], "x": jx}, "m": {"q": jq, "o": jo, "x": []},
                    "l": {"q": [], "o": [], "x": []}}[mode]
            cnt = {"q": 0, "o": 0, "x": 0}
            every = {"q": wq_every, "o": wo_every, "x": xq_every}

            def host(kind):
                cnt[kind] += 1
                if every[kind] and cnt[kind] % every[kind] == 0 and todo[kind]:
                    todo[kind].pop(0)()

            def task_q(u, j):
                p, b = units[u]
                bb = g * nb + b
                d = st[2 * u].setdefault("qc", {})
                for (a, e) in chunks(mq_, HF):
                    c = d.setdefault(a, {})

                    def prod(xk, wk):
                        host("q")
                        host("x")
                        return dot(unpk(xsb[p, bb, xk, a // 2:e // 2, :]), unpk(wqc[qslot, p, wk]))
                    if j < 2:
                        sub = bilinear(H_BETA, HORD, lambda r: prod(7 + r, 21 + j * 15 + r),
                                       {(s, jj): c[(s, 3 * j + jj)] for s in range(2) for jj in range(3) if (s, 3 * j + jj) in c})
                        for (s, jj), v in sub.items():
                            c[(s, 3 * j + jj)] = v
                    else:
                        jj = j - 2
                        sub = bilinear(S_BETA, list(S_BETA), lambda k: prod(k, jj * 7 + k),
                                       {(s, cc): c[(s, jj + 3 * cc)] for s in range(2) for cc in range(2) if (s, jj + 3 * cc) in c})
                        for (s, cc), v in sub.items():
                            c[(s, jj + 3 * cc)] = v

                done = st[2 * u].setdefault("qdone", set())
                done.add(j)
                for col in range(6):
                    if {col // 3, 2 + col % 3} <= done and col + 10 not in done:
                        done.add(col + 10)
                        v = jnp.concatenate([d[a][(s, col)] for s in range(2) for (a, e) in chunks(mq_, HF)], axis=0)
                        qbuf[g, u, col] = pltpu.bitcast((v * QSCALE).astype(bf16), u32)

            def task_k(i, h):
                p, b = units[i // 2]
                k0 = (i % 2) * PW
                kt = kvbuf.at[slot, 2 * p, b]
                d = st[i]
                lane = lax.broadcasted_iota(jnp.int32, (HF, 128), 1)
                qm = qbuf[g, i // 2, 3 * (i % 2) + 1]
                if h == 0:
                    l = [qbuf[g, i // 2, 3 * (i % 2)], jnp.where(lane < 64, qm, jnp.uint32(0))]
                else:
                    l = [jnp.where(lane >= 64, qm, jnp.uint32(0)), qbuf[g, i // 2, 3 * (i % 2) + 2]]
                l = jnp.concatenate(l, axis=1)
                rows = []
                for (a, e) in chunks(mk):
                    lc = unpk(l[a // 2:e // 2])
                    cs = [dot(lc, kt[k0 + h * 128:k0 + h * 128 + 256, c:c + nk]) for c in range(0, SK, nk)]
                    rows.append(jnp.concatenate(cs, axis=1))
                pp, rr = soft(jnp.concatenate(rows, axis=0), zvec)
                d["p%d" % h], d["r%d" % h] = pp, rr

            def task_p(i, h):
                p, b = units[i // 2]
                k0 = (i % 2) * PW
                vt = kvbuf.at[slot, 2 * p + 1, b]
                d = st[i]
                if h == 0:
                    d["ot1"] = dotnt(vt[k0:k0 + 192, :], d["p0"][:TT].astype(bf16))
                    d["oa"] = dotnt(d["p0"][TT:].astype(bf16), vt[k0:k0 + 128, :])
                else:
                    p1, r1, p2, r2 = d["p0"], d["r0"], d["p1"], d["r1"]
                    fm = lambda: dotnt(jnp.concatenate([p1[TT:], p2[TT:]], axis=0).astype(bf16), vt[k0 + 128:k0 + 256, :])
                    f2 = lambda: dotnt(vt[k0 + 192:k0 + 384, :], p2[:TT].astype(bf16))
                    fc = lambda: dotnt(p2[TT:].astype(bf16), vt[k0 + 256:k0 + 384, :])
                    if pord == 0:
                        om = fm(); ot2 = f2(); oc = fc()
                    elif pord == 1:
                        ot2 = f2(); om = fm(); oc = fc()
                    else:
                        ot2 = f2(); oc = fc(); om = fm()
                    ot1 = d["ot1"] * r1[0]
                    ot2 = ot2 * r2[0]
                    lane = lax.broadcasted_iota(jnp.int32, (R, 128), 1)
                    omr = jnp.where(lane < 64, om[:R] * r1[1], om[R:] * r2[1])
                    ta = ot1[0:128].T
                    tm = jnp.concatenate([ot1[128:192], ot2[0:64]], axis=0).T
                    tc = ot2[64:192].T
                    d["o"] = [jnp.concatenate([ta, d["oa"] * r1[1]], axis=0),
                              jnp.concatenate([tm, omr], axis=0),
                              jnp.concatenate([tc, oc * r2[1]], axis=0)]

            H_SPLIT = [HORD[:osplit], HORD[osplit:]]

            def task_o(u, j):
                p, b = units[u]
                d = st[2 * u]
                if "os" not in d:
                    o1, o2 = st[2 * u]["o"], st[2 * u + 1]["o"]
                    f1, f2 = jnp.concatenate(o1, axis=1), jnp.concatenate(o2, axis=1)
                    d["os"] = s_alpha(f1[:HF], f2[:HF], f1[HF:], f2[HF:])
                    h1 = h_alpha(*([v[:HF] for v in o1] + [v[HF:] for v in o1]))
                    h2 = h_alpha(*([v[:HF] for v in o2] + [v[HF:] for v in o2]))
                    d["oh"] = [jnp.concatenate([v1, v2], axis=1) for v1, v2 in zip(h1, h2)]
                    d["hc"] = {}

                for (a, e) in chunks(mo, HF):
                    def idx(s, col):
                        c0 = p * D + col * 128
                        return pl.ds(pl.multiple_of(row0 + b * SQ + s * HF + a, 16), e - a), slice(c0, c0 + 128)

                    def accv(s, col):
                        return jnp.where(hg == 0, 0.0, acc[idx(s, col)]) if mode == "m" else acc[idx(s, col)]

                    def put(s, col, v):
                        if mode == "l":
                            obuf[idx(s, col)] = v.astype(bf16)
                        else:
                            acc[idx(s, col)] = v

                    def prod(lhs, w0, nt):
                        host("o")
                        w = woc[wslot, p, w0:w0 + nt].reshape(nt * 64, 128)
                        return dot(lhs[a:e].astype(bf16), unpk(w))
                    if j == 0:
                        c = bilinear(S_BETA, list(S_BETA), lambda k: prod(d["os"][k], k * 3, 3), {}, accv)
                        for (s, col), v in c.items():
                            put(s, col, v)
                    else:
                        c = bilinear(H_BETA, H_SPLIT[j - 1], lambda r: prod(d["oh"][r], 21 + r * 2, 2),
                                     d["hc"].setdefault(a, {}), lambda s, col: accv(s, 2 + col))
                        if j == 2:
                            for (s, col), v in c.items():
                                put(s, 2 + col, v)
                d["odone"] = d.get("odone", 0) + 1
                if mode == "l" and d["odone"] == 3:
                    rs = pl.ds(pl.multiple_of(row0 + b * SQ, 16), SQ)
                    pltpu.make_async_copy(obuf.at[rs, p * D:(p + 1) * D], o_hbm.at[rs, p * D:(p + 1) * D], osem.at[0]).start()

            seq = []
            if mode == "q":
                seq = [("Q", u, j) for u in range(U) for j in range(5)]
            else:
                for s in range(-3, n + 1):
                    for tok in (odd if s % 2 else even).split(","):
                        k, j = tok[0], int(tok[1])
                        if k == "Q":
                            u = (s + 1) // 2 + 1 - qlag
                            if 0 <= u < U and mode == "m": seq.append(("Q", u, j))
                        elif k == "O":
                            u = s // 2 - 1
                            if 0 <= u < U: seq.append(("O", u, j))
                        elif k == "K":
                            if 0 <= s + 1 < n: seq.append(("K", s + 1, j))
                        else:
                            if 0 <= s < n: seq.append(("P", s, j))
                tl = tail if mode == "m" else ltail
                if tl:
                    mv = [x for x in seq if x[0] == "O" and x[1] == U - 2][-tl:]
                    seq = [x for x in seq if x not in mv]
                    pos = seq.index(("P", n - 1, 1)) + 1
                    seq = seq[:pos] + mv + seq[pos:]
            fns = {"Q": task_q, "K": task_k, "P": task_p, "O": task_o}
            if mode not in only:
                seq = []
                starts()
                todo = {}
            for ti, tk in enumerate(seq):
                if ti == dpos:
                    starts()
                fns[tk[0]](tk[1], tk[2])
            for lst in todo.values():
                for job in lst:
                    job()
            if mode == "l" and mode not in only:
                rs = pl.ds(row0, M)
                pltpu.make_async_copy(obuf.at[rs, :], o_hbm.at[rs, :], osem.at[0]).start()

        zv[...] = jnp.zeros((8, 128), u32)

        def loop(lo, hi, fn):
            def w(i, c):
                fn(i)
                return c
            lax.fori_loop(lo, hi, w, 0)

        loop(0, nbg, lambda sl: wq_start(0, sl, 0))
        x_start(0)
        x_start(1)
        wait_buf(wqraw, wsem.at[0, 0])

        def pro(sl):
            for a in w_pieces:
                wq_piece(0, sl, *a)
        loop(0, nbg, pro)
        for k in range(2):
            wq_start(1, k, k)
            wo_start(0, k, k)
        wait_buf(xraw.at[0], xsem.at[0])
        for a in x_pieces:
            x_piece(0, *a)
        def steps(mode, lo, hi, slot0):
            def w(t, slot):
                body(mode, t, slot)
                return jnp.where(slot == 2, 0, slot + 1)
            return lax.fori_loop(lo, hi, w, slot0)

        kv_piece(0)
        steps("q", 0, nbg, jnp.int32(0))
        kv_start(1, 0, 1)
        slot = steps("m", nbg, T, jnp.int32(0))
        steps("l", T, T + nbg, slot)
        pltpu.make_async_copy(obuf, o_hbm, osem.at[0]).wait()

    def fn(A_x, A_k, A_v, A_wq, A_wo, B_x, B_k, B_v, B_wq, B_wo):
        def kv(k):
            return jnp.swapaxes(k, 2, 3).reshape(B, H * DH, SK)

        def wo4(w):
            return w.reshape(8, 6, 128, D)
        anyspec = pl.BlockSpec(memory_space=pl.ANY)
        out = pl.pallas_call(
            kernel,
            in_specs=[anyspec] * 10,
            out_specs=anyspec,
            out_shape=jax.ShapeDtypeStruct((B * SQ, 2 * D), bf16),
            scratch_shapes=[pltpu.VMEM((B * SQ, 2 * D), f32),
                            pltpu.VMEM((B * SQ, 2 * D), bf16),
                            pltpu.VMEM((2, 2, nb, SQ, D), bf16),
                            pltpu.VMEM((2, B, 22, HF // 2, 128), u32),
                            pltpu.VMEM((nbg, U, 6, HF, 128), u32),
                            pltpu.VMEM((3, 4, nb, GW, SK), bf16),
                            pltpu.VMEM((nbg, 2, 5, SL, GW), bf16),
                            pltpu.VMEM((nbg, 2, 6, SL, D), bf16),
                            pltpu.VMEM((2, 2, 51, 64, 128), u32),
                            pltpu.VMEM((2, 2, 51, 64, 128), u32),
                            pltpu.VMEM((8, 128), u32),
                            pltpu.SemaphoreType.DMA((3,)),
                            pltpu.SemaphoreType.DMA((2, 2)),
                            pltpu.SemaphoreType.DMA((2,)),
                            pltpu.SemaphoreType.DMA((1,)),
                            ],
            compiler_params=pltpu.CompilerParams(
                vmem_limit_bytes=vmem * 1024 * 1024,
                disable_bounds_checks=True),
        )(A_x, kv(A_k), kv(A_v), A_wq, wo4(A_wo), B_x, kv(B_k), kv(B_v), B_wq, wo4(B_wo))
        return out.reshape(B, SQ, 2 * D)
    return fn


SPACE = dict(
    odd=["Q0,Q1,Q2,Q3,Q4,K0,K1,P0,P1", "K0,K1,Q0,Q1,Q2,Q3,Q4,P0,P1", "Q0,Q1,K0,K1,Q2,Q3,Q4,P0,P1", "K0,K1,P0,P1,Q0,Q1,Q2,Q3,Q4",
         "Q0,K0,Q1,K1,P0,Q2,Q3,P1,Q4", "K0,Q0,K1,Q1,P0,Q2,Q3,Q4,P1", "Q0,Q1,K0,P0,Q2,Q3,Q4,K1,P1", "Q2,Q3,Q4,Q0,Q1,K0,K1,P0,P1",
         "K0,K1,P0,Q0,Q1,P1,Q2,Q3,Q4", "Q2,Q3,Q4,K0,K1,P0,Q0,P1,Q1"],
    even=["K0,K1,P0,P1,O0,O1,O2", "K0,K1,O0,P0,P1,O1,O2", "K0,K1,P0,O0,P1,O1,O2", "K0,K1,P0,O1,O2,P1,O0", "K0,K1,O1,O2,P0,P1,O0",
          "K0,P0,K1,O0,P1,O1,O2", "K0,K1,P0,P1,O1,O2,O0", "K0,K1,O0,O1,O2,P0,P1"],
    tail=[0, 1, 2, 3], sch=[2, 3, 4, 5, 6], mq=[48, 80], mo=[48, 80], mk=[80, 160], nk=[256, 512, 128],
    wq_every=[3, 4, 7, 11, 20], wo_every=[2, 3, 5, 7], dpos=[1, 2, 3], horder=[0, 1, 2, 3], osplit=[5, 7, 10], pord=[0, 1, 2])


@jax.jit
def pallas_concat_heads__gqa_block_cached__mha_block_cached__near_ridge_kernel(A_x, A_k_cache, A_v_cache, A_wq, A_wo, B_x, B_k_cache, B_v_cache, B_wq, B_wo):
    return _build()(A_x, A_k_cache, A_v_cache, A_wq, A_wo, B_x, B_k_cache, B_v_cache, B_wq, B_wo)
```

```python
import functools
import jax, jax.numpy as jnp
from jax import lax
from jax.experimental import pallas as pl
from jax.experimental.pallas import tpu as pltpu

B, SQ, D, H, SK, DH = 16, 160, 640, 32, 512, 192
PW = 2 * DH
GW = 2 * PW
LOG2E = 1.4426950408889634
QSCALE = (DH ** -0.5) * LOG2E
NT = (((1,), (1,)), ((), ()))
f32, bf16, u32 = jnp.float32, jnp.bfloat16, jnp.uint32
TT = 128
R = SQ - TT
HF = SQ // 2


def chunks(m, tot=SQ):
    return [(r, min(r + m, tot)) for r in range(0, tot, m)]


def dot(a, b):
    return jnp.dot(a, b, preferred_element_type=f32)


def dotnt(a, b):
    return lax.dot_general(a, b, NT, preferred_element_type=f32)


def unpk(v):
    return pltpu.bitcast(v, bf16)


Q_FORMS = [((0, 0, 1), (1, 0, -1)), ((1, 0, 1),), ((0, 1, 1),), ((0, 1, 1), (1, 1, -1)), ((0, 3, 1),), ((0, 3, 1), (1, 3, -1)), ((0, 1, 1), (1, 0, -1)), ((1, 0, 1), (1, 1, -1)), ((0, 0, 1), (0, 1, -1)), ((1, 3, 1),), ((0, 4, 1),), ((0, 4, 1), (1, 4, -1)), ((0, 1, 1), (1, 3, -1)), ((0, 1, 1), (0, 3, -1)), ((1, 1, 1), (1, 3, -1)), ((0, 0, 1),), ((1, 1, 1),), ((0, 0, 1), (1, 3, -1)), ((0, 0, 1), (0, 3, -1)), ((1, 0, 1), (1, 3, -1)), ((0, 2, 1),), ((1, 2, 1),), ((1, 4, 1),), ((0, 0, 1), (1, 4, -1)), ((0, 0, 1), (0, 4, -1)), ((1, 0, 1), (1, 4, -1)), ((0, 1, 1), (1, 4, -1)), ((0, 1, 1), (0, 4, -1)), ((1, 1, 1), (1, 4, -1)), ((0, 2, 1), (1, 2, -1)), ((0, 1, 1), (1, 2, -1)), ((0, 1, 1), (0, 2, -1)), ((1, 1, 1), (1, 2, -1)), ((0, 0, 1), (1, 2, -1)), ((0, 0, 1), (0, 2, -1)), ((1, 0, 1), (1, 2, -1)), ((0, 4, 1), (1, 2, -1)), ((1, 2, 1), (1, 4, -1)), ((0, 2, 1), (0, 4, -1)), ((0, 3, 1), (1, 2, -1)), ((1, 2, 1), (1, 3, -1)), ((0, 2, 1), (0, 3, -1)), ((0, 3, 1), (1, 4, -1)), ((0, 3, 1), (0, 4, -1)), ((1, 3, 1), (1, 4, -1))]
Q_PRODS = [(0, ((0, 1, 1), (0, 2, -1)), ((0, 1, 1),)), (1, ((0, 1, 1), (1, 1, 1)), ((0, 1, 1), (1, 1, 1))), (2, ((0, 2, 1), (1, 2, 1), (2, 2, 1), (3, 2, 1), (4, 2, 1)), ((0, 2, 1), (1, 2, 1))), (3, ((1, 1, 1), (1, 3, 1), (1, 4, 1), (1, 5, 1), (1, 2, -1)), ((1, 2, 1),)), (4, ((2, 1, 1), (3, 1, 1), (4, 1, 1)), ((0, 1, 1), (1, 1, 1))), (5, ((3, 4, 1), (3, 5, 1), (3, 1, -1)), ((1, 1, 1),)), (6, ((0, 2, 1), (1, 1, 1)), ((0, 1, 1), (1, 2, -1))), (7, ((1, 1, 1),), ((1, 1, -1), (1, 2, -1))), (8, ((0, 2, 1),), ((0, 1, 1), (0, 2, 1))), (5, ((3, 0, 1), (3, 2, 1), (3, 3, -1)), ((0, 3, -1),)), (9, ((0, 3, 1), (1, 3, 1), (3, 3, 1)), ((0, 3, 1), (1, 3, 1))), (10, ((2, 3, 1), (4, 3, 1)), ((0, 3, 1), (1, 3, 1))), (11, ((4, 3, 1), (4, 5, -1)), ((1, 3, -1),)), (12, ((1, 3, 1), (3, 2, 1)), ((0, 3, 1), (1, 2, -1))), (13, ((3, 2, 1),), ((0, 2, -1), (0, 3, -1))), (14, ((1, 3, 1),), ((1, 2, 1), (1, 3, 1))), (15, ((0, 0, 1), (2, 0, 1), (3, 0, 1), (4, 0, 1)), ((0, 0, 1), (1, 0, 1))), (0, ((0, 3, 1), (0, 4, 1), (0, 5, 1), (0, 0, -1)), ((1, 0, 1),)), (2, ((1, 0, 1),), ((0, 0, 1),)), (16, ((1, 0, 1),), ((1, 0, 1),)), (17, ((0, 3, 1), (3, 0, 1)), ((0, 3, 1), (1, 0, -1))), (18, ((3, 0, 1),), ((0, 0, -1), (0, 3, -1))), (19, ((0, 3, 1),), ((1, 0, 1), (1, 3, 1))), (20, ((2, 4, 1),), ((0, 4, 1),)), (21, ((2, 4, 1),), ((1, 4, 1),)), (11, ((4, 0, 1), (4, 1, 1), (4, 2, 1), (4, 4, -1)), ((0, 4, -1),)), (22, ((0, 4, 1), (1, 4, 1), (3, 4, 1), (4, 4, 1)), ((0, 4, 1), (1, 4, 1))), (23, ((0, 4, 1), (4, 0, 1)), ((0, 4, 1), (1, 0, -1))), (24, ((4, 0, 1),), ((0, 0, -1), (0, 4, -1))), (25, ((0, 4, 1),), ((1, 0, 1), (1, 4, 1))), (26, ((1, 4, 1), (4, 2, 1)), ((0, 4, 1), (1, 2, -1))), (27, ((4, 2, 1),), ((0, 2, -1), (0, 4, -1))), (28, ((1, 4, 1),), ((1, 2, 1), (1, 4, 1))), (29, ((2, 0, 1), (2, 1, 1), (2, 2, 1), (2, 3, 1), (2, 5, -1)), ((0, 5, -1),)), (21, ((0, 5, 1), (1, 5, 1), (2, 5, 1), (3, 5, 1), (4, 5, 1)), ((0, 5, 1), (1, 5, 1))), (30, ((1, 5, 1), (2, 2, 1)), ((0, 5, 1), (1, 2, -1))), (31, ((2, 2, 1),), ((0, 2, -1), (0, 5, -1))), (32, ((1, 5, 1),), ((1, 2, 1), (1, 5, 1))), (33, ((0, 5, 1), (2, 0, 1)), ((0, 5, 1), (1, 0, -1))), (34, ((2, 0, 1),), ((0, 0, -1), (0, 5, -1))), (35, ((0, 5, 1),), ((1, 0, 1), (1, 5, 1))), (36, ((2, 3, 1), (4, 5, 1)), ((0, 5, 1), (1, 3, -1))), (37, ((4, 5, 1),), ((1, 3, -1), (1, 5, -1))), (38, ((2, 3, 1),), ((0, 3, 1), (0, 5, 1))), (39, ((2, 1, 1), (3, 5, 1)), ((0, 5, 1), (1, 1, -1))), (40, ((3, 5, 1),), ((1, 1, -1), (1, 5, -1))), (41, ((2, 1, 1),), ((0, 1, 1), (0, 5, 1))), (42, ((3, 4, 1), (4, 1, 1)), ((0, 4, 1), (1, 1, -1))), (43, ((4, 1, 1),), ((0, 1, -1), (0, 4, -1))), (44, ((3, 4, 1),), ((1, 1, 1), (1, 4, 1)))]
O_FORMS = [((0, 0, 1),), ((0, 0, 1), (1, 0, -1)), ((0, 1, 1), (1, 1, -1)), ((1, 1, 1),), ((1, 0, 1),), ((0, 2, 1),), ((0, 2, 1), (1, 2, -1)), ((0, 2, 1), (1, 1, -1)), ((1, 1, 1), (1, 2, -1)), ((0, 1, 1), (0, 2, -1)), ((0, 1, 1),), ((0, 3, 1), (1, 3, -1)), ((1, 3, 1),), ((0, 2, 1), (1, 3, -1)), ((0, 2, 1), (0, 3, -1)), ((1, 2, 1), (1, 3, -1)), ((0, 0, 1), (1, 3, -1)), ((0, 0, 1), (0, 3, -1)), ((1, 0, 1), (1, 3, -1)), ((0, 3, 1),), ((0, 4, 1), (1, 4, -1)), ((1, 4, 1),), ((0, 0, 1), (1, 4, -1)), ((0, 0, 1), (0, 4, -1)), ((1, 0, 1), (1, 4, -1)), ((0, 2, 1), (1, 4, -1)), ((0, 2, 1), (0, 4, -1)), ((1, 2, 1), (1, 4, -1)), ((0, 4, 1),), ((0, 5, 1), (1, 5, -1)), ((1, 5, 1),), ((0, 2, 1), (1, 5, -1)), ((0, 2, 1), (0, 5, -1)), ((1, 2, 1), (1, 5, -1)), ((0, 0, 1), (1, 5, -1)), ((0, 0, 1), (0, 5, -1)), ((1, 0, 1), (1, 5, -1)), ((0, 1, 1), (1, 5, -1)), ((1, 1, 1), (1, 5, -1)), ((0, 1, 1), (0, 5, -1)), ((0, 1, 1), (1, 4, -1)), ((0, 1, 1), (0, 4, -1)), ((1, 1, 1), (1, 4, -1)), ((0, 3, 1), (1, 5, -1)), ((1, 3, 1), (1, 5, -1)), ((0, 3, 1), (0, 5, -1))]
O_PRODS = [(0, ((0, 0, 1), (3, 0, 1), (4, 0, 1), (5, 0, 1)), ((0, 0, 1), (1, 0, 1))), (1, ((0, 2, 1), (0, 3, 1), (0, 4, 1), (0, 0, -1)), ((1, 0, 1),)), (2, ((1, 0, 1), (1, 1, -1)), ((0, 0, 1),)), (3, ((1, 0, 1), (2, 0, 1)), ((0, 0, 1), (1, 0, 1))), (0, ((0, 1, 1),), ((0, 1, 1),)), (4, ((0, 1, 1),), ((1, 1, 1),)), (5, ((1, 1, 1), (2, 1, 1), (3, 1, 1), (4, 1, 1), (5, 1, 1)), ((0, 1, 1), (1, 1, 1))), (6, ((2, 0, 1), (2, 2, 1), (2, 3, 1), (2, 4, 1), (2, 1, -1)), ((1, 1, 1),)), (7, ((1, 1, 1), (2, 0, 1)), ((0, 0, 1), (1, 1, -1))), (8, ((2, 0, 1),), ((1, 0, -1), (1, 1, -1))), (9, ((1, 1, 1),), ((0, 0, 1), (0, 1, 1))), (10, ((1, 3, 1), (4, 3, 1), (5, 3, 1)), ((0, 3, 1), (1, 3, 1))), (2, ((1, 2, 1), (1, 4, 1), (1, 3, -1)), ((1, 3, 1),)), (11, ((3, 0, 1), (3, 1, 1), (3, 3, -1)), ((0, 3, -1),)), (12, ((0, 3, 1), (2, 3, 1), (3, 3, 1)), ((0, 3, 1), (1, 3, 1))), (13, ((2, 3, 1), (3, 1, 1)), ((0, 3, 1), (1, 1, -1))), (14, ((3, 1, 1),), ((0, 1, -1), (0, 3, -1))), (15, ((2, 3, 1),), ((1, 1, 1), (1, 3, 1))), (16, ((0, 3, 1), (3, 0, 1)), ((0, 3, 1), (1, 0, -1))), (17, ((3, 0, 1),), ((0, 0, -1), (0, 3, -1))), (18, ((0, 3, 1),), ((1, 0, 1), (1, 3, 1))), (19, ((3, 4, 1), (5, 4, 1)), ((0, 4, 1), (1, 4, 1))), (11, ((3, 4, 1), (3, 2, -1)), ((1, 4, -1),)), (20, ((4, 0, 1), (4, 1, 1), (4, 3, 1), (4, 4, -1)), ((0, 4, -1),)), (21, ((0, 4, 1), (1, 4, 1), (2, 4, 1), (4, 4, 1)), ((0, 4, 1), (1, 4, 1))), (22, ((0, 4, 1), (4, 0, 1)), ((0, 4, 1), (1, 0, -1))), (23, ((4, 0, 1),), ((0, 0, -1), (0, 4, -1))), (24, ((0, 4, 1),), ((1, 0, 1), (1, 4, 1))), (25, ((2, 4, 1), (4, 1, 1)), ((0, 4, 1), (1, 1, -1))), (26, ((4, 1, 1),), ((0, 1, -1), (0, 4, -1))), (27, ((2, 4, 1),), ((1, 1, 1), (1, 4, 1))), (28, ((4, 2, 1),), ((0, 2, 1),)), (21, ((4, 2, 1),), ((1, 2, 1),)), (29, ((5, 0, 1), (5, 1, 1), (5, 3, 1), (5, 4, 1), (5, 2, -1)), ((0, 2, -1),)), (30, ((0, 2, 1), (1, 2, 1), (2, 2, 1), (3, 2, 1), (5, 2, 1)), ((0, 2, 1), (1, 2, 1))), (31, ((2, 2, 1), (5, 1, 1)), ((0, 2, 1), (1, 1, -1))), (32, ((5, 1, 1),), ((0, 1, -1), (0, 2, -1))), (33, ((2, 2, 1),), ((1, 1, 1), (1, 2, 1))), (34, ((0, 2, 1), (5, 0, 1)), ((0, 2, 1), (1, 0, -1))), (35, ((5, 0, 1),), ((0, 0, -1), (0, 2, -1))), (36, ((0, 2, 1),), ((1, 0, 1), (1, 2, 1))), (37, ((1, 2, 1), (5, 3, 1)), ((0, 2, 1), (1, 3, -1))), (38, ((1, 2, 1),), ((1, 2, 1), (1, 3, 1))), (39, ((5, 3, 1),), ((0, 2, -1), (0, 3, -1))), (40, ((1, 4, 1), (4, 3, 1)), ((0, 4, 1), (1, 3, -1))), (41, ((4, 3, 1),), ((0, 3, -1), (0, 4, -1))), (42, ((1, 4, 1),), ((1, 3, 1), (1, 4, 1))), (43, ((3, 2, 1), (5, 4, 1)), ((0, 2, 1), (1, 4, -1))), (44, ((3, 2, 1),), ((1, 2, 1), (1, 4, 1))), (45, ((5, 4, 1),), ((0, 2, -1), (0, 4, -1)))]
NPR = 50


def lincomb(terms, get):
    v = get(terms[0][:-1])
    for t in terms[1:]:
        v = v + get(t[:-1]) if t[-1] > 0 else v - get(t[:-1])
    return v


def pcombos(term_lists, load):
    us, lo, hi = {}, {}, {}

    def packed(k):
        if k not in us:
            us[k] = pltpu.bitcast(load(*k), u32)
        return us[k]

    def half(cache, idx):
        def get(k):
            if k not in cache:
                cache[k] = pltpu.unpack_elementwise(packed(k), index=idx, packed_dtype=bf16, unpacked_dtype=f32)
            return cache[k]
        return get
    return [packed(t[0][:-1]) if len(t) == 1 else
            pltpu.pack_elementwise([lincomb(t, half(lo, 0)), lincomb(t, half(hi, 1))], packed_dtype=bf16).astype(u32)
            for t in term_lists]


def last_use(prods):
    last = {}
    for r, (_, _, beta) in enumerate(prods):
        for (s, j, _) in beta:
            last[(s, j)] = r
    return last


def bilinear(prods, rs, prod, c, init, done):
    last = last_use(prods)
    for r in rs:
        m = prod(r)
        for (s, j, sg) in prods[r][2]:
            if (s, j) not in c and init is not None:
                c[(s, j)] = init(s, j)
            if (s, j) in c:
                c[(s, j)] = c[(s, j)] + m if sg > 0 else c[(s, j)] - m
            else:
                c[(s, j)] = m if sg > 0 else -m
            if last[(s, j)] == r:
                done(s, j, c[(s, j)])


def split(nparts, total=NPR):
    return [list(range(k * total // nparts, (k + 1) * total // nparts)) for k in range(nparts)]


def _build(NG=8, nb=2, vmem=110, mk=160, nk=256, mq=48, mo=80,
          odd="Q0,Q1,Q2,Q3,Q4,K0,K1,P0,P1", even="K0,K1,P0,P1,O0,O1,O2",
          tail=1, qlag=2, mqq=80, dpos=1, sch=4, wq_every=4, wo_every=5, xq_every=3, head="", ltail=1, only="qml", wparts=5, xparts=3, pord=0, lodd="K0,K1,P0,P1", leven="K0,K1,P0,P1,O0,O1,O2", lsch=4, lmo=80, lmk=160, qord="01234", wqq_every=4, tl=0, ltl=0, oanch=0, nocse=0):
    nbg = B // nb
    M = nb * SQ
    T = NG * nbg
    assert nbg == 8
    SL = 128 // nbg
    LG = nbg.bit_length() - 1

    def recip(l):
        r = pl.reciprocal(l, approx=True)
        return r * (2.0 - l * r)

    def soft(s, zvec, sch, tl, prev):
        ps, ts, ls = [], [], []
        for r in range(SQ // 8):
            sb = s[r * 8:(r + 1) * 8]
            m = jnp.broadcast_to(jnp.max(sb, axis=-1, keepdims=True), (8, 128))
            src = None
            if tl >= 3:
                if r // 2 >= sch and (r % 2 == 0 or tl == 4):
                    src = ls[r // 2 - sch]
            elif sch and r >= sch:
                src = ts[r - sch] if tl else ps[r - sch][:, 384:512]
            elif tl == 2 and prev:
                src = prev[r - sch]
            if src is not None:
                m = pltpu.bitcast(pltpu.bitcast(m, u32) | (pltpu.bitcast(src, u32) & zvec), f32)
            pb = jnp.exp2(sb - jnp.concatenate([m] * 4, axis=1))
            ps.append(pb)
            ts.append((pb[:, 0:128] + pb[:, 128:256]) + (pb[:, 256:384] + pb[:, 384:512]))
            if tl >= 3 and r % 2 == 1:
                pk = pltpu.bitcast(jnp.concatenate(ps[-2:], axis=0).astype(bf16), u32)
                ps[-2:] = [pk[:4], pk[4:]] if False else [pk, None]
                lk = (pk[:, 0:128] | pk[:, 128:256]) | (pk[:, 256:384] | pk[:, 384:512])
                ls.append(lk | pltpu.bitcast(ts[-1], u32) | pltpu.bitcast(ts[-2], u32))
        p = jnp.concatenate([x for x in ps if x is not None], axis=0)
        prev[:] = ts
        t = jnp.concatenate(ts[:TT // 8], axis=0)
        trem = jnp.concatenate(ts[TT // 8:], axis=0)
        rrow = recip(jnp.sum(t.T, axis=0, keepdims=True))
        rrem = jnp.broadcast_to(recip(jnp.sum(trem, axis=-1, keepdims=True)), (R, 128))
        return p, (rrow, rrem)

    units = [(p, b) for p in range(2) for b in range(nb)]
    U = len(units)
    n = 2 * U

    def kernel(xa, kta, vta, wqa, woa, xb, ktb, vtb, wqb, wob, o_hbm,
               acc, obuf, xraw, xsb, qbuf, kvbuf, wqraw, woraw, wqc, woc, zv,
               kvsem, wsem, xsem, osem):
        xs, kvs, wqs, wos = (xa, xb), (kta, vta, ktb, vtb), (wqa, wqb), (woa, wob)

        def kv_start(sl, hg_, g_):
            for a in range(4):
                pltpu.make_async_copy(
                    kvs[a].at[pl.ds(g_ * nb, nb), pl.ds(pl.multiple_of(hg_ * GW, GW), GW), :],
                    kvbuf.at[sl, a], kvsem.at[sl]).start()

        def kv_piece(k):
            a, b = k // nb, k % nb
            pltpu.make_async_copy(kvs[a].at[b, pl.ds(0, GW), :], kvbuf.at[0, a, b], kvsem.at[0]).start()

        def wq_start(hg_, sl, par):
            cq = pl.ds(pl.multiple_of(hg_ * GW, GW), GW)
            for p in range(2):
                for kt in range(5):
                    pltpu.make_async_copy(wqs[p].at[pl.ds(pl.multiple_of(kt * 128 + sl * SL, SL), SL), cq],
                                          wqraw.at[sl, p, kt], wsem.at[par, 0]).start()

        def wo_start(hg_, sl, par):
            for p in range(2):
                pltpu.make_async_copy(wos[p].at[hg_, :, pl.ds(pl.multiple_of(sl * SL, SL), SL), :],
                                      woraw.at[sl, p], wsem.at[par, 1]).start()

        def wait_buf(v, sem):
            pltpu.make_async_copy(v, v, sem).wait()

        def x_start(g_):
            for p in range(2):
                pltpu.make_async_copy(xs[p].at[pl.ds(g_ * nb, nb)], xraw.at[g_ & 1, p], xsem.at[g_ & 1]).start()

        def ct(c):
            return slice(c * 128, (c + 1) * 128)

        def w_piece(raw, dst, prods, ws, sl, p, rs):
            rows = pl.ds(pl.multiple_of(sl * (SL // 2), 8), SL // 2)
            vs = pcombos([prods[r][1] for r in rs], lambda i, j: raw[sl, p, i, :, ct(j)])
            for r, v in zip(rs, vs):
                dst[ws, p, r, rows, :] = v

        wq_piece = functools.partial(w_piece, wqraw, wqc, Q_PRODS)
        wo_piece = functools.partial(w_piece, woraw, woc, O_PRODS)
        w_pieces = [(p, rs) for p in range(2) for rs in split(wparts)]

        def x_piece(g_, p, b, ks, r0):
            vs = pcombos([Q_FORMS[k] for k in ks],
                         lambda s, i: xraw[g_ & 1, p, b, s * HF + r0:s * HF + r0 + 16, ct(i)])
            for k, v in zip(ks, vs):
                xsb[p, g_ * nb + b, k, r0 // 2:r0 // 2 + 8, :] = v

        x_pieces = [(p, b, ks, r0) for p in range(2) for b in range(nb) for r0 in range(0, HF, 16)
                    for ks in split(xparts, len(Q_FORMS))]

        def body(mode, t, slot):
            g = t & (nbg - 1)
            hg1 = lax.shift_right_logical(t, LG)
            hg = hg1 - 1
            par = t & 1
            slot2 = jnp.where(slot == 0, 2, slot - 1)
            qslot = hg1 & 1
            wslot = 1 - qslot
            row0 = pl.multiple_of(g * M, M)

            def starts():
                t1, t2 = t + 1, t + 2
                if mode != "q":
                    @pl.when(t2 < T + nbg)
                    def _():
                        kv_start(slot2, lax.shift_right_logical(t2, LG) - 1, t2 & (nbg - 1))
                if mode == "q":
                    for k in range(1, nbg):
                        pl.when(g + 1 == k)(functools.partial(kv_piece, k))
                if mode != "l":
                    hg2 = lax.shift_right_logical(t2, LG)

                    @pl.when(hg2 + 1 < NG)
                    def _():
                        wq_start(hg2 + 1, t2 & (nbg - 1), par)

                    @pl.when(hg2 < NG)
                    def _():
                        wo_start(hg2, t2 & (nbg - 1), par)

            if mode == "q":
                @pl.when(g + 2 < nbg)
                def _():
                    x_start(g + 2)

            if mode == "q":
                @pl.when(g + 1 < nbg)
                def _():
                    wait_buf(xraw.at[(g + 1) & 1], xsem.at[(g + 1) & 1])
            if mode != "l":
                @pl.when(hg1 + 1 < NG)
                def _():
                    wait_buf(wqraw.at[g], wsem.at[par, 0])
                wait_buf(woraw.at[g], wsem.at[par, 1])
            if mode != "q":
                wait_buf(kvbuf.at[slot], kvsem.at[slot])

            st = [dict() for _ in range(n)]
            mq_ = mqq if mode == "q" else mq
            mo_ = mo if mode == "m" else lmo
            mk_ = mk if mode == "m" else lmk
            zvec = zv[...]
            tprev = []
            jq = [functools.partial(wq_piece, 1 - qslot, g, *a) for a in w_pieces]
            jo = [functools.partial(wo_piece, 1 - wslot, g, *a) for a in w_pieces]
            gx = jnp.minimum(g + 1, nbg - 1)
            jx = [functools.partial(x_piece, gx, *a) for a in x_pieces]
            todo = {"q": {"q": jq + jo, "o": [], "x": jx}, "m": {"q": jq, "o": jo, "x": []},
                    "l": {"q": [], "o": [], "x": []}}[mode]
            cnt = {"q": 0, "o": 0, "x": 0}
            every = {"q": wq_every if mode == "m" else wqq_every, "o": wo_every, "x": xq_every}

            def host(kind):
                cnt[kind] += 1
                if every[kind] and cnt[kind] % every[kind] == 0 and todo[kind]:
                    todo[kind].pop(0)()

            def task_q(u, j):
                p, b = units[u]
                bb = g * nb + b
                d = st[2 * u].setdefault("qc", {})
                fin = st[2 * u].setdefault("qf", {})
                for (a, e) in chunks(mq_, HF):
                    def prod(r):
                        host("q")
                        host("x")
                        return dot(unpk(xsb[p, bb, Q_PRODS[r][0], a // 2:e // 2, :]), unpk(wqc[qslot, p, r]))

                    def done(s, col, v):
                        qbuf[g, u, col, (s * HF + a) // 2:(s * HF + e) // 2, :] = pltpu.bitcast((v * QSCALE).astype(bf16), u32)
                    bilinear(Q_PRODS, split(5)[j], prod, d.setdefault(a, {}), None, done)

            def task_k(i, h):
                p, b = units[i // 2]
                k0 = (i % 2) * PW
                kt = kvbuf.at[slot, 2 * p, b]
                d = st[i]
                lane = lax.broadcasted_iota(jnp.int32, (HF, 128), 1)
                qm = qbuf[g, i // 2, 3 * (i % 2) + 1]
                if h == 0:
                    l = [qbuf[g, i // 2, 3 * (i % 2)], jnp.where(lane < 64, qm, jnp.uint32(0))]
                else:
                    l = [jnp.where(lane >= 64, qm, jnp.uint32(0)), qbuf[g, i // 2, 3 * (i % 2) + 2]]
                l = jnp.concatenate(l, axis=1)
                rows = []
                for (a, e) in chunks(mk_):
                    lc = unpk(l[a // 2:e // 2])
                    cs = [dot(lc, kt[k0 + h * 128:k0 + h * 128 + 256, c:c + nk]) for c in range(0, SK, nk)]
                    rows.append(jnp.concatenate(cs, axis=1))
                pp, rr = soft(jnp.concatenate(rows, axis=0), zvec, sch if mode == "m" else lsch, tl if mode == "m" else ltl, tprev)
                if pp.dtype == u32:
                    d["pt%d" % h], d["pr%d" % h] = unpk(pp[:TT // 2]), unpk(pp[TT // 2:])
                    d["pf%d" % h] = pp[TT // 2:]
                    if h == 1:
                        d["pm"] = unpk(jnp.concatenate([d["pf0"], d["pf1"]], axis=0))
                else:
                    d["pt%d" % h], d["pr%d" % h] = pp[:TT].astype(bf16), pp[TT:].astype(bf16)
                    d["pf%d" % h] = pp[TT:]
                    if h == 1:
                        d["pm"] = jnp.concatenate([d["pf0"], d["pf1"]], axis=0).astype(bf16)
                d["r%d" % h] = rr

            def task_p(i, h):
                p, b = units[i // 2]
                k0 = (i % 2) * PW
                vt = kvbuf.at[slot, 2 * p + 1, b]
                d = st[i]
                if h == 0:
                    d["ot1"] = dotnt(vt[k0:k0 + 192, :], d["pt0"])
                    d["oa"] = dotnt(d["pr0"], vt[k0:k0 + 128, :])
                else:
                    r1, r2 = d["r0"], d["r1"]
                    fm = lambda: dotnt(d["pm"], vt[k0 + 128:k0 + 256, :])
                    f2 = lambda: dotnt(vt[k0 + 192:k0 + 384, :], d["pt1"])
                    fc = lambda: dotnt(d["pr1"], vt[k0 + 256:k0 + 384, :])
                    if pord == 0:
                        om = fm(); ot2 = f2(); oc = fc()
                    elif pord == 1:
                        ot2 = f2(); om = fm(); oc = fc()
                    else:
                        ot2 = f2(); oc = fc(); om = fm()
                    ot1 = d["ot1"] * r1[0]
                    ot2 = ot2 * r2[0]
                    lane = lax.broadcasted_iota(jnp.int32, (R, 128), 1)
                    omr = jnp.where(lane < 64, om[:R] * r1[1], om[R:] * r2[1])
                    ta = ot1[0:128].T
                    tm = jnp.concatenate([ot1[128:192], ot2[0:64]], axis=0).T
                    tc = ot2[64:192].T
                    d["o"] = [jnp.concatenate([ta, d["oa"] * r1[1]], axis=0),
                              jnp.concatenate([tm, omr], axis=0),
                              jnp.concatenate([tc, oc * r2[1]], axis=0)]

            def task_o(u, j):
                p, b = units[u]
                d = st[2 * u]
                o = st[2 * u]["o"] + st[2 * u + 1]["o"]
                for (a, e) in chunks(mo_, HF):
                    def idx(s, col):
                        c0 = p * D + col * 128
                        return pl.ds(pl.multiple_of(row0 + b * SQ + s * HF + a, 16), e - a), slice(c0, c0 + 128)

                    def accv(s, col):
                        return jnp.where(hg == 0, 0.0, acc[idx(s, col)]) if mode == "m" else acc[idx(s, col)]

                    def put(s, col, v):
                        if mode == "l":
                            obuf[idx(s, col)] = v.astype(bf16)
                        else:
                            acc[idx(s, col)] = v

                    def prod(r):
                        host("o")
                        key = ("of", O_PRODS[r][0], a)
                        if key not in d:
                            d[key] = lincomb(O_FORMS[O_PRODS[r][0]],
                                             lambda k: o[k[1]][k[0] * HF + a:k[0] * HF + e]).astype(bf16)
                        return dot(d[key], unpk(woc[wslot, p, r]))
                    bilinear(O_PRODS, split(3)[j], prod, d.setdefault(("oc", a), {}), accv, put)
                d["odone"] = d.get("odone", 0) + 1
                if mode == "l" and d["odone"] == 3:
                    rs = pl.ds(pl.multiple_of(row0 + b * SQ, 16), SQ)
                    pltpu.make_async_copy(obuf.at[rs, p * D:(p + 1) * D], o_hbm.at[rs, p * D:(p + 1) * D], osem.at[0]).start()

            seq = []
            if mode == "q":
                seq = [("Q", u, int(j)) for u in range(U) for j in str(qord).zfill(5)]
            else:
                pats = (even, odd) if mode == "m" else (leven, lodd)
                for s in range(-3, n + 2):
                    for tok in pats[s % 2].split(","):
                        k, j = tok[0], int(tok[1])
                        if k == "Q":
                            u = (s + 1) // 2 + 1 - qlag
                            if 0 <= u < U and mode == "m": seq.append(("Q", u, j))
                        elif k == "O":
                            u = s // 2 - 1
                            if 0 <= u < U: seq.append(("O", u, j))
                        elif k == "K":
                            if 0 <= s + 1 < n: seq.append(("K", s + 1, j))
                        else:
                            if 0 <= s < n: seq.append(("P", s, j))
                tl_ = tail if mode == "m" else ltail
                if tl_:
                    mv = [x for x in seq if x[0] == "O" and x[1] == U - 2][-tl_:]
                    seq = [x for x in seq if x not in mv]
                    pos = seq.index(("P", n - 1, 1)) + 1
                    seq = seq[:pos] + mv + seq[pos:]
            fns = {"Q": task_q, "K": task_k, "P": task_p, "O": task_o}
            if mode not in only:
                seq = []
                starts()
                todo = {}
            for ti, tk in enumerate(seq):
                if ti == dpos:
                    starts()
                fns[tk[0]](tk[1], tk[2])
            for lst in todo.values():
                for job in lst:
                    job()
            if mode == "l" and mode not in only:
                rs = pl.ds(row0, M)
                pltpu.make_async_copy(obuf.at[rs, :], o_hbm.at[rs, :], osem.at[0]).start()

        zv[...] = jnp.zeros((8, 128), u32)

        def loop(lo, hi, fn):
            def w(i, c):
                fn(i)
                return c
            lax.fori_loop(lo, hi, w, 0)

        loop(0, nbg, lambda sl: wq_start(0, sl, 0))
        x_start(0)
        x_start(1)
        wait_buf(wqraw, wsem.at[0, 0])

        def pro(sl):
            for a in w_pieces:
                wq_piece(0, sl, *a)
        loop(0, nbg, pro)
        for k in range(2):
            wq_start(1, k, k)
            wo_start(0, k, k)
        wait_buf(xraw.at[0], xsem.at[0])
        for a in x_pieces:
            x_piece(0, *a)
        def steps(mode, lo, hi, slot0):
            def w(t, slot):
                body(mode, t, slot)
                return jnp.where(slot == 2, 0, slot + 1)
            return lax.fori_loop(lo, hi, w, slot0)

        kv_piece(0)
        steps("q", 0, nbg, jnp.int32(0))
        kv_start(1, 0, 1)
        slot = steps("m", nbg, T, jnp.int32(0))
        steps("l", T, T + nbg, slot)
        pltpu.make_async_copy(obuf, o_hbm, osem.at[0]).wait()

    def fn(A_x, A_k, A_v, A_wq, A_wo, B_x, B_k, B_v, B_wq, B_wo):
        def kv(k):
            return jnp.swapaxes(k, 2, 3).reshape(B, H * DH, SK)

        def wo4(w):
            return w.reshape(8, 6, 128, D)
        anyspec = pl.BlockSpec(memory_space=pl.ANY)
        out = pl.pallas_call(
            kernel,
            in_specs=[anyspec] * 10,
            out_specs=anyspec,
            out_shape=jax.ShapeDtypeStruct((B * SQ, 2 * D), bf16),
            scratch_shapes=[pltpu.VMEM((B * SQ, 2 * D), f32),
                            pltpu.VMEM((B * SQ, 2 * D), bf16),
                            pltpu.VMEM((2, 2, nb, SQ, D), bf16),
                            pltpu.VMEM((2, B, len(Q_FORMS), HF // 2, 128), u32),
                            pltpu.VMEM((nbg, U, 6, HF, 128), u32),
                            pltpu.VMEM((3, 4, nb, GW, SK), bf16),
                            pltpu.VMEM((nbg, 2, 5, SL, GW), bf16),
                            pltpu.VMEM((nbg, 2, 6, SL, D), bf16),
                            pltpu.VMEM((2, 2, NPR, 64, 128), u32),
                            pltpu.VMEM((2, 2, NPR, 64, 128), u32),
                            pltpu.VMEM((8, 128), u32),
                            pltpu.SemaphoreType.DMA((3,)),
                            pltpu.SemaphoreType.DMA((2, 2)),
                            pltpu.SemaphoreType.DMA((2,)),
                            pltpu.SemaphoreType.DMA((1,)),
                            ],
            compiler_params=pltpu.CompilerParams(
                vmem_limit_bytes=vmem * 1024 * 1024,
                disable_bounds_checks=True),
        )(A_x, kv(A_k), kv(A_v), A_wq, wo4(A_wo), B_x, kv(B_k), kv(B_v), B_wq, wo4(B_wo))
        return out.reshape(B, SQ, 2 * D)
    return fn


SPACE = dict(
    odd=["Q0,Q1,Q2,Q3,Q4,K0,K1,P0,P1", "K0,K1,Q0,Q1,Q2,Q3,Q4,P0,P1", "Q0,Q1,K0,K1,Q2,Q3,Q4,P0,P1", "K0,K1,P0,P1,Q0,Q1,Q2,Q3,Q4",
         "Q0,K0,K1,Q1,Q2,Q3,Q4,P0,P1", "Q0,Q1,Q2,Q3,K0,K1,P0,P1,Q4", "Q0,Q1,Q2,K0,K1,P0,P1,Q3,Q4", "Q0,Q1,Q2,Q3,Q4,K0,P0,K1,P1"],
    even=["K0,K1,P0,P1,O0,O1,O2", "K0,P0,K1,O0,P1,O1,O2", "K0,K1,P0,O0,P1,O1,O2", "K0,P0,K1,P1,O0,O1,O2", "K0,K1,O0,P0,P1,O1,O2",
          "K0,K1,P0,O0,O1,P1,O2"],
    tail=[1, 2, 3], sch=[3, 4, 5, 6], tl=[0, 1, 2], mq=[48, 80], mo=[48, 80], mk=[80, 160],
    wq_every=[3, 4, 5, 7, 11, 19], wo_every=[2, 3, 4, 5, 7, 9], dpos=[1, 2, 3], pord=[0, 1, 2], wparts=[3, 5, 10])


@jax.jit
def pallas_concat_heads__gqa_block_cached__mha_block_cached__near_ridge_kernel(A_x, A_k_cache, A_v_cache, A_wq, A_wo, B_x, B_k_cache, B_v_cache, B_wq, B_wo):
    return _build(xq_every=2, mq=80, tail=2, odd='K0,K1,P0,P1,Q0,Q1,Q2,Q3,Q4')(A_x, A_k_cache, A_v_cache, A_wq, A_wo, B_x, B_k_cache, B_v_cache, B_wq, B_wo)
```

```python
import functools

import jax
import jax.numpy as jnp
from jax import lax
from jax.experimental import pallas as pl
from jax.experimental.pallas import tpu as pltpu

B, SQ, D, H, SK, DH = 16, 160, 640, 32, 512, 192
PW = 2 * DH
GW = 2 * PW
NG = H * DH // GW
NB = 2
NBG = B // NB
LG = NBG.bit_length() - 1
T = NG * NBG
SL = 128 // NBG
NS = 3
HF = SQ // 2
TT = 128
R = SQ - TT
QSCALE = (DH ** -0.5) * 1.4426950408889634
NT = (((1,), (1,)), ((), ()))
f32, bf16, u32 = jnp.float32, jnp.bfloat16, jnp.uint32

Q_FORMS = (
    ((0,0,1),(1,0,-1)), ((1,0,1),), ((0,1,1),), ((0,1,1),(1,1,-1)), ((0,3,1),), ((0,3,1),(1,3,-1)),
    ((0,1,1),(1,0,-1)), ((1,0,1),(1,1,-1)), ((0,0,1),(0,1,-1)), ((1,3,1),), ((0,4,1),), ((0,4,1),(1,4,-1)),
    ((0,1,1),(1,3,-1)), ((0,1,1),(0,3,-1)), ((1,1,1),(1,3,-1)), ((0,0,1),), ((1,1,1),), ((0,0,1),(1,3,-1)),
    ((0,0,1),(0,3,-1)), ((1,0,1),(1,3,-1)), ((0,2,1),), ((1,2,1),), ((1,4,1),), ((0,0,1),(1,4,-1)),
    ((0,0,1),(0,4,-1)), ((1,0,1),(1,4,-1)), ((0,1,1),(1,4,-1)), ((0,1,1),(0,4,-1)), ((1,1,1),(1,4,-1)),
    ((0,2,1),(1,2,-1)), ((0,1,1),(1,2,-1)), ((0,1,1),(0,2,-1)), ((1,1,1),(1,2,-1)), ((0,0,1),(1,2,-1)),
    ((0,0,1),(0,2,-1)), ((1,0,1),(1,2,-1)), ((0,4,1),(1,2,-1)), ((1,2,1),(1,4,-1)), ((0,2,1),(0,4,-1)),
    ((0,3,1),(1,2,-1)), ((1,2,1),(1,3,-1)), ((0,2,1),(0,3,-1)), ((0,3,1),(1,4,-1)), ((0,3,1),(0,4,-1)),
    ((1,3,1),(1,4,-1)),
)
Q_PRODS = (
    (0,((0,1,1),(0,2,-1)),((0,1,1),)), (1,((0,1,1),(1,1,1)),((0,1,1),(1,1,1))),
    (2,((0,2,1),(1,2,1),(2,2,1),(3,2,1),(4,2,1)),((0,2,1),(1,2,1))),
    (3,((1,1,1),(1,3,1),(1,4,1),(1,5,1),(1,2,-1)),((1,2,1),)), (4,((2,1,1),(3,1,1),(4,1,1)),((0,1,1),(1,1,1))),
    (5,((3,4,1),(3,5,1),(3,1,-1)),((1,1,1),)), (6,((0,2,1),(1,1,1)),((0,1,1),(1,2,-1))),
    (7,((1,1,1),),((1,1,-1),(1,2,-1))), (8,((0,2,1),),((0,1,1),(0,2,1))),
    (5,((3,0,1),(3,2,1),(3,3,-1)),((0,3,-1),)), (9,((0,3,1),(1,3,1),(3,3,1)),((0,3,1),(1,3,1))),
    (10,((2,3,1),(4,3,1)),((0,3,1),(1,3,1))), (11,((4,3,1),(4,5,-1)),((1,3,-1),)),
    (12,((1,3,1),(3,2,1)),((0,3,1),(1,2,-1))), (13,((3,2,1),),((0,2,-1),(0,3,-1))),
    (14,((1,3,1),),((1,2,1),(1,3,1))), (15,((0,0,1),(2,0,1),(3,0,1),(4,0,1)),((0,0,1),(1,0,1))),
    (0,((0,3,1),(0,4,1),(0,5,1),(0,0,-1)),((1,0,1),)), (2,((1,0,1),),((0,0,1),)), (16,((1,0,1),),((1,0,1),)),
    (17,((0,3,1),(3,0,1)),((0,3,1),(1,0,-1))), (18,((3,0,1),),((0,0,-1),(0,3,-1))),
    (19,((0,3,1),),((1,0,1),(1,3,1))), (20,((2,4,1),),((0,4,1),)), (21,((2,4,1),),((1,4,1),)),
    (11,((4,0,1),(4,1,1),(4,2,1),(4,4,-1)),((0,4,-1),)), (22,((0,4,1),(1,4,1),(3,4,1),(4,4,1)),((0,4,1),(1,4,1))),
    (23,((0,4,1),(4,0,1)),((0,4,1),(1,0,-1))), (24,((4,0,1),),((0,0,-1),(0,4,-1))),
    (25,((0,4,1),),((1,0,1),(1,4,1))), (26,((1,4,1),(4,2,1)),((0,4,1),(1,2,-1))),
    (27,((4,2,1),),((0,2,-1),(0,4,-1))), (28,((1,4,1),),((1,2,1),(1,4,1))),
    (29,((2,0,1),(2,1,1),(2,2,1),(2,3,1),(2,5,-1)),((0,5,-1),)),
    (21,((0,5,1),(1,5,1),(2,5,1),(3,5,1),(4,5,1)),((0,5,1),(1,5,1))), (30,((1,5,1),(2,2,1)),((0,5,1),(1,2,-1))),
    (31,((2,2,1),),((0,2,-1),(0,5,-1))), (32,((1,5,1),),((1,2,1),(1,5,1))),
    (33,((0,5,1),(2,0,1)),((0,5,1),(1,0,-1))), (34,((2,0,1),),((0,0,-1),(0,5,-1))),
    (35,((0,5,1),),((1,0,1),(1,5,1))), (36,((2,3,1),(4,5,1)),((0,5,1),(1,3,-1))),
    (37,((4,5,1),),((1,3,-1),(1,5,-1))), (38,((2,3,1),),((0,3,1),(0,5,1))),
    (39,((2,1,1),(3,5,1)),((0,5,1),(1,1,-1))), (40,((3,5,1),),((1,1,-1),(1,5,-1))),
    (41,((2,1,1),),((0,1,1),(0,5,1))), (42,((3,4,1),(4,1,1)),((0,4,1),(1,1,-1))),
    (43,((4,1,1),),((0,1,-1),(0,4,-1))), (44,((3,4,1),),((1,1,1),(1,4,1))),
)
O_FORMS = (
    ((0,0,1),), ((0,0,1),(1,0,-1)), ((0,1,1),(1,1,-1)), ((1,1,1),), ((1,0,1),), ((0,2,1),), ((0,2,1),(1,2,-1)),
    ((0,2,1),(1,1,-1)), ((1,1,1),(1,2,-1)), ((0,1,1),(0,2,-1)), ((0,1,1),), ((0,3,1),(1,3,-1)), ((1,3,1),),
    ((0,2,1),(1,3,-1)), ((0,2,1),(0,3,-1)), ((1,2,1),(1,3,-1)), ((0,0,1),(1,3,-1)), ((0,0,1),(0,3,-1)),
    ((1,0,1),(1,3,-1)), ((0,3,1),), ((0,4,1),(1,4,-1)), ((1,4,1),), ((0,0,1),(1,4,-1)), ((0,0,1),(0,4,-1)),
    ((1,0,1),(1,4,-1)), ((0,2,1),(1,4,-1)), ((0,2,1),(0,4,-1)), ((1,2,1),(1,4,-1)), ((0,4,1),), ((0,5,1),(1,5,-1)),
    ((1,5,1),), ((0,2,1),(1,5,-1)), ((0,2,1),(0,5,-1)), ((1,2,1),(1,5,-1)), ((0,0,1),(1,5,-1)), ((0,0,1),(0,5,-1)),
    ((1,0,1),(1,5,-1)), ((0,1,1),(1,5,-1)), ((1,1,1),(1,5,-1)), ((0,1,1),(0,5,-1)), ((0,1,1),(1,4,-1)),
    ((0,1,1),(0,4,-1)), ((1,1,1),(1,4,-1)), ((0,3,1),(1,5,-1)), ((1,3,1),(1,5,-1)), ((0,3,1),(0,5,-1)),
)
O_PRODS = (
    (0,((0,0,1),(3,0,1),(4,0,1),(5,0,1)),((0,0,1),(1,0,1))), (1,((0,2,1),(0,3,1),(0,4,1),(0,0,-1)),((1,0,1),)),
    (2,((1,0,1),(1,1,-1)),((0,0,1),)), (3,((1,0,1),(2,0,1)),((0,0,1),(1,0,1))), (0,((0,1,1),),((0,1,1),)),
    (4,((0,1,1),),((1,1,1),)), (5,((1,1,1),(2,1,1),(3,1,1),(4,1,1),(5,1,1)),((0,1,1),(1,1,1))),
    (6,((2,0,1),(2,2,1),(2,3,1),(2,4,1),(2,1,-1)),((1,1,1),)), (7,((1,1,1),(2,0,1)),((0,0,1),(1,1,-1))),
    (8,((2,0,1),),((1,0,-1),(1,1,-1))), (9,((1,1,1),),((0,0,1),(0,1,1))),
    (10,((1,3,1),(4,3,1),(5,3,1)),((0,3,1),(1,3,1))), (2,((1,2,1),(1,4,1),(1,3,-1)),((1,3,1),)),
    (11,((3,0,1),(3,1,1),(3,3,-1)),((0,3,-1),)), (12,((0,3,1),(2,3,1),(3,3,1)),((0,3,1),(1,3,1))),
    (13,((2,3,1),(3,1,1)),((0,3,1),(1,1,-1))), (14,((3,1,1),),((0,1,-1),(0,3,-1))),
    (15,((2,3,1),),((1,1,1),(1,3,1))), (16,((0,3,1),(3,0,1)),((0,3,1),(1,0,-1))),
    (17,((3,0,1),),((0,0,-1),(0,3,-1))), (18,((0,3,1),),((1,0,1),(1,3,1))),
    (19,((3,4,1),(5,4,1)),((0,4,1),(1,4,1))), (11,((3,4,1),(3,2,-1)),((1,4,-1),)),
    (20,((4,0,1),(4,1,1),(4,3,1),(4,4,-1)),((0,4,-1),)), (21,((0,4,1),(1,4,1),(2,4,1),(4,4,1)),((0,4,1),(1,4,1))),
    (22,((0,4,1),(4,0,1)),((0,4,1),(1,0,-1))), (23,((4,0,1),),((0,0,-1),(0,4,-1))),
    (24,((0,4,1),),((1,0,1),(1,4,1))), (25,((2,4,1),(4,1,1)),((0,4,1),(1,1,-1))),
    (26,((4,1,1),),((0,1,-1),(0,4,-1))), (27,((2,4,1),),((1,1,1),(1,4,1))), (28,((4,2,1),),((0,2,1),)),
    (21,((4,2,1),),((1,2,1),)), (29,((5,0,1),(5,1,1),(5,3,1),(5,4,1),(5,2,-1)),((0,2,-1),)),
    (30,((0,2,1),(1,2,1),(2,2,1),(3,2,1),(5,2,1)),((0,2,1),(1,2,1))), (31,((2,2,1),(5,1,1)),((0,2,1),(1,1,-1))),
    (32,((5,1,1),),((0,1,-1),(0,2,-1))), (33,((2,2,1),),((1,1,1),(1,2,1))),
    (34,((0,2,1),(5,0,1)),((0,2,1),(1,0,-1))), (35,((5,0,1),),((0,0,-1),(0,2,-1))),
    (36,((0,2,1),),((1,0,1),(1,2,1))), (37,((1,2,1),(5,3,1)),((0,2,1),(1,3,-1))), (38,((1,2,1),),((1,2,1),(1,3,1))),
    (39,((5,3,1),),((0,2,-1),(0,3,-1))), (40,((1,4,1),(4,3,1)),((0,4,1),(1,3,-1))),
    (41,((4,3,1),),((0,3,-1),(0,4,-1))), (42,((1,4,1),),((1,3,1),(1,4,1))),
    (43,((3,2,1),(5,4,1)),((0,2,1),(1,4,-1))), (44,((3,2,1),),((1,2,1),(1,4,1))),
    (45,((5,4,1),),((0,2,-1),(0,4,-1))),
)
NPR = len(Q_PRODS)

ODD = ("K0", "K1", "P0", "P1", "Q0", "Q1", "Q2", "Q3", "Q4")
EVEN = ("K0", "K1", "P0", "P1", "O0", "O1", "O2")
SOFTMAX_LAG = 4


def _dot(a, b):
    return jnp.dot(a, b, preferred_element_type=f32)


def _dot_nt(a, b):
    return lax.dot_general(a, b, NT, preferred_element_type=f32)


def _unpk(v):
    return pltpu.bitcast(v, bf16)


def _tile(c):
    return slice(c * 128, (c + 1) * 128)


def _split(nparts, total=NPR):
    return [list(range(k * total // nparts, (k + 1) * total // nparts)) for k in range(nparts)]


def _lincomb(terms, get):
    v = get(terms[0][:-1])
    for t in terms[1:]:
        v = v + get(t[:-1]) if t[-1] > 0 else v - get(t[:-1])
    return v


def _packed_combos(term_lists, load):
    packed, halves = {}, ({}, {})

    def word(k):
        if k not in packed:
            packed[k] = pltpu.bitcast(load(*k), u32)
        return packed[k]

    def half(idx, k):
        if k not in halves[idx]:
            halves[idx][k] = pltpu.unpack_elementwise(word(k), index=idx, packed_dtype=bf16, unpacked_dtype=f32)
        return halves[idx][k]

    return [word(t[0][:-1]) if len(t) == 1 else
            pltpu.pack_elementwise([_lincomb(t, functools.partial(half, i)) for i in range(2)], packed_dtype=bf16)
            for t in term_lists]


def _bilinear(prods, rs, prod, c, init, done):
    last = {(s, j): r for r, p in enumerate(prods) for (s, j, _) in p[2]}
    for r in rs:
        m = prod(r)
        for (s, j, sg) in prods[r][2]:
            if (s, j) not in c and init is not None:
                c[(s, j)] = init(s, j)
            if (s, j) in c:
                c[(s, j)] = c[(s, j)] + m if sg > 0 else c[(s, j)] - m
            else:
                c[(s, j)] = m if sg > 0 else -m
            if last[(s, j)] == r:
                done(s, j, c[(s, j)])


def _recip(l):
    r = pl.reciprocal(l, approx=True)
    return r * (2.0 - l * r)


def _softmax(s, zero):
    ps = []
    for r in range(SQ // 8):
        sb = s[r * 8:(r + 1) * 8]
        m = jnp.broadcast_to(jnp.max(sb, axis=-1, keepdims=True), (8, 128))
        if r >= SOFTMAX_LAG:
            link = pltpu.bitcast(ps[r - SOFTMAX_LAG][:, 384:512], u32) & zero
            m = pltpu.bitcast(pltpu.bitcast(m, u32) | link, f32)
        ps.append(jnp.exp2(sb - jnp.concatenate([m] * 4, axis=1)))
    p = jnp.concatenate(ps, axis=0)
    t = (p[:, 0:128] + p[:, 128:256]) + (p[:, 256:384] + p[:, 384:512])
    r_row = _recip(jnp.sum(t[:TT].T, axis=0, keepdims=True))
    r_col = jnp.broadcast_to(_recip(jnp.sum(t[TT:], axis=-1, keepdims=True)), (R, 128))
    return p, r_row, r_col


def _kernel(xa, kta, vta, wqa, woa, xb, ktb, vtb, wqb, wob, o_hbm,
            acc, obuf, xraw, xc, qbuf, kvbuf, wqraw, woraw, wqc, woc, zv,
            kvsem, wsem, xsem, osem):
    xs, kvs, wqs, wos = (xa, xb), (kta, vta, ktb, vtb), (wqa, wqb), (woa, wob)

    def ring(slot, k):
        v = slot + k
        return jnp.where(v >= NS, v - NS, v)

    def kv_start(sl, t):
        hg, g = lax.shift_right_logical(t, LG) - 1, t & (NBG - 1)
        for a in range(4):
            pltpu.make_async_copy(kvs[a].at[pl.ds(g * NB, NB), pl.ds(pl.multiple_of(hg * GW, GW), GW), :],
                                  kvbuf.at[sl, a], kvsem.at[sl]).start()

    def kv_piece(k):
        a, b = k // NB, k % NB
        pltpu.make_async_copy(kvs[a].at[b, pl.ds(0, GW), :], kvbuf.at[0, a, b], kvsem.at[0]).start()

    def wq_start(hg, sl):
        cols = pl.ds(pl.multiple_of(hg * GW, GW), GW)
        for p in range(2):
            for kt in range(5):
                pltpu.make_async_copy(wqs[p].at[pl.ds(pl.multiple_of(kt * 128 + sl * SL, SL), SL), cols],
                                      wqraw.at[sl, p, kt], wsem.at[sl, 0]).start()

    def wo_start(hg, sl):
        for p in range(2):
            pltpu.make_async_copy(wos[p].at[hg, :, pl.ds(pl.multiple_of(sl * SL, SL), SL), :],
                                  woraw.at[sl, p], wsem.at[sl, 1]).start()

    def x_start(g):
        for p in range(2):
            pltpu.make_async_copy(xs[p].at[pl.ds(g * NB, NB)], xraw.at[g & 1, p], xsem.at[g & 1]).start()

    def wait_filled(v, sem):
        pltpu.make_async_copy(v, v, sem).wait()

    def w_piece(raw, dst, prods, ws, sl, p, rs):
        rows = pl.ds(pl.multiple_of(sl * (SL // 2), 8), SL // 2)
        vs = _packed_combos([prods[r][1] for r in rs], lambda i, j: raw[sl, p, i, :, _tile(j)])
        for r, v in zip(rs, vs):
            dst[ws, p, r, rows, :] = v

    wq_piece = functools.partial(w_piece, wqraw, wqc, Q_PRODS)
    wo_piece = functools.partial(w_piece, woraw, woc, O_PRODS)
    w_pieces = [(p, rs) for p in range(2) for rs in _split(5)]

    def x_piece(g, p, b, ks, r0):
        vs = _packed_combos([Q_FORMS[k] for k in ks],
                            lambda s, i: xraw[g & 1, p, b, s * HF + r0:s * HF + r0 + 16, _tile(i)])
        for k, v in zip(ks, vs):
            xc[p, g * NB + b, k, r0 // 2:r0 // 2 + 8, :] = v

    x_pieces = [(p, b, ks, r0) for p in range(2) for b in range(NB) for r0 in range(0, HF, 16)
                for ks in _split(3, len(Q_FORMS))]

    units = [(p, b) for p in range(2) for b in range(NB)]
    nu = len(units)

    def step(mode, t, slot):
        g = t & (NBG - 1)
        hq = lax.shift_right_logical(t, LG)
        qslot = hq & 1
        oslot = 1 - qslot
        gx = jnp.minimum(g + 1, NBG - 1)

        def prefetch():
            t2 = t + 2
            if mode == "start":
                for k in range(1, NBG):
                    pl.when(g + 1 == k)(functools.partial(kv_piece, k))
            else:
                pl.when(t2 < T + NBG)(functools.partial(kv_start, ring(slot, 2), t2))
            if mode != "last":
                h2, g2 = lax.shift_right_logical(t2, LG), t2 & (NBG - 1)
                pl.when(h2 + 1 < NG)(functools.partial(wq_start, h2 + 1, g2))
                pl.when(h2 < NG)(functools.partial(wo_start, h2, g2))

        if mode == "start":
            pl.when(g + 2 < NBG)(functools.partial(x_start, g + 2))
            pl.when(g + 1 < NBG)(functools.partial(wait_filled, xraw.at[gx & 1], xsem.at[gx & 1]))
        if mode != "last":
            pl.when(hq + 1 < NG)(functools.partial(wait_filled, wqraw.at[g], wsem.at[g, 0]))
            wait_filled(woraw.at[g], wsem.at[g, 1])
        if mode != "start":
            wait_filled(kvbuf.at[slot], kvsem.at[slot])

        st = [dict() for _ in range(2 * nu)]
        zero = zv[...]
        jq = [functools.partial(wq_piece, 1 - qslot, g, *a) for a in w_pieces]
        jo = [functools.partial(wo_piece, 1 - oslot, g, *a) for a in w_pieces]
        jx = [functools.partial(x_piece, gx, *a) for a in x_pieces]
        todo = {"start": (jq + jo, [], jx), "last": ([], [], [])}.get(mode, (jq, jo, []))
        every = (3 if mode == "start" else 5, 4, 1)
        count = [0, 0, 0]

        def side_job(kind):
            count[kind] += 1
            if count[kind] % every[kind] == 0 and todo[kind]:
                todo[kind].pop(0)()

        def task_q(u, j):
            p, b = units[u]

            def prod(r):
                side_job(0)
                side_job(2)
                return _dot(_unpk(xc[p, g * NB + b, Q_PRODS[r][0]]), _unpk(wqc[qslot, p, r]))

            def done(s, col, v):
                qbuf[g * nu + u, col, s * HF // 2:(s + 1) * HF // 2, :] = pltpu.bitcast((v * QSCALE).astype(bf16), u32)

            _bilinear(Q_PRODS, _split(5)[j], prod, st[2 * u].setdefault("qc", {}), None, done)

        def task_k(i, h):
            p, b = units[i // 2]
            k0 = (i % 2) * PW + h * 128
            kt = kvbuf.at[slot, 2 * p, b]
            lane = lax.broadcasted_iota(jnp.int32, (HF, 128), 1)
            q = [qbuf[g * nu + i // 2, 3 * (i % 2) + h + c] for c in range(2)]
            q[1 - h] = jnp.where((lane < 64) if h == 0 else (lane >= 64), q[1 - h], jnp.uint32(0))
            q = _unpk(jnp.concatenate(q, axis=1))
            s = jnp.concatenate([_dot(q, kt[k0:k0 + 256, c:c + 256]) for c in (0, 256)], axis=1)
            st[i][h] = _softmax(s, zero)

        def task_p(i, h):
            p, b = units[i // 2]
            k0 = (i % 2) * PW
            vt = kvbuf.at[slot, 2 * p + 1, b]
            d = st[i]
            if h == 0:
                d["ot"] = _dot_nt(vt[k0:k0 + 192, :], d[0][0][:TT].astype(bf16))
                d["oa"] = _dot_nt(d[0][0][TT:].astype(bf16), vt[k0:k0 + 128, :])
                return
            (p1, row1, col1), (p2, row2, col2) = d[0], d[1]
            om = _dot_nt(jnp.concatenate([p1[TT:], p2[TT:]], axis=0).astype(bf16), vt[k0 + 128:k0 + 256, :])
            ot2 = _dot_nt(vt[k0 + 192:k0 + 384, :], p2[:TT].astype(bf16))
            oc = _dot_nt(p2[TT:].astype(bf16), vt[k0 + 256:k0 + 384, :])
            ot1 = d["ot"] * row1
            ot2 = ot2 * row2
            lane = lax.broadcasted_iota(jnp.int32, (R, 128), 1)
            om = jnp.where(lane < 64, om[:R] * col1, om[R:] * col2)
            ta = ot1[0:128].T
            tm = jnp.concatenate([ot1[128:192], ot2[0:64]], axis=0).T
            tc = ot2[64:192].T
            d["o"] = [jnp.concatenate([ta, d["oa"] * col1], axis=0),
                      jnp.concatenate([tm, om], axis=0),
                      jnp.concatenate([tc, oc * col2], axis=0)]

        def task_o(u, j):
            p, b = units[u]
            d = st[2 * u]
            o = st[2 * u]["o"] + st[2 * u + 1]["o"]
            row0 = (g * NB + b) * SQ

            def idx(s, col):
                return pl.ds(pl.multiple_of(row0 + s * HF, 16), HF), _tile(p * 5 + col)

            def done(s, col, v):
                if mode == "last":
                    obuf[idx(s, col)] = v.astype(bf16)
                else:
                    acc[idx(s, col)] = v

            def prod(r):
                side_job(1)
                f = O_PRODS[r][0]
                if ("form", f) not in d:
                    d["form", f] = _lincomb(O_FORMS[f], lambda k: o[k[1]][k[0] * HF:(k[0] + 1) * HF]).astype(bf16)
                return _dot(d["form", f], _unpk(woc[oslot, p, r]))

            init = None if mode == "first" else (lambda s, col: acc[idx(s, col)])
            _bilinear(O_PRODS, _split(3)[j], prod, d.setdefault("oc", {}), init, done)
            if mode == "last" and j == 2:
                win = (pl.ds(pl.multiple_of(row0, 16), SQ), pl.ds(p * D, D))
                pltpu.make_async_copy(obuf.at[win], o_hbm.at[win], osem.at[0]).start()

        if mode == "start":
            seq = [("Q", u, j) for u in range(nu) for j in range(5)]
        else:
            seq = []
            for s in range(-1, 2 * nu + 1):
                for kind, j in (ODD if s % 2 else EVEN):
                    i = {"Q": (s - 1) // 2, "O": s // 2 - 1, "K": s + 1, "P": s}[kind]
                    if 0 <= i < (nu if kind in "QO" else 2 * nu) and (kind != "Q" or mode != "last"):
                        seq.append((kind, i, int(j)))
            late = [x for x in seq if x[:2] == ("O", nu - 2)][(2 if mode == "last" else 1):]
            seq = [x for x in seq if x not in late]
            pos = seq.index(("P", 2 * nu - 1, 1)) + 1
            seq[pos:pos] = late
        tasks = {"Q": task_q, "K": task_k, "P": task_p, "O": task_o}
        for n, (kind, i, j) in enumerate(seq):
            if n == 1:
                prefetch()
            tasks[kind](i, j)
        for jobs in todo:
            for job in jobs:
                job()

    def loop(lo, hi, fn):
        def body(i, c):
            fn(i)
            return c
        lax.fori_loop(lo, hi, body, 0)

    def steps(mode, lo, hi, slot0):
        def body(t, slot):
            step(mode, t, slot)
            return ring(slot, 1)
        return lax.fori_loop(lo, hi, body, slot0)

    def first_wq(sl):
        wait_filled(wqraw.at[sl], wsem.at[sl, 0])
        for a in w_pieces:
            wq_piece(0, sl, *a)

        @pl.when(sl < 2)
        def _():
            wq_start(1, sl)
            wo_start(0, sl)

    zv[...] = jnp.zeros((8, 128), u32)
    loop(0, 1, x_start)
    loop(0, NBG, functools.partial(wq_start, 0))
    x_start(1)
    wait_filled(xraw.at[0], xsem.at[0])
    for a in x_pieces:
        x_piece(0, *a)
    loop(0, NBG, first_wq)
    kv_piece(0)
    steps("start", 0, NBG, jnp.int32(0))
    kv_start(1, NBG + 1)
    slot = steps("first", NBG, 2 * NBG, jnp.int32(0))
    slot = steps("mid", 2 * NBG, T, slot)
    steps("last", T, T + NBG, slot)
    pltpu.make_async_copy(obuf, o_hbm, osem.at[0]).wait()


@jax.jit
def pallas_concat_heads__gqa_block_cached__mha_block_cached__near_ridge_kernel(
    A_x: jax.Array,
    A_k_cache: jax.Array,
    A_v_cache: jax.Array,
    A_wq: jax.Array,
    A_wo: jax.Array,
    B_x: jax.Array,
    B_k_cache: jax.Array,
    B_v_cache: jax.Array,
    B_wq: jax.Array,
    B_wo: jax.Array,
):
    def kv(c):
        return jnp.swapaxes(c, 2, 3).reshape(B, H * DH, SK)

    def wo(w):
        return w.reshape(NG, GW // 128, 128, D)

    hbm = pl.BlockSpec(memory_space=pl.ANY)
    out = pl.pallas_call(
        _kernel,
        in_specs=[hbm] * 10,
        out_specs=hbm,
        out_shape=jax.ShapeDtypeStruct((B * SQ, 2 * D), bf16),
        scratch_shapes=[
            pltpu.VMEM((B * SQ, 2 * D), f32),
            pltpu.VMEM((B * SQ, 2 * D), bf16),
            pltpu.VMEM((2, 2, NB, SQ, D), bf16),
            pltpu.VMEM((2, B, len(Q_FORMS), HF // 2, 128), u32),
            pltpu.VMEM((NBG * 2 * NB, 6, HF, 128), u32),
            pltpu.VMEM((NS, 4, NB, GW, SK), bf16),
            pltpu.VMEM((NBG, 2, 5, SL, GW), bf16),
            pltpu.VMEM((NBG, 2, 6, SL, D), bf16),
            pltpu.VMEM((2, 2, NPR, 64, 128), u32),
            pltpu.VMEM((2, 2, NPR, 64, 128), u32),
            pltpu.VMEM((8, 128), u32),
            pltpu.SemaphoreType.DMA((NS,)),
            pltpu.SemaphoreType.DMA((NBG, 2)),
            pltpu.SemaphoreType.DMA((2,)),
            pltpu.SemaphoreType.DMA((1,)),
        ],
        compiler_params=pltpu.CompilerParams(vmem_limit_bytes=112 * 1024 * 1024, disable_bounds_checks=True),
    )(A_x, kv(A_k_cache), kv(A_v_cache), A_wq, wo(A_wo), B_x, kv(B_k_cache), kv(B_v_cache), B_wq, wo(B_wo))
    return out.reshape(B, SQ, 2 * D)
```

```python
import functools

import jax
import jax.numpy as jnp
from jax import lax
from jax.experimental import pallas as pl
from jax.experimental.pallas import tpu as pltpu

B, SQ, D, H, SK, DH = 16, 160, 640, 32, 512, 192
PW = 2 * DH
GW = 2 * PW
NG = H * DH // GW
NB = 2
NBG = B // NB
LG = NBG.bit_length() - 1
T = NG * NBG
SL = 128 // NBG
NS = 3
HF = SQ // 2
TT = 128
R = SQ - TT
QSCALE = (DH ** -0.5) * 1.4426950408889634
NT = (((1,), (1,)), ((), ()))
f32, bf16, u32 = jnp.float32, jnp.bfloat16, jnp.uint32

Q_FORMS = (
    ((0,0,1),(1,0,-1)), ((1,0,1),), ((0,1,1),), ((0,1,1),(1,1,-1)), ((0,3,1),), ((0,3,1),(1,3,-1)),
    ((0,1,1),(1,0,-1)), ((1,0,1),(1,1,-1)), ((0,0,1),(0,1,-1)), ((1,3,1),), ((0,4,1),), ((0,4,1),(1,4,-1)),
    ((0,1,1),(1,3,-1)), ((0,1,1),(0,3,-1)), ((1,1,1),(1,3,-1)), ((0,0,1),), ((1,1,1),), ((0,0,1),(1,3,-1)),
    ((0,0,1),(0,3,-1)), ((1,0,1),(1,3,-1)), ((0,2,1),), ((1,2,1),), ((1,4,1),), ((0,0,1),(1,4,-1)),
    ((0,0,1),(0,4,-1)), ((1,0,1),(1,4,-1)), ((0,1,1),(1,4,-1)), ((0,1,1),(0,4,-1)), ((1,1,1),(1,4,-1)),
    ((0,2,1),(1,2,-1)), ((0,1,1),(1,2,-1)), ((0,1,1),(0,2,-1)), ((1,1,1),(1,2,-1)), ((0,0,1),(1,2,-1)),
    ((0,0,1),(0,2,-1)), ((1,0,1),(1,2,-1)), ((0,4,1),(1,2,-1)), ((1,2,1),(1,4,-1)), ((0,2,1),(0,4,-1)),
    ((0,3,1),(1,2,-1)), ((1,2,1),(1,3,-1)), ((0,2,1),(0,3,-1)), ((0,3,1),(1,4,-1)), ((0,3,1),(0,4,-1)),
    ((1,3,1),(1,4,-1)),
)
Q_PRODS = (
    (0,((0,1,1),(0,2,-1)),((0,1,1),)), (1,((0,1,1),(1,1,1)),((0,1,1),(1,1,1))),
    (2,((0,2,1),(1,2,1),(2,2,1),(3,2,1),(4,2,1)),((0,2,1),(1,2,1))),
    (3,((1,1,1),(1,3,1),(1,4,1),(1,5,1),(1,2,-1)),((1,2,1),)), (4,((2,1,1),(3,1,1),(4,1,1)),((0,1,1),(1,1,1))),
    (5,((3,4,1),(3,5,1),(3,1,-1)),((1,1,1),)), (6,((0,2,1),(1,1,1)),((0,1,1),(1,2,-1))),
    (7,((1,1,1),),((1,1,-1),(1,2,-1))), (8,((0,2,1),),((0,1,1),(0,2,1))),
    (5,((3,0,1),(3,2,1),(3,3,-1)),((0,3,-1),)), (9,((0,3,1),(1,3,1),(3,3,1)),((0,3,1),(1,3,1))),
    (10,((2,3,1),(4,3,1)),((0,3,1),(1,3,1))), (11,((4,3,1),(4,5,-1)),((1,3,-1),)),
    (12,((1,3,1),(3,2,1)),((0,3,1),(1,2,-1))), (13,((3,2,1),),((0,2,-1),(0,3,-1))),
    (14,((1,3,1),),((1,2,1),(1,3,1))), (15,((0,0,1),(2,0,1),(3,0,1),(4,0,1)),((0,0,1),(1,0,1))),
    (0,((0,3,1),(0,4,1),(0,5,1),(0,0,-1)),((1,0,1),)), (2,((1,0,1),),((0,0,1),)), (16,((1,0,1),),((1,0,1),)),
    (17,((0,3,1),(3,0,1)),((0,3,1),(1,0,-1))), (18,((3,0,1),),((0,0,-1),(0,3,-1))),
    (19,((0,3,1),),((1,0,1),(1,3,1))), (20,((2,4,1),),((0,4,1),)), (21,((2,4,1),),((1,4,1),)),
    (11,((4,0,1),(4,1,1),(4,2,1),(4,4,-1)),((0,4,-1),)), (22,((0,4,1),(1,4,1),(3,4,1),(4,4,1)),((0,4,1),(1,4,1))),
    (23,((0,4,1),(4,0,1)),((0,4,1),(1,0,-1))), (24,((4,0,1),),((0,0,-1),(0,4,-1))),
    (25,((0,4,1),),((1,0,1),(1,4,1))), (26,((1,4,1),(4,2,1)),((0,4,1),(1,2,-1))),
    (27,((4,2,1),),((0,2,-1),(0,4,-1))), (28,((1,4,1),),((1,2,1),(1,4,1))),
    (29,((2,0,1),(2,1,1),(2,2,1),(2,3,1),(2,5,-1)),((0,5,-1),)),
    (21,((0,5,1),(1,5,1),(2,5,1),(3,5,1),(4,5,1)),((0,5,1),(1,5,1))), (30,((1,5,1),(2,2,1)),((0,5,1),(1,2,-1))),
    (31,((2,2,1),),((0,2,-1),(0,5,-1))), (32,((1,5,1),),((1,2,1),(1,5,1))),
    (33,((0,5,1),(2,0,1)),((0,5,1),(1,0,-1))), (34,((2,0,1),),((0,0,-1),(0,5,-1))),
    (35,((0,5,1),),((1,0,1),(1,5,1))), (36,((2,3,1),(4,5,1)),((0,5,1),(1,3,-1))),
    (37,((4,5,1),),((1,3,-1),(1,5,-1))), (38,((2,3,1),),((0,3,1),(0,5,1))),
    (39,((2,1,1),(3,5,1)),((0,5,1),(1,1,-1))), (40,((3,5,1),),((1,1,-1),(1,5,-1))),
    (41,((2,1,1),),((0,1,1),(0,5,1))), (42,((3,4,1),(4,1,1)),((0,4,1),(1,1,-1))),
    (43,((4,1,1),),((0,1,-1),(0,4,-1))), (44,((3,4,1),),((1,1,1),(1,4,1))),
)
O_FORMS = (
    ((0,0,1),), ((0,0,1),(1,0,-1)), ((0,1,1),(1,1,-1)), ((1,1,1),), ((1,0,1),), ((0,2,1),), ((0,2,1),(1,2,-1)),
    ((0,2,1),(1,1,-1)), ((1,1,1),(1,2,-1)), ((0,1,1),(0,2,-1)), ((0,1,1),), ((0,3,1),(1,3,-1)), ((1,3,1),),
    ((0,2,1),(1,3,-1)), ((0,2,1),(0,3,-1)), ((1,2,1),(1,3,-1)), ((0,0,1),(1,3,-1)), ((0,0,1),(0,3,-1)),
    ((1,0,1),(1,3,-1)), ((0,3,1),), ((0,4,1),(1,4,-1)), ((1,4,1),), ((0,0,1),(1,4,-1)), ((0,0,1),(0,4,-1)),
    ((1,0,1),(1,4,-1)), ((0,2,1),(1,4,-1)), ((0,2,1),(0,4,-1)), ((1,2,1),(1,4,-1)), ((0,4,1),), ((0,5,1),(1,5,-1)),
    ((1,5,1),), ((0,2,1),(1,5,-1)), ((0,2,1),(0,5,-1)), ((1,2,1),(1,5,-1)), ((0,0,1),(1,5,-1)), ((0,0,1),(0,5,-1)),
    ((1,0,1),(1,5,-1)), ((0,1,1),(1,5,-1)), ((1,1,1),(1,5,-1)), ((0,1,1),(0,5,-1)), ((0,1,1),(1,4,-1)),
    ((0,1,1),(0,4,-1)), ((1,1,1),(1,4,-1)), ((0,3,1),(1,5,-1)), ((1,3,1),(1,5,-1)), ((0,3,1),(0,5,-1)),
)
O_PRODS = (
    (0,((0,0,1),(3,0,1),(4,0,1),(5,0,1)),((0,0,1),(1,0,1))), (1,((0,2,1),(0,3,1),(0,4,1),(0,0,-1)),((1,0,1),)),
    (2,((1,0,1),(1,1,-1)),((0,0,1),)), (3,((1,0,1),(2,0,1)),((0,0,1),(1,0,1))), (0,((0,1,1),),((0,1,1),)),
    (4,((0,1,1),),((1,1,1),)), (5,((1,1,1),(2,1,1),(3,1,1),(4,1,1),(5,1,1)),((0,1,1),(1,1,1))),
    (6,((2,0,1),(2,2,1),(2,3,1),(2,4,1),(2,1,-1)),((1,1,1),)), (7,((1,1,1),(2,0,1)),((0,0,1),(1,1,-1))),
    (8,((2,0,1),),((1,0,-1),(1,1,-1))), (9,((1,1,1),),((0,0,1),(0,1,1))),
    (10,((1,3,1),(4,3,1),(5,3,1)),((0,3,1),(1,3,1))), (2,((1,2,1),(1,4,1),(1,3,-1)),((1,3,1),)),
    (11,((3,0,1),(3,1,1),(3,3,-1)),((0,3,-1),)), (12,((0,3,1),(2,3,1),(3,3,1)),((0,3,1),(1,3,1))),
    (13,((2,3,1),(3,1,1)),((0,3,1),(1,1,-1))), (14,((3,1,1),),((0,1,-1),(0,3,-1))),
    (15,((2,3,1),),((1,1,1),(1,3,1))), (16,((0,3,1),(3,0,1)),((0,3,1),(1,0,-1))),
    (17,((3,0,1),),((0,0,-1),(0,3,-1))), (18,((0,3,1),),((1,0,1),(1,3,1))),
    (19,((3,4,1),(5,4,1)),((0,4,1),(1,4,1))), (11,((3,4,1),(3,2,-1)),((1,4,-1),)),
    (20,((4,0,1),(4,1,1),(4,3,1),(4,4,-1)),((0,4,-1),)), (21,((0,4,1),(1,4,1),(2,4,1),(4,4,1)),((0,4,1),(1,4,1))),
    (22,((0,4,1),(4,0,1)),((0,4,1),(1,0,-1))), (23,((4,0,1),),((0,0,-1),(0,4,-1))),
    (24,((0,4,1),),((1,0,1),(1,4,1))), (25,((2,4,1),(4,1,1)),((0,4,1),(1,1,-1))),
    (26,((4,1,1),),((0,1,-1),(0,4,-1))), (27,((2,4,1),),((1,1,1),(1,4,1))), (28,((4,2,1),),((0,2,1),)),
    (21,((4,2,1),),((1,2,1),)), (29,((5,0,1),(5,1,1),(5,3,1),(5,4,1),(5,2,-1)),((0,2,-1),)),
    (30,((0,2,1),(1,2,1),(2,2,1),(3,2,1),(5,2,1)),((0,2,1),(1,2,1))), (31,((2,2,1),(5,1,1)),((0,2,1),(1,1,-1))),
    (32,((5,1,1),),((0,1,-1),(0,2,-1))), (33,((2,2,1),),((1,1,1),(1,2,1))),
    (34,((0,2,1),(5,0,1)),((0,2,1),(1,0,-1))), (35,((5,0,1),),((0,0,-1),(0,2,-1))),
    (36,((0,2,1),),((1,0,1),(1,2,1))), (37,((1,2,1),(5,3,1)),((0,2,1),(1,3,-1))), (38,((1,2,1),),((1,2,1),(1,3,1))),
    (39,((5,3,1),),((0,2,-1),(0,3,-1))), (40,((1,4,1),(4,3,1)),((0,4,1),(1,3,-1))),
    (41,((4,3,1),),((0,3,-1),(0,4,-1))), (42,((1,4,1),),((1,3,1),(1,4,1))),
    (43,((3,2,1),(5,4,1)),((0,2,1),(1,4,-1))), (44,((3,2,1),),((1,2,1),(1,4,1))),
    (45,((5,4,1),),((0,2,-1),(0,4,-1))),
)
NPR = len(Q_PRODS)
XC_FORMS = len(Q_FORMS) + 1

ODD = ("K0", "K1", "P0", "P1", "Q0", "Q1", "Q2", "Q3", "Q4")
EVEN = ("K0", "K1", "P0", "P1", "O0", "O1", "O2")
SOFTMAX_LAG = 4


def _dot(a, b):
    return jnp.dot(a, b, preferred_element_type=f32)


def _dot_nt(a, b):
    return lax.dot_general(a, b, NT, preferred_element_type=f32)


def _unpk(v):
    return pltpu.bitcast(v, bf16)


def _tile(c):
    return slice(c * 128, (c + 1) * 128)


def _split(nparts, total=NPR):
    return [list(range(k * total // nparts, (k + 1) * total // nparts)) for k in range(nparts)]


def _lincomb(terms, get):
    v = get(terms[0][:-1])
    for t in terms[1:]:
        v = v + get(t[:-1]) if t[-1] > 0 else v - get(t[:-1])
    return v


def _packed_combos(term_lists, load):
    wide = {}

    def get(k):
        if k not in wide:
            wide[k] = load(*k).astype(f32)
        return wide[k]

    out = {n: pltpu.bitcast(load(*t[0][:-1]), u32) for n, t in enumerate(term_lists) if len(t) == 1}
    sums = [n for n in range(len(term_lists)) if n not in out]
    for pair in (sums[n:n + 2] for n in range(0, len(sums), 2)):
        v = jnp.concatenate([_lincomb(term_lists[n], get) for n in pair], axis=1)
        v = pltpu.bitcast(v.astype(bf16), u32)
        for c, n in enumerate(pair):
            out[n] = v[:, _tile(c)]
    return [out[n] for n in range(len(term_lists))]


def _bilinear(prods, rs, prod, c, init, done):
    last = {(s, j): r for r, p in enumerate(prods) for (s, j, _) in p[2]}
    for r in rs:
        m = prod(r)
        for (s, j, sg) in prods[r][2]:
            if (s, j) not in c and init is not None:
                c[(s, j)] = init(s, j)
            if (s, j) in c:
                c[(s, j)] = c[(s, j)] + m if sg > 0 else c[(s, j)] - m
            else:
                c[(s, j)] = m if sg > 0 else -m
            if last[(s, j)] == r:
                done(s, j, c[(s, j)])


def _recip(l):
    r = pl.reciprocal(l, approx=True)
    return r * (2.0 - l * r)


def _softmax(s, zero):
    ps = []
    for r in range(SQ // 8):
        sb = s[r * 8:(r + 1) * 8]
        m = jnp.broadcast_to(jnp.max(sb, axis=-1, keepdims=True), (8, 128))
        if r >= SOFTMAX_LAG:
            link = pltpu.bitcast(ps[r - SOFTMAX_LAG][:, 384:512], u32) & zero
            m = pltpu.bitcast(pltpu.bitcast(m, u32) | link, f32)
        ps.append(jnp.exp2(sb - jnp.concatenate([m] * 4, axis=1)))
    p = jnp.concatenate(ps, axis=0)
    t = (p[:, 0:128] + p[:, 128:256]) + (p[:, 256:384] + p[:, 384:512])
    r_row = _recip(jnp.sum(t[:TT].T, axis=0, keepdims=True))
    r_col = jnp.broadcast_to(_recip(jnp.sum(t[TT:], axis=-1, keepdims=True)), (R, 128))
    return p, r_row, r_col


def _kernel(xa, kta, vta, wqa, woa, xb, ktb, vtb, wqb, wob, o_hbm,
            acc, obuf, xraw, xc, qbuf, kvbuf, wqraw, woraw, wqc, woc, zv,
            kvsem, wsem, xsem, osem):
    xs, kvs, wqs, wos = (xa, xb), (kta, vta, ktb, vtb), (wqa, wqb), (woa, wob)

    def ring(slot, k):
        v = slot + k
        return jnp.where(v >= NS, v - NS, v)

    def kv_start(sl, t):
        hg, g = lax.shift_right_logical(t, LG) - 1, t & (NBG - 1)
        for a in range(4):
            pltpu.make_async_copy(kvs[a].at[pl.ds(g * NB, NB), pl.ds(pl.multiple_of(hg * GW, GW), GW), :],
                                  kvbuf.at[sl, a], kvsem.at[sl]).start()

    def kv_piece(k):
        a, b = k // NB, k % NB
        pltpu.make_async_copy(kvs[a].at[b, pl.ds(0, GW), :], kvbuf.at[0, a, b], kvsem.at[0]).start()

    def wq_start(hg, sl):
        cols = pl.ds(pl.multiple_of(hg * GW, GW), GW)
        for p in range(2):
            for kt in range(5):
                pltpu.make_async_copy(wqs[p].at[pl.ds(pl.multiple_of(kt * 128 + sl * SL, SL), SL), cols],
                                      wqraw.at[sl, p, kt], wsem.at[sl, 0]).start()

    def wo_start(hg, sl):
        for p in range(2):
            pltpu.make_async_copy(wos[p].at[hg, :, pl.ds(pl.multiple_of(sl * SL, SL), SL), :],
                                  woraw.at[sl, p], wsem.at[sl, 1]).start()

    def x_start(g):
        for p in range(2):
            pltpu.make_async_copy(xs[p].at[pl.ds(g * NB, NB)], xraw.at[g & 1, p], xsem.at[g & 1]).start()

    def wait_filled(v, sem):
        pltpu.make_async_copy(v, v, sem).wait()

    def w_piece(raw, dst, prods, ws, sl, p, rs):
        rows = pl.ds(pl.multiple_of(sl * (SL // 2), 8), SL // 2)
        vs = _packed_combos([prods[r][1] for r in rs], lambda i, j: raw[sl, p, i, :, _tile(j)])
        for r, v in zip(rs, vs):
            dst[ws, p, r, rows, :] = v

    wq_piece = functools.partial(w_piece, wqraw, wqc, Q_PRODS)
    wo_piece = functools.partial(w_piece, woraw, woc, O_PRODS)
    w_pieces = [(p, rs) for p in range(2) for rs in _split(5)]

    def x_piece(g, p, b, ks, r0):
        vs = _packed_combos([Q_FORMS[k] for k in ks],
                            lambda s, i: xraw[g & 1, p, b, s * HF + r0:s * HF + r0 + 16, _tile(i)])
        for k, v in zip(ks, vs):
            xc[p, g * NB + b, k, r0 // 2:r0 // 2 + 8, :] = v

    x_pieces = [(p, b, ks, r0) for p in range(2) for b in range(NB) for r0 in range(0, HF, 16)
                for ks in _split(5, len(Q_FORMS))]

    units = [(p, b) for p in range(2) for b in range(NB)]
    nu = len(units)

    def step(mode, t, slot):
        g = t & (NBG - 1)
        hq = lax.shift_right_logical(t, LG)
        qslot = hq & 1
        oslot = 1 - qslot
        gx = jnp.minimum(g + 1, NBG - 1)

        def prefetch():
            t2 = t + 2
            if mode == "start":
                for k in range(1, NBG):
                    pl.when(g + 1 == k)(functools.partial(kv_piece, k))
            else:
                pl.when(t2 < T + NBG)(functools.partial(kv_start, ring(slot, 2), t2))
            if mode != "last":
                h2, g2 = lax.shift_right_logical(t2, LG), t2 & (NBG - 1)
                pl.when(h2 + 1 < NG)(functools.partial(wq_start, h2 + 1, g2))
                pl.when(h2 < NG)(functools.partial(wo_start, h2, g2))

        if mode == "start":
            pl.when(g + 2 < NBG)(functools.partial(x_start, g + 2))
            pl.when(g + 1 < NBG)(functools.partial(wait_filled, xraw.at[gx & 1], xsem.at[gx & 1]))
        if mode != "last":
            pl.when(hq + 1 < NG)(functools.partial(wait_filled, wqraw.at[g], wsem.at[g, 0]))
            wait_filled(woraw.at[g], wsem.at[g, 1])
        if mode != "start":
            wait_filled(kvbuf.at[slot], kvsem.at[slot])

        st = [dict() for _ in range(2 * nu)]
        zero = zv[...]
        jq = [functools.partial(wq_piece, 1 - qslot, g, *a) for a in w_pieces]
        jo = [functools.partial(wo_piece, 1 - oslot, g, *a) for a in w_pieces]
        jx = [functools.partial(x_piece, gx, *a) for a in x_pieces]
        todo = {"start": (jq + jo, [], jx), "last": ([], [], [])}.get(mode, (jq, jo, []))
        every = (3 if mode == "start" else 5, 4, 1)
        count = [0, 0, 0]

        def side_job(kind):
            count[kind] += 1
            if count[kind] % every[kind] == 0 and todo[kind]:
                todo[kind].pop(0)()

        def task_q(u, j):
            p, b = units[u]

            def prod(r):
                side_job(0)
                side_job(2)
                return _dot(_unpk(xc[p, g * NB + b, Q_PRODS[r][0]]), _unpk(wqc[qslot, p, r]))

            def done(s, col, v):
                qbuf[g * nu + u, col, s * HF // 2:(s + 1) * HF // 2, :] = pltpu.bitcast((v * QSCALE).astype(bf16), u32)

            _bilinear(Q_PRODS, _split(5)[j], prod, st[2 * u].setdefault("qc", {}), None, done)

        def task_k(i, h):
            p, b = units[i // 2]
            k0 = (i % 2) * PW + h * 128
            kt = kvbuf.at[slot, 2 * p, b]
            lane = lax.broadcasted_iota(jnp.int32, (HF, 128), 1)
            q = [qbuf[g * nu + i // 2, 3 * (i % 2) + h + c] for c in range(2)]
            q[1 - h] = jnp.where((lane < 64) if h == 0 else (lane >= 64), q[1 - h], jnp.uint32(0))
            q = _unpk(jnp.concatenate(q, axis=1))
            s = jnp.concatenate([_dot(q, kt[k0:k0 + 256, c:c + 256]) for c in (0, 256)], axis=1)
            st[i][h] = _softmax(s, zero)

        def task_p(i, h):
            p, b = units[i // 2]
            k0 = (i % 2) * PW
            vt = kvbuf.at[slot, 2 * p + 1, b]
            d = st[i]
            if h == 0:
                d["ot"] = _dot_nt(vt[k0:k0 + 192, :], d[0][0][:TT].astype(bf16))
                d["oa"] = _dot_nt(d[0][0][TT:].astype(bf16), vt[k0:k0 + 128, :])
                return
            (p1, row1, col1), (p2, row2, col2) = d[0], d[1]
            om = _dot_nt(jnp.concatenate([p1[TT:], p2[TT:]], axis=0).astype(bf16), vt[k0 + 128:k0 + 256, :])
            ot2 = _dot_nt(vt[k0 + 192:k0 + 384, :], p2[:TT].astype(bf16))
            oc = _dot_nt(p2[TT:].astype(bf16), vt[k0 + 256:k0 + 384, :])
            ot1 = d["ot"] * row1
            ot2 = ot2 * row2
            lane = lax.broadcasted_iota(jnp.int32, (R, 128), 1)
            om = jnp.where(lane < 64, om[:R] * col1, om[R:] * col2)
            ta = ot1[0:128].T
            tm = jnp.concatenate([ot1[128:192], ot2[0:64]], axis=0).T
            tc = ot2[64:192].T
            d["o"] = [jnp.concatenate([ta, d["oa"] * col1], axis=0),
                      jnp.concatenate([tm, om], axis=0),
                      jnp.concatenate([tc, oc * col2], axis=0)]

        def task_o(u, j):
            p, b = units[u]
            d = st[2 * u]
            o = st[2 * u]["o"] + st[2 * u + 1]["o"]
            row0 = (g * NB + b) * SQ

            def idx(s, col):
                return pl.ds(pl.multiple_of(row0 + s * HF, 16), HF), _tile(p * 5 + col)

            def done(s, col, v):
                if mode == "last":
                    obuf[idx(s, col)] = v.astype(bf16)
                else:
                    acc[idx(s, col)] = v

            def prod(r):
                side_job(1)
                f = O_PRODS[r][0]
                if ("form", f) not in d:
                    d["form", f] = _lincomb(O_FORMS[f], lambda k: o[k[1]][k[0] * HF:(k[0] + 1) * HF]).astype(bf16)
                return _dot(d["form", f], _unpk(woc[oslot, p, r]))

            init = None if mode == "first" else (lambda s, col: acc[idx(s, col)])
            _bilinear(O_PRODS, _split(3)[j], prod, d.setdefault("oc", {}), init, done)
            if mode == "last" and j == 2:
                win = (pl.ds(pl.multiple_of(row0, 16), SQ), pl.ds(p * D, D))
                pltpu.make_async_copy(obuf.at[win], o_hbm.at[win], osem.at[0]).start()

        if mode == "start":
            seq = [("Q", u, j) for u in range(nu) for j in range(5)]
        else:
            seq = []
            for s in range(-1, 2 * nu + 1):
                for kind, j in (ODD if s % 2 else EVEN):
                    i = {"Q": (s - 1) // 2, "O": s // 2 - 1, "K": s + 1, "P": s}[kind]
                    if 0 <= i < (nu if kind in "QO" else 2 * nu) and (kind != "Q" or mode != "last"):
                        seq.append((kind, i, int(j)))
            late = [x for x in seq if x[:2] == ("O", nu - 2)][{"last": 2, "first": 1, "mid": 0}[mode]:]
            seq = [x for x in seq if x not in late]
            pos = seq.index(("P", 2 * nu - 1, 1)) + 1
            seq[pos:pos] = late
        tasks = {"Q": task_q, "K": task_k, "P": task_p, "O": task_o}
        for n, (kind, i, j) in enumerate(seq):
            if n == 1:
                prefetch()
            tasks[kind](i, j)
        for jobs in todo:
            for job in jobs:
                job()

    def loop(lo, hi, fn):
        def body(i, c):
            fn(i)
            return c
        lax.fori_loop(lo, hi, body, 0)

    def steps(mode, lo, hi, slot0):
        def body(t, slot):
            step(mode, t, slot)
            return ring(slot, 1)
        return lax.fori_loop(lo, hi, body, slot0)

    def first_wq(sl):
        wait_filled(wqraw.at[sl], wsem.at[sl, 0])
        for a in w_pieces:
            wq_piece(0, sl, *a)

        @pl.when(sl < 2)
        def _():
            wq_start(1, sl)
            wo_start(0, sl)

    zv[...] = jnp.zeros((8, 128), u32)
    loop(0, 1, x_start)
    loop(0, NBG, functools.partial(wq_start, 0))
    x_start(1)
    wait_filled(xraw.at[0], xsem.at[0])
    for a in x_pieces:
        x_piece(0, *a)
    loop(0, NBG, first_wq)
    kv_piece(0)
    steps("start", 0, NBG, jnp.int32(0))
    kv_start(1, NBG + 1)
    slot = steps("first", NBG, 2 * NBG, jnp.int32(0))
    slot = steps("mid", 2 * NBG, T, slot)
    steps("last", T, T + NBG, slot)
    pltpu.make_async_copy(obuf, o_hbm, osem.at[0]).wait()


@jax.jit
def pallas_concat_heads__gqa_block_cached__mha_block_cached__near_ridge_kernel(
    A_x: jax.Array,
    A_k_cache: jax.Array,
    A_v_cache: jax.Array,
    A_wq: jax.Array,
    A_wo: jax.Array,
    B_x: jax.Array,
    B_k_cache: jax.Array,
    B_v_cache: jax.Array,
    B_wq: jax.Array,
    B_wo: jax.Array,
):
    def kv(c):
        return jnp.swapaxes(c, 2, 3).reshape(B, H * DH, SK)

    def wo(w):
        return w.reshape(NG, GW // 128, 128, D)

    hbm = pl.BlockSpec(memory_space=pl.ANY)
    out = pl.pallas_call(
        _kernel,
        in_specs=[hbm] * 10,
        out_specs=hbm,
        out_shape=jax.ShapeDtypeStruct((B * SQ, 2 * D), bf16),
        scratch_shapes=[
            pltpu.VMEM((B * SQ, 2 * D), f32),
            pltpu.VMEM((B * SQ, 2 * D), bf16),
            pltpu.VMEM((2, 2, NB, SQ, D), bf16),
            pltpu.VMEM((2, B, XC_FORMS, HF // 2, 128), u32),
            pltpu.VMEM((NBG * 2 * NB, 6, HF, 128), u32),
            pltpu.VMEM((NS, 4, NB, GW, SK), bf16),
            pltpu.VMEM((NBG, 2, 5, SL, GW), bf16),
            pltpu.VMEM((NBG, 2, 6, SL, D), bf16),
            pltpu.VMEM((2, 2, NPR, 64, 128), u32),
            pltpu.VMEM((2, 2, NPR, 64, 128), u32),
            pltpu.VMEM((8, 128), u32),
            pltpu.SemaphoreType.DMA((NS,)),
            pltpu.SemaphoreType.DMA((NBG, 2)),
            pltpu.SemaphoreType.DMA((2,)),
            pltpu.SemaphoreType.DMA((1,)),
        ],
        compiler_params=pltpu.CompilerParams(vmem_limit_bytes=112 * 1024 * 1024, disable_bounds_checks=True),
    )(A_x, kv(A_k_cache), kv(A_v_cache), A_wq, wo(A_wo), B_x, kv(B_k_cache), kv(B_v_cache), B_wq, wo(B_wo))
    return out.reshape(B, SQ, 2 * D)
```

```python
import functools

import jax
import jax.numpy as jnp
from jax import lax
from jax.experimental import pallas as pl
from jax.experimental.pallas import tpu as pltpu

B, SQ, D, H, SK, DH = 16, 160, 640, 32, 512, 192
PW = 2 * DH
GW = 2 * PW
NG = H * DH // GW
NB = 2
NBG = B // NB
LG = NBG.bit_length() - 1
T = NG * NBG
SL = 128 // NBG
NS = 3
HF = SQ // 2
TT = 128
R = SQ - TT
QSCALE = (DH ** -0.5) * 1.4426950408889634
NT = (((1,), (1,)), ((), ()))
f32, bf16, u32 = jnp.float32, jnp.bfloat16, jnp.uint32

Q_FORMS = (
    ((0,0,1),(1,0,-1)), ((1,0,1),), ((0,1,1),), ((0,1,1),(1,1,-1)), ((0,3,1),), ((0,3,1),(1,3,-1)),
    ((0,1,1),(1,0,-1)), ((1,0,1),(1,1,-1)), ((0,0,1),(0,1,-1)), ((1,3,1),), ((0,4,1),), ((0,4,1),(1,4,-1)),
    ((0,1,1),(1,3,-1)), ((0,1,1),(0,3,-1)), ((1,1,1),(1,3,-1)), ((0,0,1),), ((1,1,1),), ((0,0,1),(1,3,-1)),
    ((0,0,1),(0,3,-1)), ((1,0,1),(1,3,-1)), ((0,2,1),), ((1,2,1),), ((1,4,1),), ((0,0,1),(1,4,-1)),
    ((0,0,1),(0,4,-1)), ((1,0,1),(1,4,-1)), ((0,1,1),(1,4,-1)), ((0,1,1),(0,4,-1)), ((1,1,1),(1,4,-1)),
    ((0,2,1),(1,2,-1)), ((0,1,1),(1,2,-1)), ((0,1,1),(0,2,-1)), ((1,1,1),(1,2,-1)), ((0,0,1),(1,2,-1)),
    ((0,0,1),(0,2,-1)), ((1,0,1),(1,2,-1)), ((0,4,1),(1,2,-1)), ((1,2,1),(1,4,-1)), ((0,2,1),(0,4,-1)),
    ((0,3,1),(1,2,-1)), ((1,2,1),(1,3,-1)), ((0,2,1),(0,3,-1)), ((0,3,1),(1,4,-1)), ((0,3,1),(0,4,-1)),
    ((1,3,1),(1,4,-1)),
)
Q_PRODS = (
    (0,((0,1,1),(0,2,-1)),((0,1,1),)), (1,((0,1,1),(1,1,1)),((0,1,1),(1,1,1))),
    (2,((0,2,1),(1,2,1),(2,2,1),(3,2,1),(4,2,1)),((0,2,1),(1,2,1))),
    (3,((1,1,1),(1,3,1),(1,4,1),(1,5,1),(1,2,-1)),((1,2,1),)), (4,((2,1,1),(3,1,1),(4,1,1)),((0,1,1),(1,1,1))),
    (5,((3,4,1),(3,5,1),(3,1,-1)),((1,1,1),)), (6,((0,2,1),(1,1,1)),((0,1,1),(1,2,-1))),
    (7,((1,1,1),),((1,1,-1),(1,2,-1))), (8,((0,2,1),),((0,1,1),(0,2,1))),
    (5,((3,0,1),(3,2,1),(3,3,-1)),((0,3,-1),)), (9,((0,3,1),(1,3,1),(3,3,1)),((0,3,1),(1,3,1))),
    (10,((2,3,1),(4,3,1)),((0,3,1),(1,3,1))), (11,((4,3,1),(4,5,-1)),((1,3,-1),)),
    (12,((1,3,1),(3,2,1)),((0,3,1),(1,2,-1))), (13,((3,2,1),),((0,2,-1),(0,3,-1))),
    (14,((1,3,1),),((1,2,1),(1,3,1))), (15,((0,0,1),(2,0,1),(3,0,1),(4,0,1)),((0,0,1),(1,0,1))),
    (0,((0,3,1),(0,4,1),(0,5,1),(0,0,-1)),((1,0,1),)), (2,((1,0,1),),((0,0,1),)), (16,((1,0,1),),((1,0,1),)),
    (17,((0,3,1),(3,0,1)),((0,3,1),(1,0,-1))), (18,((3,0,1),),((0,0,-1),(0,3,-1))),
    (19,((0,3,1),),((1,0,1),(1,3,1))), (20,((2,4,1),),((0,4,1),)), (21,((2,4,1),),((1,4,1),)),
    (11,((4,0,1),(4,1,1),(4,2,1),(4,4,-1)),((0,4,-1),)), (22,((0,4,1),(1,4,1),(3,4,1),(4,4,1)),((0,4,1),(1,4,1))),
    (23,((0,4,1),(4,0,1)),((0,4,1),(1,0,-1))), (24,((4,0,1),),((0,0,-1),(0,4,-1))),
    (25,((0,4,1),),((1,0,1),(1,4,1))), (26,((1,4,1),(4,2,1)),((0,4,1),(1,2,-1))),
    (27,((4,2,1),),((0,2,-1),(0,4,-1))), (28,((1,4,1),),((1,2,1),(1,4,1))),
    (29,((2,0,1),(2,1,1),(2,2,1),(2,3,1),(2,5,-1)),((0,5,-1),)),
    (21,((0,5,1),(1,5,1),(2,5,1),(3,5,1),(4,5,1)),((0,5,1),(1,5,1))), (30,((1,5,1),(2,2,1)),((0,5,1),(1,2,-1))),
    (31,((2,2,1),),((0,2,-1),(0,5,-1))), (32,((1,5,1),),((1,2,1),(1,5,1))),
    (33,((0,5,1),(2,0,1)),((0,5,1),(1,0,-1))), (34,((2,0,1),),((0,0,-1),(0,5,-1))),
    (35,((0,5,1),),((1,0,1),(1,5,1))), (36,((2,3,1),(4,5,1)),((0,5,1),(1,3,-1))),
    (37,((4,5,1),),((1,3,-1),(1,5,-1))), (38,((2,3,1),),((0,3,1),(0,5,1))),
    (39,((2,1,1),(3,5,1)),((0,5,1),(1,1,-1))), (40,((3,5,1),),((1,1,-1),(1,5,-1))),
    (41,((2,1,1),),((0,1,1),(0,5,1))), (42,((3,4,1),(4,1,1)),((0,4,1),(1,1,-1))),
    (43,((4,1,1),),((0,1,-1),(0,4,-1))), (44,((3,4,1),),((1,1,1),(1,4,1))),
)
O_FORMS = (
    ((0,0,1),), ((0,0,1),(1,0,-1)), ((0,1,1),(1,1,-1)), ((1,1,1),), ((1,0,1),), ((0,2,1),), ((0,2,1),(1,2,-1)),
    ((0,2,1),(1,1,-1)), ((1,1,1),(1,2,-1)), ((0,1,1),(0,2,-1)), ((0,1,1),), ((0,3,1),(1,3,-1)), ((1,3,1),),
    ((0,2,1),(1,3,-1)), ((0,2,1),(0,3,-1)), ((1,2,1),(1,3,-1)), ((0,0,1),(1,3,-1)), ((0,0,1),(0,3,-1)),
    ((1,0,1),(1,3,-1)), ((0,3,1),), ((0,4,1),(1,4,-1)), ((1,4,1),), ((0,0,1),(1,4,-1)), ((0,0,1),(0,4,-1)),
    ((1,0,1),(1,4,-1)), ((0,2,1),(1,4,-1)), ((0,2,1),(0,4,-1)), ((1,2,1),(1,4,-1)), ((0,4,1),), ((0,5,1),(1,5,-1)),
    ((1,5,1),), ((0,2,1),(1,5,-1)), ((0,2,1),(0,5,-1)), ((1,2,1),(1,5,-1)), ((0,0,1),(1,5,-1)), ((0,0,1),(0,5,-1)),
    ((1,0,1),(1,5,-1)), ((0,1,1),(1,5,-1)), ((1,1,1),(1,5,-1)), ((0,1,1),(0,5,-1)), ((0,1,1),(1,4,-1)),
    ((0,1,1),(0,4,-1)), ((1,1,1),(1,4,-1)), ((0,3,1),(1,5,-1)), ((1,3,1),(1,5,-1)), ((0,3,1),(0,5,-1)),
)
O_PRODS = (
    (0,((0,0,1),(3,0,1),(4,0,1),(5,0,1)),((0,0,1),(1,0,1))), (1,((0,2,1),(0,3,1),(0,4,1),(0,0,-1)),((1,0,1),)),
    (2,((1,0,1),(1,1,-1)),((0,0,1),)), (3,((1,0,1),(2,0,1)),((0,0,1),(1,0,1))), (0,((0,1,1),),((0,1,1),)),
    (4,((0,1,1),),((1,1,1),)), (5,((1,1,1),(2,1,1),(3,1,1),(4,1,1),(5,1,1)),((0,1,1),(1,1,1))),
    (6,((2,0,1),(2,2,1),(2,3,1),(2,4,1),(2,1,-1)),((1,1,1),)), (7,((1,1,1),(2,0,1)),((0,0,1),(1,1,-1))),
    (8,((2,0,1),),((1,0,-1),(1,1,-1))), (9,((1,1,1),),((0,0,1),(0,1,1))),
    (10,((1,3,1),(4,3,1),(5,3,1)),((0,3,1),(1,3,1))), (2,((1,2,1),(1,4,1),(1,3,-1)),((1,3,1),)),
    (11,((3,0,1),(3,1,1),(3,3,-1)),((0,3,-1),)), (12,((0,3,1),(2,3,1),(3,3,1)),((0,3,1),(1,3,1))),
    (13,((2,3,1),(3,1,1)),((0,3,1),(1,1,-1))), (14,((3,1,1),),((0,1,-1),(0,3,-1))),
    (15,((2,3,1),),((1,1,1),(1,3,1))), (16,((0,3,1),(3,0,1)),((0,3,1),(1,0,-1))),
    (17,((3,0,1),),((0,0,-1),(0,3,-1))), (18,((0,3,1),),((1,0,1),(1,3,1))),
    (19,((3,4,1),(5,4,1)),((0,4,1),(1,4,1))), (11,((3,4,1),(3,2,-1)),((1,4,-1),)),
    (20,((4,0,1),(4,1,1),(4,3,1),(4,4,-1)),((0,4,-1),)), (21,((0,4,1),(1,4,1),(2,4,1),(4,4,1)),((0,4,1),(1,4,1))),
    (22,((0,4,1),(4,0,1)),((0,4,1),(1,0,-1))), (23,((4,0,1),),((0,0,-1),(0,4,-1))),
    (24,((0,4,1),),((1,0,1),(1,4,1))), (25,((2,4,1),(4,1,1)),((0,4,1),(1,1,-1))),
    (26,((4,1,1),),((0,1,-1),(0,4,-1))), (27,((2,4,1),),((1,1,1),(1,4,1))), (28,((4,2,1),),((0,2,1),)),
    (21,((4,2,1),),((1,2,1),)), (29,((5,0,1),(5,1,1),(5,3,1),(5,4,1),(5,2,-1)),((0,2,-1),)),
    (30,((0,2,1),(1,2,1),(2,2,1),(3,2,1),(5,2,1)),((0,2,1),(1,2,1))), (31,((2,2,1),(5,1,1)),((0,2,1),(1,1,-1))),
    (32,((5,1,1),),((0,1,-1),(0,2,-1))), (33,((2,2,1),),((1,1,1),(1,2,1))),
    (34,((0,2,1),(5,0,1)),((0,2,1),(1,0,-1))), (35,((5,0,1),),((0,0,-1),(0,2,-1))),
    (36,((0,2,1),),((1,0,1),(1,2,1))), (37,((1,2,1),(5,3,1)),((0,2,1),(1,3,-1))), (38,((1,2,1),),((1,2,1),(1,3,1))),
    (39,((5,3,1),),((0,2,-1),(0,3,-1))), (40,((1,4,1),(4,3,1)),((0,4,1),(1,3,-1))),
    (41,((4,3,1),),((0,3,-1),(0,4,-1))), (42,((1,4,1),),((1,3,1),(1,4,1))),
    (43,((3,2,1),(5,4,1)),((0,2,1),(1,4,-1))), (44,((3,2,1),),((1,2,1),(1,4,1))),
    (45,((5,4,1),),((0,2,-1),(0,4,-1))),
)
NPR = len(Q_PRODS)
XC_FORMS = len(Q_FORMS) + 1
XC_ZERO = B + NB

ODD = ("K0", "K1", "P0", "P1", "Q0", "Q1", "Q2", "Q3", "Q4")
EVEN = ("K0", "K1", "P0", "P1", "O0", "O1", "O2")
SOFTMAX_LAG = 4


def _dot(a, b):
    return jnp.dot(a, b, preferred_element_type=f32)


def _dot_nt(a, b):
    return lax.dot_general(a, b, NT, preferred_element_type=f32)


def _unpk(v):
    return pltpu.bitcast(v, bf16)


def _tile(c):
    return slice(c * 128, (c + 1) * 128)


def _split(nparts, total=NPR):
    return [list(range(k * total // nparts, (k + 1) * total // nparts)) for k in range(nparts)]


def _lincomb(terms, get):
    v = get(terms[0][:-1])
    for t in terms[1:]:
        v = v + get(t[:-1]) if t[-1] > 0 else v - get(t[:-1])
    return v


def _packed_combos(term_lists, load, link=None):
    wide = {}

    def get(k):
        if k not in wide:
            v = load(*k)
            if link is not None and not wide:
                v = pltpu.bitcast(pltpu.bitcast(v, u32) | link, bf16)
            wide[k] = v.astype(f32)
        return wide[k]

    out = {n: pltpu.bitcast(load(*t[0][:-1]), u32) for n, t in enumerate(term_lists) if len(t) == 1}
    sums = [n for n in range(len(term_lists)) if n not in out]
    for pair in (sums[n:n + 2] for n in range(0, len(sums), 2)):
        v = jnp.concatenate([_lincomb(term_lists[n], get) for n in pair], axis=1)
        v = pltpu.bitcast(v.astype(bf16), u32)
        for c, n in enumerate(pair):
            out[n] = v[:, _tile(c)]
    return [out[n] for n in range(len(term_lists))]


def _bilinear(prods, rs, prod, c, init, done):
    last = {(s, j): r for r, p in enumerate(prods) for (s, j, _) in p[2]}
    for r in rs:
        m = prod(r)
        for (s, j, sg) in prods[r][2]:
            if (s, j) not in c and init is not None:
                c[(s, j)] = init(s, j)
            if (s, j) in c:
                c[(s, j)] = c[(s, j)] + m if sg > 0 else c[(s, j)] - m
            else:
                c[(s, j)] = m if sg > 0 else -m
            if last[(s, j)] == r:
                done(s, j, c[(s, j)])


def _recip(l):
    r = pl.reciprocal(l, approx=True)
    return r * (2.0 - l * r)


def _softmax(s, zero):
    ps = []
    for r in range(SQ // 8):
        sb = s[r * 8:(r + 1) * 8]
        m = jnp.broadcast_to(jnp.max(sb, axis=-1, keepdims=True), (8, 128))
        if r >= SOFTMAX_LAG:
            link = pltpu.bitcast(ps[r - SOFTMAX_LAG][:, 384:512], u32) & zero
            m = pltpu.bitcast(pltpu.bitcast(m, u32) | link, f32)
        ps.append(jnp.exp2(sb - jnp.concatenate([m] * 4, axis=1)))
    p = jnp.concatenate(ps, axis=0)
    t = (p[:, 0:128] + p[:, 128:256]) + (p[:, 256:384] + p[:, 384:512])
    r_row = _recip(jnp.sum(t[:TT].T, axis=0, keepdims=True))
    r_col = jnp.broadcast_to(_recip(jnp.sum(t[TT:], axis=-1, keepdims=True)), (R, 128))
    return p, r_row, r_col


def _kernel(xa, kta, vta, wqa, woa, xb, ktb, vtb, wqb, wob, o_hbm,
            acc, obuf, xraw, xc, qbuf, kvbuf, wqraw, woraw, wqc, woc, zv, zs,
            kvsem, wsem, xsem, osem):
    xs, kvs, wqs, wos = (xa, xb), (kta, vta, ktb, vtb), (wqa, wqb), (woa, wob)

    def ring(slot, k):
        v = slot + k
        return jnp.where(v >= NS, v - NS, v)

    def kv_start(sl, t):
        hg, g = lax.shift_right_logical(t, LG) - 1, t & (NBG - 1)
        for a in range(4):
            pltpu.make_async_copy(kvs[a].at[pl.ds(g * NB, NB), pl.ds(pl.multiple_of(hg * GW, GW), GW), :],
                                  kvbuf.at[sl, a], kvsem.at[sl]).start()

    def kv_piece(k):
        a, b = k // NB, k % NB
        pltpu.make_async_copy(kvs[a].at[b, pl.ds(0, GW), :], kvbuf.at[0, a, b], kvsem.at[0]).start()

    def wq_start(hg, sl):
        cols = pl.ds(pl.multiple_of(hg * GW, GW), GW)
        for p in range(2):
            for kt in range(5):
                pltpu.make_async_copy(wqs[p].at[pl.ds(pl.multiple_of(kt * 128 + sl * SL, SL), SL), cols],
                                      wqraw.at[sl, p, kt], wsem.at[sl, 0]).start()

    def wo_start(hg, sl):
        for p in range(2):
            pltpu.make_async_copy(wos[p].at[hg, :, pl.ds(pl.multiple_of(sl * SL, SL), SL), :],
                                  woraw.at[sl, p], wsem.at[sl, 1]).start()

    def x_start(g):
        for p in range(2):
            pltpu.make_async_copy(xs[p].at[pl.ds(g * NB, NB)], xraw.at[g & 1, p], xsem.at[g & 1]).start()

    def wait_filled(v, sem):
        pltpu.make_async_copy(v, v, sem).wait()

    def w_piece(raw, dst, prods, ws, sl, p, rs):
        rows = pl.ds(pl.multiple_of(sl * (SL // 2), 8), SL // 2)
        vs = _packed_combos([prods[r][1] for r in rs], lambda i, j: raw[sl, p, i, :, _tile(j)])
        for r, v in zip(rs, vs):
            dst[ws, p, r, rows, :] = v

    wq_piece = functools.partial(w_piece, wqraw, wqc, Q_PRODS)
    wo_piece = functools.partial(w_piece, woraw, woc, O_PRODS)
    w_pieces = [(p, rs) for p in range(2) for rs in _split(5)]

    def x_piece(g, row, link, p, b, ks, r0):
        vs = _packed_combos([Q_FORMS[k] for k in ks],
                            lambda s, i: xraw[g & 1, p, b, s * HF + r0:s * HF + r0 + 16, _tile(i)], link())
        for k, v in zip(ks, vs):
            xc[p, row(b), k, r0 // 2:r0 // 2 + 8, :] = v

    x_pieces = [(p, b, ks, r0) for p in range(2) for b in range(NB) for r0 in range(0, HF, 16)
                for ks in _split(5, len(Q_FORMS))]

    units = [(p, b) for p in range(2) for b in range(NB)]
    nu = len(units)

    def step(mode, t, slot):
        g = t & (NBG - 1)
        hq = lax.shift_right_logical(t, LG)
        qslot = hq & 1
        oslot = 1 - qslot
        gb = g * NB

        def prefetch():
            t2 = t + 2
            if mode == "start":
                for k in range(1, NBG):
                    pl.when(g + 1 == k)(functools.partial(kv_piece, k))
            else:
                pl.when(t2 < T + NBG)(functools.partial(kv_start, ring(slot, 2), t2))
            if mode != "last":
                h2, g2 = lax.shift_right_logical(t2, LG), t2 & (NBG - 1)
                pl.when(h2 + 1 < NG)(functools.partial(wq_start, h2 + 1, g2))
                pl.when(h2 < NG)(functools.partial(wo_start, h2, g2))

        if mode == "start":
            pl.when(g + 2 < NBG)(functools.partial(x_start, g + 2))
            pl.when(g + 1 < NBG)(functools.partial(wait_filled, xraw.at[(g + 1) & 1], xsem.at[(g + 1) & 1]))
        if mode != "last":
            pl.when(hq + 1 < NG)(functools.partial(wait_filled, wqraw.at[g], wsem.at[g, 0]))
            wait_filled(woraw.at[g], wsem.at[g, 1])
        if mode != "start":
            wait_filled(kvbuf.at[slot], kvsem.at[slot])

        st = [dict() for _ in range(2 * nu)]
        zero = zv[...]
        jq = [functools.partial(wq_piece, 1 - qslot, g, *a) for a in w_pieces]
        jo = [functools.partial(wo_piece, 1 - oslot, g, *a) for a in w_pieces]

        def x_link():
            link = xc[0, zs[0] + XC_ZERO, 0, 0:8, :]
            for _ in range(4):
                link = (link + zero) & zero
            return link

        jx = [functools.partial(x_piece, g + 1, lambda b: gb + (NB + b), x_link, *a) for a in x_pieces]
        todo = {"start": (jq + jo, [], jx), "last": ([], [], [])}.get(mode, (jq, jo, []))
        every = (5, 4, 2)
        count = [0, 0, 0]

        def side_job(kind):
            count[kind] += 1
            if count[kind] % every[kind] == 0 and todo[kind]:
                todo[kind].pop(0)()

        def task_q(u, j):
            p, b = units[u]

            def prod(r):
                side_job(0)
                side_job(2)
                return _dot(_unpk(xc[p, gb + b, Q_PRODS[r][0]]), _unpk(wqc[qslot, p, r]))

            def done(s, col, v):
                qbuf[g * nu + u, col, s * HF // 2:(s + 1) * HF // 2, :] = pltpu.bitcast((v * QSCALE).astype(bf16), u32)

            _bilinear(Q_PRODS, _split(5)[j], prod, st[2 * u].setdefault("qc", {}), None, done)

        def task_k(i, h):
            p, b = units[i // 2]
            k0 = (i % 2) * PW + h * 128
            kt = kvbuf.at[slot, 2 * p, b]
            lane = lax.broadcasted_iota(jnp.int32, (HF, 128), 1)
            q = [qbuf[g * nu + i // 2, 3 * (i % 2) + h + c] for c in range(2)]
            q[1 - h] = jnp.where((lane < 64) if h == 0 else (lane >= 64), q[1 - h], jnp.uint32(0))
            q = _unpk(jnp.concatenate(q, axis=1))
            s = jnp.concatenate([_dot(q, kt[k0:k0 + 256, c:c + 256]) for c in (0, 256)], axis=1)
            st[i][h] = _softmax(s, zero)

        def task_p(i, h):
            p, b = units[i // 2]
            k0 = (i % 2) * PW
            vt = kvbuf.at[slot, 2 * p + 1, b]
            d = st[i]
            if h == 0:
                d["ot"] = _dot_nt(vt[k0:k0 + 192, :], d[0][0][:TT].astype(bf16))
                d["oa"] = _dot_nt(d[0][0][TT:].astype(bf16), vt[k0:k0 + 128, :])
                return
            (p1, row1, col1), (p2, row2, col2) = d[0], d[1]
            om = _dot_nt(jnp.concatenate([p1[TT:], p2[TT:]], axis=0).astype(bf16), vt[k0 + 128:k0 + 256, :])
            ot2 = _dot_nt(vt[k0 + 192:k0 + 384, :], p2[:TT].astype(bf16))
            oc = _dot_nt(p2[TT:].astype(bf16), vt[k0 + 256:k0 + 384, :])
            ot1 = d["ot"] * row1
            ot2 = ot2 * row2
            lane = lax.broadcasted_iota(jnp.int32, (R, 128), 1)
            om = jnp.where(lane < 64, om[:R] * col1, om[R:] * col2)
            ta = ot1[0:128].T
            tm = jnp.concatenate([ot1[128:192], ot2[0:64]], axis=0).T
            tc = ot2[64:192].T
            d["o"] = [jnp.concatenate([ta, d["oa"] * col1], axis=0),
                      jnp.concatenate([tm, om], axis=0),
                      jnp.concatenate([tc, oc * col2], axis=0)]

        def task_o(u, j):
            p, b = units[u]
            d = st[2 * u]
            o = st[2 * u]["o"] + st[2 * u + 1]["o"]
            row0 = (g * NB + b) * SQ

            def idx(s, col):
                return pl.ds(pl.multiple_of(row0 + s * HF, 16), HF), _tile(p * 5 + col)

            def done(s, col, v):
                if mode == "last":
                    obuf[idx(s, col)] = v.astype(bf16)
                else:
                    acc[idx(s, col)] = v

            def prod(r):
                side_job(1)
                f = O_PRODS[r][0]
                if ("form", f) not in d:
                    d["form", f] = _lincomb(O_FORMS[f], lambda k: o[k[1]][k[0] * HF:(k[0] + 1) * HF]).astype(bf16)
                return _dot(d["form", f], _unpk(woc[oslot, p, r]))

            init = None if mode == "first" else (lambda s, col: acc[idx(s, col)])
            _bilinear(O_PRODS, _split(3)[j], prod, d.setdefault("oc", {}), init, done)
            if mode == "last" and j == 2:
                win = (pl.ds(pl.multiple_of(row0, 16), SQ), pl.ds(p * D, D))
                pltpu.make_async_copy(obuf.at[win], o_hbm.at[win], osem.at[0]).start()

        if mode == "start":
            seq = [("Q", u, j) for u in range(nu) for j in range(5)]
        else:
            seq = []
            for s in range(-1, 2 * nu + 1):
                for kind, j in (ODD if s % 2 else EVEN):
                    i = {"Q": (s - 1) // 2, "O": s // 2 - 1, "K": s + 1, "P": s}[kind]
                    if 0 <= i < (nu if kind in "QO" else 2 * nu) and (kind != "Q" or mode != "last"):
                        seq.append((kind, i, int(j)))
            late = [x for x in seq if x[:2] == ("O", nu - 2)][{"last": 2, "first": 1, "mid": 0}[mode]:]
            seq = [x for x in seq if x not in late]
            pos = seq.index(("P", 2 * nu - 1, 1)) + 1
            seq[pos:pos] = late
        tasks = {"Q": task_q, "K": task_k, "P": task_p, "O": task_o}
        for n, (kind, i, j) in enumerate(seq):
            if n == 1:
                prefetch()
            tasks[kind](i, j)
        for jobs in todo:
            for job in jobs:
                job()

    def loop(lo, hi, fn):
        def body(i, c):
            fn(i)
            return c
        lax.fori_loop(lo, hi, body, 0)

    def steps(mode, lo, hi, slot0):
        def body(t, slot):
            step(mode, t, slot)
            return ring(slot, 1)
        return lax.fori_loop(lo, hi, body, slot0)

    def first_wq(sl):
        wait_filled(wqraw.at[sl], wsem.at[sl, 0])
        for a in w_pieces:
            wq_piece(0, sl, *a)

        @pl.when(sl < 2)
        def _():
            wq_start(1, sl)
            wo_start(0, sl)

    zv[...] = jnp.zeros((8, 128), u32)
    zs[0] = 0
    xc[0, XC_ZERO, 0] = jnp.zeros((HF // 2, 128), u32)
    loop(0, 1, x_start)
    loop(0, NBG, functools.partial(wq_start, 0))
    x_start(1)
    wait_filled(xraw.at[0], xsem.at[0])
    for a in x_pieces:
        x_piece(0, lambda b: b, lambda: None, *a)
    loop(0, NBG, first_wq)
    kv_piece(0)
    steps("start", 0, NBG, jnp.int32(0))
    kv_start(1, NBG + 1)
    slot = steps("first", NBG, 2 * NBG, jnp.int32(0))
    slot = steps("mid", 2 * NBG, T, slot)
    steps("last", T, T + NBG, slot)
    pltpu.make_async_copy(obuf, o_hbm, osem.at[0]).wait()


@jax.jit
def pallas_concat_heads__gqa_block_cached__mha_block_cached__near_ridge_kernel(
    A_x: jax.Array,
    A_k_cache: jax.Array,
    A_v_cache: jax.Array,
    A_wq: jax.Array,
    A_wo: jax.Array,
    B_x: jax.Array,
    B_k_cache: jax.Array,
    B_v_cache: jax.Array,
    B_wq: jax.Array,
    B_wo: jax.Array,
):
    def kv(c):
        return jnp.swapaxes(c, 2, 3).reshape(B, H * DH, SK)

    def wo(w):
        return w.reshape(NG, GW // 128, 128, D)

    hbm = pl.BlockSpec(memory_space=pl.ANY)
    out = pl.pallas_call(
        _kernel,
        in_specs=[hbm] * 10,
        out_specs=hbm,
        out_shape=jax.ShapeDtypeStruct((B * SQ, 2 * D), bf16),
        scratch_shapes=[
            pltpu.VMEM((B * SQ, 2 * D), f32),
            pltpu.VMEM((B * SQ, 2 * D), bf16),
            pltpu.VMEM((2, 2, NB, SQ, D), bf16),
            pltpu.VMEM((2, B + 2 * NB, XC_FORMS, HF // 2, 128), u32),
            pltpu.VMEM((NBG * 2 * NB, 6, HF, 128), u32),
            pltpu.VMEM((NS, 4, NB, GW, SK), bf16),
            pltpu.VMEM((NBG, 2, 5, SL, GW), bf16),
            pltpu.VMEM((NBG, 2, 6, SL, D), bf16),
            pltpu.VMEM((2, 2, NPR, 64, 128), u32),
            pltpu.VMEM((2, 2, NPR, 64, 128), u32),
            pltpu.VMEM((8, 128), u32),
            pltpu.SMEM((1,), jnp.int32),
            pltpu.SemaphoreType.DMA((NS,)),
            pltpu.SemaphoreType.DMA((NBG, 2)),
            pltpu.SemaphoreType.DMA((2,)),
            pltpu.SemaphoreType.DMA((1,)),
        ],
        compiler_params=pltpu.CompilerParams(vmem_limit_bytes=112 * 1024 * 1024, disable_bounds_checks=True),
    )(A_x, kv(A_k_cache), kv(A_v_cache), A_wq, wo(A_wo), B_x, kv(B_k_cache), kv(B_v_cache), B_wq, wo(B_wo))
    return out.reshape(B, SQ, 2 * D)
```

```python
import functools

import jax
import jax.numpy as jnp
from jax import lax
from jax.experimental import pallas as pl
from jax.experimental.pallas import tpu as pltpu

B, SQ, D, H, SK, DH = 16, 160, 640, 32, 512, 192
PW = 2 * DH
GW = 2 * PW
NG = H * DH // GW
NB = 2
NBG = B // NB
LG = NBG.bit_length() - 1
T = NG * NBG
SL = 128 // NBG
NS = 3
HF = SQ // 2
TT = 128
R = SQ - TT
QSCALE = (DH ** -0.5) * 1.4426950408889634
NT = (((1,), (1,)), ((), ()))
f32, bf16, u32 = jnp.float32, jnp.bfloat16, jnp.uint32

Q_FORMS = (
    ((0,0,1),(1,0,-1)), ((1,0,1),), ((0,1,1),), ((0,1,1),(1,1,-1)), ((0,3,1),), ((0,3,1),(1,3,-1)),
    ((0,1,1),(1,0,-1)), ((1,0,1),(1,1,-1)), ((0,0,1),(0,1,-1)), ((1,3,1),), ((0,4,1),), ((0,4,1),(1,4,-1)),
    ((0,1,1),(1,3,-1)), ((0,1,1),(0,3,-1)), ((1,1,1),(1,3,-1)), ((0,0,1),), ((1,1,1),), ((0,0,1),(1,3,-1)),
    ((0,0,1),(0,3,-1)), ((1,0,1),(1,3,-1)), ((0,2,1),), ((1,2,1),), ((1,4,1),), ((0,0,1),(1,4,-1)),
    ((0,0,1),(0,4,-1)), ((1,0,1),(1,4,-1)), ((0,1,1),(1,4,-1)), ((0,1,1),(0,4,-1)), ((1,1,1),(1,4,-1)),
    ((0,2,1),(1,2,-1)), ((0,1,1),(1,2,-1)), ((0,1,1),(0,2,-1)), ((1,1,1),(1,2,-1)), ((0,0,1),(1,2,-1)),
    ((0,0,1),(0,2,-1)), ((1,0,1),(1,2,-1)), ((0,4,1),(1,2,-1)), ((1,2,1),(1,4,-1)), ((0,2,1),(0,4,-1)),
    ((0,3,1),(1,2,-1)), ((1,2,1),(1,3,-1)), ((0,2,1),(0,3,-1)), ((0,3,1),(1,4,-1)), ((0,3,1),(0,4,-1)),
    ((1,3,1),(1,4,-1)),
)
Q_PRODS = (
    (0,((0,1,1),(0,2,-1)),((0,1,1),)), (1,((0,1,1),(1,1,1)),((0,1,1),(1,1,1))),
    (2,((0,2,1),(1,2,1),(2,2,1),(3,2,1),(4,2,1)),((0,2,1),(1,2,1))),
    (3,((1,1,1),(1,3,1),(1,4,1),(1,5,1),(1,2,-1)),((1,2,1),)), (4,((2,1,1),(3,1,1),(4,1,1)),((0,1,1),(1,1,1))),
    (5,((3,4,1),(3,5,1),(3,1,-1)),((1,1,1),)), (6,((0,2,1),(1,1,1)),((0,1,1),(1,2,-1))),
    (7,((1,1,1),),((1,1,-1),(1,2,-1))), (8,((0,2,1),),((0,1,1),(0,2,1))),
    (5,((3,0,1),(3,2,1),(3,3,-1)),((0,3,-1),)), (9,((0,3,1),(1,3,1),(3,3,1)),((0,3,1),(1,3,1))),
    (10,((2,3,1),(4,3,1)),((0,3,1),(1,3,1))), (11,((4,3,1),(4,5,-1)),((1,3,-1),)),
    (12,((1,3,1),(3,2,1)),((0,3,1),(1,2,-1))), (13,((3,2,1),),((0,2,-1),(0,3,-1))),
    (14,((1,3,1),),((1,2,1),(1,3,1))), (15,((0,0,1),(2,0,1),(3,0,1),(4,0,1)),((0,0,1),(1,0,1))),
    (0,((0,3,1),(0,4,1),(0,5,1),(0,0,-1)),((1,0,1),)), (2,((1,0,1),),((0,0,1),)), (16,((1,0,1),),((1,0,1),)),
    (17,((0,3,1),(3,0,1)),((0,3,1),(1,0,-1))), (18,((3,0,1),),((0,0,-1),(0,3,-1))),
    (19,((0,3,1),),((1,0,1),(1,3,1))), (20,((2,4,1),),((0,4,1),)), (21,((2,4,1),),((1,4,1),)),
    (11,((4,0,1),(4,1,1),(4,2,1),(4,4,-1)),((0,4,-1),)), (22,((0,4,1),(1,4,1),(3,4,1),(4,4,1)),((0,4,1),(1,4,1))),
    (23,((0,4,1),(4,0,1)),((0,4,1),(1,0,-1))), (24,((4,0,1),),((0,0,-1),(0,4,-1))),
    (25,((0,4,1),),((1,0,1),(1,4,1))), (26,((1,4,1),(4,2,1)),((0,4,1),(1,2,-1))),
    (27,((4,2,1),),((0,2,-1),(0,4,-1))), (28,((1,4,1),),((1,2,1),(1,4,1))),
    (29,((2,0,1),(2,1,1),(2,2,1),(2,3,1),(2,5,-1)),((0,5,-1),)),
    (21,((0,5,1),(1,5,1),(2,5,1),(3,5,1),(4,5,1)),((0,5,1),(1,5,1))), (30,((1,5,1),(2,2,1)),((0,5,1),(1,2,-1))),
    (31,((2,2,1),),((0,2,-1),(0,5,-1))), (32,((1,5,1),),((1,2,1),(1,5,1))),
    (33,((0,5,1),(2,0,1)),((0,5,1),(1,0,-1))), (34,((2,0,1),),((0,0,-1),(0,5,-1))),
    (35,((0,5,1),),((1,0,1),(1,5,1))), (36,((2,3,1),(4,5,1)),((0,5,1),(1,3,-1))),
    (37,((4,5,1),),((1,3,-1),(1,5,-1))), (38,((2,3,1),),((0,3,1),(0,5,1))),
    (39,((2,1,1),(3,5,1)),((0,5,1),(1,1,-1))), (40,((3,5,1),),((1,1,-1),(1,5,-1))),
    (41,((2,1,1),),((0,1,1),(0,5,1))), (42,((3,4,1),(4,1,1)),((0,4,1),(1,1,-1))),
    (43,((4,1,1),),((0,1,-1),(0,4,-1))), (44,((3,4,1),),((1,1,1),(1,4,1))),
)
O_FORMS = (
    ((0,0,1),), ((0,0,1),(1,0,-1)), ((0,1,1),(1,1,-1)), ((1,1,1),), ((1,0,1),), ((0,2,1),), ((0,2,1),(1,2,-1)),
    ((0,2,1),(1,1,-1)), ((1,1,1),(1,2,-1)), ((0,1,1),(0,2,-1)), ((0,1,1),), ((0,3,1),(1,3,-1)), ((1,3,1),),
    ((0,2,1),(1,3,-1)), ((0,2,1),(0,3,-1)), ((1,2,1),(1,3,-1)), ((0,0,1),(1,3,-1)), ((0,0,1),(0,3,-1)),
    ((1,0,1),(1,3,-1)), ((0,3,1),), ((0,4,1),(1,4,-1)), ((1,4,1),), ((0,0,1),(1,4,-1)), ((0,0,1),(0,4,-1)),
    ((1,0,1),(1,4,-1)), ((0,2,1),(1,4,-1)), ((0,2,1),(0,4,-1)), ((1,2,1),(1,4,-1)), ((0,4,1),), ((0,5,1),(1,5,-1)),
    ((1,5,1),), ((0,2,1),(1,5,-1)), ((0,2,1),(0,5,-1)), ((1,2,1),(1,5,-1)), ((0,0,1),(1,5,-1)), ((0,0,1),(0,5,-1)),
    ((1,0,1),(1,5,-1)), ((0,1,1),(1,5,-1)), ((1,1,1),(1,5,-1)), ((0,1,1),(0,5,-1)), ((0,1,1),(1,4,-1)),
    ((0,1,1),(0,4,-1)), ((1,1,1),(1,4,-1)), ((0,3,1),(1,5,-1)), ((1,3,1),(1,5,-1)), ((0,3,1),(0,5,-1)),
)
O_PRODS = (
    (0,((0,0,1),(3,0,1),(4,0,1),(5,0,1)),((0,0,1),(1,0,1))), (1,((0,2,1),(0,3,1),(0,4,1),(0,0,-1)),((1,0,1),)),
    (2,((1,0,1),(1,1,-1)),((0,0,1),)), (3,((1,0,1),(2,0,1)),((0,0,1),(1,0,1))), (0,((0,1,1),),((0,1,1),)),
    (4,((0,1,1),),((1,1,1),)), (5,((1,1,1),(2,1,1),(3,1,1),(4,1,1),(5,1,1)),((0,1,1),(1,1,1))),
    (6,((2,0,1),(2,2,1),(2,3,1),(2,4,1),(2,1,-1)),((1,1,1),)), (7,((1,1,1),(2,0,1)),((0,0,1),(1,1,-1))),
    (8,((2,0,1),),((1,0,-1),(1,1,-1))), (9,((1,1,1),),((0,0,1),(0,1,1))),
    (10,((1,3,1),(4,3,1),(5,3,1)),((0,3,1),(1,3,1))), (2,((1,2,1),(1,4,1),(1,3,-1)),((1,3,1),)),
    (11,((3,0,1),(3,1,1),(3,3,-1)),((0,3,-1),)), (12,((0,3,1),(2,3,1),(3,3,1)),((0,3,1),(1,3,1))),
    (13,((2,3,1),(3,1,1)),((0,3,1),(1,1,-1))), (14,((3,1,1),),((0,1,-1),(0,3,-1))),
    (15,((2,3,1),),((1,1,1),(1,3,1))), (16,((0,3,1),(3,0,1)),((0,3,1),(1,0,-1))),
    (17,((3,0,1),),((0,0,-1),(0,3,-1))), (18,((0,3,1),),((1,0,1),(1,3,1))),
    (19,((3,4,1),(5,4,1)),((0,4,1),(1,4,1))), (11,((3,4,1),(3,2,-1)),((1,4,-1),)),
    (20,((4,0,1),(4,1,1),(4,3,1),(4,4,-1)),((0,4,-1),)), (21,((0,4,1),(1,4,1),(2,4,1),(4,4,1)),((0,4,1),(1,4,1))),
    (22,((0,4,1),(4,0,1)),((0,4,1),(1,0,-1))), (23,((4,0,1),),((0,0,-1),(0,4,-1))),
    (24,((0,4,1),),((1,0,1),(1,4,1))), (25,((2,4,1),(4,1,1)),((0,4,1),(1,1,-1))),
    (26,((4,1,1),),((0,1,-1),(0,4,-1))), (27,((2,4,1),),((1,1,1),(1,4,1))), (28,((4,2,1),),((0,2,1),)),
    (21,((4,2,1),),((1,2,1),)), (29,((5,0,1),(5,1,1),(5,3,1),(5,4,1),(5,2,-1)),((0,2,-1),)),
    (30,((0,2,1),(1,2,1),(2,2,1),(3,2,1),(5,2,1)),((0,2,1),(1,2,1))), (31,((2,2,1),(5,1,1)),((0,2,1),(1,1,-1))),
    (32,((5,1,1),),((0,1,-1),(0,2,-1))), (33,((2,2,1),),((1,1,1),(1,2,1))),
    (34,((0,2,1),(5,0,1)),((0,2,1),(1,0,-1))), (35,((5,0,1),),((0,0,-1),(0,2,-1))),
    (36,((0,2,1),),((1,0,1),(1,2,1))), (37,((1,2,1),(5,3,1)),((0,2,1),(1,3,-1))), (38,((1,2,1),),((1,2,1),(1,3,1))),
    (39,((5,3,1),),((0,2,-1),(0,3,-1))), (40,((1,4,1),(4,3,1)),((0,4,1),(1,3,-1))),
    (41,((4,3,1),),((0,3,-1),(0,4,-1))), (42,((1,4,1),),((1,3,1),(1,4,1))),
    (43,((3,2,1),(5,4,1)),((0,2,1),(1,4,-1))), (44,((3,2,1),),((1,2,1),(1,4,1))),
    (45,((5,4,1),),((0,2,-1),(0,4,-1))),
)
NPR = len(Q_PRODS)
XC_FORMS = len(Q_FORMS) + 1
XC_ZERO = B + NB


def _dot(a, b):
    return jnp.dot(a, b, preferred_element_type=f32)


def _dot_nt(a, b):
    return lax.dot_general(a, b, NT, preferred_element_type=f32)


def _unpk(v):
    return pltpu.bitcast(v, bf16)


def _tile(c):
    return slice(c * 128, (c + 1) * 128)


def _split(nparts, total=NPR):
    return [list(range(k * total // nparts, (k + 1) * total // nparts)) for k in range(nparts)]


def _lincomb(terms, get):
    v = get(terms[0][:-1])
    for t in terms[1:]:
        v = v + get(t[:-1]) if t[-1] > 0 else v - get(t[:-1])
    return v


def _packed_combos(term_lists, load, link=None):
    wide = {}

    def get(k):
        if k not in wide:
            v = load(*k)
            if link is not None and not wide:
                v = pltpu.bitcast(pltpu.bitcast(v, u32) | link, bf16)
            wide[k] = v.astype(f32)
        return wide[k]

    out = {n: pltpu.bitcast(load(*t[0][:-1]), u32) for n, t in enumerate(term_lists) if len(t) == 1}
    sums = [n for n in range(len(term_lists)) if n not in out]
    for pair in (sums[n:n + 2] for n in range(0, len(sums), 2)):
        v = jnp.concatenate([_lincomb(term_lists[n], get) for n in pair], axis=1)
        v = pltpu.bitcast(v.astype(bf16), u32)
        for c, n in enumerate(pair):
            out[n] = v[:, _tile(c)]
    return [out[n] for n in range(len(term_lists))]


def _bilinear(prods, rs, prod, c, init, done):
    last = {(s, j): r for r, p in enumerate(prods) for (s, j, _) in p[2]}
    for r in rs:
        m = prod(r)
        for (s, j, sg) in prods[r][2]:
            if (s, j) not in c and init is not None:
                c[(s, j)] = init(s, j)
            if (s, j) in c:
                c[(s, j)] = c[(s, j)] + m if sg > 0 else c[(s, j)] - m
            else:
                c[(s, j)] = m if sg > 0 else -m
            if last[(s, j)] == r:
                done(s, j, c[(s, j)])


def _recip(l):
    r = pl.reciprocal(l, approx=True)
    return r * (2.0 - l * r)


def _softmax(s, zero, lag):
    ps = []
    for r in range(SQ // 8):
        sb = s[r * 8:(r + 1) * 8]
        m = jnp.broadcast_to(jnp.max(sb, axis=-1, keepdims=True), (8, 128))
        if r >= lag:
            link = pltpu.bitcast(ps[r - lag][:, 384:512], u32) & zero
            m = pltpu.bitcast(pltpu.bitcast(m, u32) | link, f32)
        ps.append(jnp.exp2(sb - jnp.concatenate([m] * 4, axis=1)))
    p = jnp.concatenate(ps, axis=0)
    t = (p[:, 0:128] + p[:, 128:256]) + (p[:, 256:384] + p[:, 384:512])
    r_row = _recip(jnp.sum(t[:TT].T, axis=0, keepdims=True))
    r_col = jnp.broadcast_to(_recip(jnp.sum(t[TT:], axis=-1, keepdims=True)), (R, 128))
    return p, r_row, r_col


def _schedule(mode, nu):
    if mode == "start":
        return [("Q", u, rs) for u in range(nu) for rs in _split(5)]
    order = []
    for s in range(-1, 2 * nu + 1):
        order += [("K", s + 1, h) for h in range(2) if s + 1 < 2 * nu]
        order += [("P", s, h) for h in range(2) if 0 <= s < 2 * nu]
        kind, u = ("Q", (s - 1) // 2) if s % 2 else ("O", s // 2 - 1)
        if u >= 0 and (kind == "O" or mode != "last"):
            order += [(kind, u, r) for r in range(NPR)]
    late = [x for x in order if x[:2] == ("O", nu - 2)][(0 if mode == "last" else 33):]
    order = [x for x in order if x not in late]
    pos = order.index(("P", 2 * nu - 1, 1)) + 1
    order[pos:pos] = late
    seq, run = [], []
    for n, task in enumerate(order + [None]):
        if task is not None and task[0] in "QO":
            run.append(task)
            continue
        if n and order[n - 1][0] in "QO":
            keep = len(run) - (len(run) % 4 if task is not None else 0)
            for kind, u, r in run[:keep]:
                if seq[-1][:2] == (kind, u):
                    seq[-1][2].append(r)
                else:
                    seq.append((kind, u, [r]))
            run = run[keep:]
        if task is not None:
            seq.append(task)
    return seq


def _kernel(xa, kta, vta, wqa, woa, xb, ktb, vtb, wqb, wob, o_hbm,
            acc, obuf, xraw, xc, qbuf, kvbuf, wqraw, woraw, wqc, woc, zv, zs,
            kvsem, wsem, xsem, osem):
    xs, kvs, wqs, wos = (xa, xb), (kta, vta, ktb, vtb), (wqa, wqb), (woa, wob)

    def ring(slot, k):
        v = slot + k
        return jnp.where(v >= NS, v - NS, v)

    def kv_start(sl, t):
        hg, g = lax.shift_right_logical(t, LG) - 1, t & (NBG - 1)
        for a in range(4):
            pltpu.make_async_copy(kvs[a].at[pl.ds(g * NB, NB), pl.ds(pl.multiple_of(hg * GW, GW), GW), :],
                                  kvbuf.at[sl, a], kvsem.at[sl]).start()

    def kv_piece(k):
        a, b = k // NB, k % NB
        pltpu.make_async_copy(kvs[a].at[b, pl.ds(0, GW), :], kvbuf.at[0, a, b], kvsem.at[0]).start()

    def wq_start(hg, sl):
        cols = pl.ds(pl.multiple_of(hg * GW, GW), GW)
        for p in range(2):
            for kt in range(5):
                pltpu.make_async_copy(wqs[p].at[pl.ds(pl.multiple_of(kt * 128 + sl * SL, SL), SL), cols],
                                      wqraw.at[sl, p, kt], wsem.at[sl, 0]).start()

    def wo_start(hg, sl):
        for p in range(2):
            pltpu.make_async_copy(wos[p].at[hg, :, pl.ds(pl.multiple_of(sl * SL, SL), SL), :],
                                  woraw.at[sl, p], wsem.at[sl, 1]).start()

    def x_start(g):
        for p in range(2):
            pltpu.make_async_copy(xs[p].at[pl.ds(g * NB, NB)], xraw.at[g & 1, p], xsem.at[g & 1]).start()

    def wait_filled(v, sem):
        pltpu.make_async_copy(v, v, sem).wait()

    def w_piece(raw, dst, prods, ws, sl, p, rs):
        rows = pl.ds(pl.multiple_of(sl * (SL // 2), 8), SL // 2)
        vs = _packed_combos([prods[r][1] for r in rs], lambda i, j: raw[sl, p, i, :, _tile(j)])
        for r, v in zip(rs, vs):
            dst[ws, p, r, rows, :] = v

    wq_piece = functools.partial(w_piece, wqraw, wqc, Q_PRODS)
    wo_piece = functools.partial(w_piece, woraw, woc, O_PRODS)
    w_pieces = [(p, rs) for p in range(2) for rs in _split(5)]

    def x_piece(g, row, link, p, b, ks, r0):
        vs = _packed_combos([Q_FORMS[k] for k in ks],
                            lambda s, i: xraw[g & 1, p, b, s * HF + r0:s * HF + r0 + 16, _tile(i)], link())
        for k, v in zip(ks, vs):
            xc[p, row(b), k, r0 // 2:r0 // 2 + 8, :] = v

    x_pieces = [(p, b, ks, r0) for p in range(2) for b in range(NB) for r0 in range(0, HF, 16)
                for ks in _split(5, len(Q_FORMS))]

    units = [(p, b) for p in range(2) for b in range(NB)]
    nu = len(units)

    def step(mode, t, slot):
        g = t & (NBG - 1)
        hq = lax.shift_right_logical(t, LG)
        qslot = hq & 1
        oslot = 1 - qslot
        gb = g * NB

        def prefetch():
            t2 = t + 2
            if mode == "start":
                for k in range(1, NBG):
                    pl.when(g + 1 == k)(functools.partial(kv_piece, k))
            else:
                pl.when(t2 < T + NBG)(functools.partial(kv_start, ring(slot, 2), t2))
            if mode != "last":
                h2, g2 = lax.shift_right_logical(t2, LG), t2 & (NBG - 1)
                pl.when(h2 + 1 < NG)(functools.partial(wq_start, h2 + 1, g2))
                pl.when(h2 < NG)(functools.partial(wo_start, h2, g2))

        if mode == "start":
            pl.when(g + 2 < NBG)(functools.partial(x_start, g + 2))
            pl.when(g + 1 < NBG)(functools.partial(wait_filled, xraw.at[(g + 1) & 1], xsem.at[(g + 1) & 1]))
        if mode != "last":
            pl.when(hq + 1 < NG)(functools.partial(wait_filled, wqraw.at[g], wsem.at[g, 0]))
            wait_filled(woraw.at[g], wsem.at[g, 1])
        if mode != "start":
            wait_filled(kvbuf.at[slot], kvsem.at[slot])

        st = [dict() for _ in range(2 * nu)]
        zero = zv[...]
        jq = [functools.partial(wq_piece, 1 - qslot, g, *a) for a in w_pieces]
        jo = [functools.partial(wo_piece, 1 - oslot, g, *a) for a in w_pieces]

        def x_link():
            link = xc[0, zs[0] + XC_ZERO, 0, 0:8, :]
            for _ in range(4):
                link = (link + zero) & zero
            return link

        jx = [functools.partial(x_piece, g + 1, lambda b: gb + (NB + b), x_link, *a) for a in x_pieces]
        todo = {"start": (jq + jo, [], jx), "last": ([], [], [])}.get(mode, (jq, jo, []))
        every = (5, 4, 2)
        count = [0, 0, 0]

        def side_job(kind):
            count[kind] += 1
            if count[kind] % every[kind] == 0 and todo[kind]:
                todo[kind].pop(0)()

        def task_q(u, rs):
            p, b = units[u]

            def prod(r):
                side_job(0)
                side_job(2)
                return _dot(_unpk(xc[p, gb + b, Q_PRODS[r][0]]), _unpk(wqc[qslot, p, r]))

            def done(s, col, v):
                qbuf[g * nu + u, col, s * HF // 2:(s + 1) * HF // 2, :] = pltpu.bitcast((v * QSCALE).astype(bf16), u32)

            _bilinear(Q_PRODS, rs, prod, st[2 * u].setdefault("qc", {}), None, done)

        def task_k(i, h):
            p, b = units[i // 2]
            k0 = (i % 2) * PW + h * 128
            kt = kvbuf.at[slot, 2 * p, b]
            lane = lax.broadcasted_iota(jnp.int32, (HF, 128), 1)
            q = [qbuf[g * nu + i // 2, 3 * (i % 2) + h + c] for c in range(2)]
            q[1 - h] = jnp.where((lane < 64) if h == 0 else (lane >= 64), q[1 - h], jnp.uint32(0))
            q = _unpk(jnp.concatenate(q, axis=1))
            s = jnp.concatenate([_dot(q, kt[k0:k0 + 256, c:c + 256]) for c in (0, 256)], axis=1)
            st[i][h] = _softmax(s, zero, 4 if mode == "last" else 5)

        def task_p(i, h):
            p, b = units[i // 2]
            k0 = (i % 2) * PW
            vt = kvbuf.at[slot, 2 * p + 1, b]
            d = st[i]
            if h == 0:
                d["ot"] = _dot_nt(vt[k0:k0 + 192, :], d[0][0][:TT].astype(bf16))
                d["oa"] = _dot_nt(d[0][0][TT:].astype(bf16), vt[k0:k0 + 128, :])
                return
            (p1, row1, col1), (p2, row2, col2) = d[0], d[1]
            om = _dot_nt(jnp.concatenate([p1[TT:], p2[TT:]], axis=0).astype(bf16), vt[k0 + 128:k0 + 256, :])
            ot2 = _dot_nt(vt[k0 + 192:k0 + 384, :], p2[:TT].astype(bf16))
            oc = _dot_nt(p2[TT:].astype(bf16), vt[k0 + 256:k0 + 384, :])
            ot1 = d["ot"] * row1
            ot2 = ot2 * row2
            lane = lax.broadcasted_iota(jnp.int32, (R, 128), 1)
            om = jnp.where(lane < 64, om[:R] * col1, om[R:] * col2)
            ta = ot1[0:128].T
            tm = jnp.concatenate([ot1[128:192], ot2[0:64]], axis=0).T
            tc = ot2[64:192].T
            d["o"] = [jnp.concatenate([ta, d["oa"] * col1], axis=0),
                      jnp.concatenate([tm, om], axis=0),
                      jnp.concatenate([tc, oc * col2], axis=0)]

        def task_o(u, rs):
            p, b = units[u]
            d = st[2 * u]
            o = st[2 * u]["o"] + st[2 * u + 1]["o"]
            row0 = (g * NB + b) * SQ

            def idx(s, col):
                return pl.ds(pl.multiple_of(row0 + s * HF, 16), HF), _tile(p * 5 + col)

            def done(s, col, v):
                if mode == "last":
                    obuf[idx(s, col)] = v.astype(bf16)
                else:
                    acc[idx(s, col)] = v

            def prod(r):
                side_job(1)
                f = O_PRODS[r][0]
                if ("form", f) not in d:
                    d["form", f] = _lincomb(O_FORMS[f], lambda k: o[k[1]][k[0] * HF:(k[0] + 1) * HF]).astype(bf16)
                return _dot(d["form", f], _unpk(woc[oslot, p, r]))

            init = None if mode == "first" else (lambda s, col: acc[idx(s, col)])
            _bilinear(O_PRODS, rs, prod, d.setdefault("oc", {}), init, done)
            if mode == "last" and rs[-1] == NPR - 1:
                win = (pl.ds(pl.multiple_of(row0, 16), SQ), pl.ds(p * D, D))
                pltpu.make_async_copy(obuf.at[win], o_hbm.at[win], osem.at[0]).start()

        tasks = {"Q": task_q, "K": task_k, "P": task_p, "O": task_o}
        for n, (kind, i, arg) in enumerate(_schedule(mode, nu)):
            if n == 1:
                prefetch()
            tasks[kind](i, arg)
        for jobs in todo:
            for job in jobs:
                job()

    def loop(lo, hi, fn):
        def body(i, c):
            fn(i)
            return c
        lax.fori_loop(lo, hi, body, 0)

    def steps(mode, lo, hi, slot0):
        def body(t, slot):
            step(mode, t, slot)
            return ring(slot, 1)
        return lax.fori_loop(lo, hi, body, slot0)

    def first_wq(sl):
        wait_filled(wqraw.at[sl], wsem.at[sl, 0])
        for a in w_pieces:
            wq_piece(0, sl, *a)

        @pl.when(sl < 2)
        def _():
            wq_start(1, sl)
            wo_start(0, sl)

    zv[...] = jnp.zeros((8, 128), u32)
    zs[0] = 0
    xc[0, XC_ZERO, 0] = jnp.zeros((HF // 2, 128), u32)
    loop(0, 1, x_start)
    loop(0, NBG, functools.partial(wq_start, 0))
    x_start(1)
    wait_filled(xraw.at[0], xsem.at[0])
    for a in x_pieces:
        x_piece(0, lambda b: b, lambda: None, *a)
    loop(0, NBG, first_wq)
    kv_piece(0)
    steps("start", 0, NBG, jnp.int32(0))
    kv_start(1, NBG + 1)
    slot = steps("first", NBG, 2 * NBG, jnp.int32(0))
    slot = steps("mid", 2 * NBG, T, slot)
    steps("last", T, T + NBG, slot)
    pltpu.make_async_copy(obuf, o_hbm, osem.at[0]).wait()


@jax.jit
def pallas_concat_heads__gqa_block_cached__mha_block_cached__near_ridge_kernel(
    A_x: jax.Array,
    A_k_cache: jax.Array,
    A_v_cache: jax.Array,
    A_wq: jax.Array,
    A_wo: jax.Array,
    B_x: jax.Array,
    B_k_cache: jax.Array,
    B_v_cache: jax.Array,
    B_wq: jax.Array,
    B_wo: jax.Array,
):
    def kv(c):
        return jnp.swapaxes(c, 2, 3).reshape(B, H * DH, SK)

    def wo(w):
        return w.reshape(NG, GW // 128, 128, D)

    hbm = pl.BlockSpec(memory_space=pl.ANY)
    out = pl.pallas_call(
        _kernel,
        in_specs=[hbm] * 10,
        out_specs=hbm,
        out_shape=jax.ShapeDtypeStruct((B * SQ, 2 * D), bf16),
        scratch_shapes=[
            pltpu.VMEM((B * SQ, 2 * D), f32),
            pltpu.VMEM((B * SQ, 2 * D), bf16),
            pltpu.VMEM((2, 2, NB, SQ, D), bf16),
            pltpu.VMEM((2, B + 2 * NB, XC_FORMS, HF // 2, 128), u32),
            pltpu.VMEM((NBG * 2 * NB, 6, HF, 128), u32),
            pltpu.VMEM((NS, 4, NB, GW, SK), bf16),
            pltpu.VMEM((NBG, 2, 5, SL, GW), bf16),
            pltpu.VMEM((NBG, 2, 6, SL, D), bf16),
            pltpu.VMEM((2, 2, NPR, 64, 128), u32),
            pltpu.VMEM((2, 2, NPR, 64, 128), u32),
            pltpu.VMEM((8, 128), u32),
            pltpu.SMEM((1,), jnp.int32),
            pltpu.SemaphoreType.DMA((NS,)),
            pltpu.SemaphoreType.DMA((NBG, 2)),
            pltpu.SemaphoreType.DMA((2,)),
            pltpu.SemaphoreType.DMA((1,)),
        ],
        compiler_params=pltpu.CompilerParams(vmem_limit_bytes=112 * 1024 * 1024, disable_bounds_checks=True),
    )(A_x, kv(A_k_cache), kv(A_v_cache), A_wq, wo(A_wo), B_x, kv(B_k_cache), kv(B_v_cache), B_wq, wo(B_wo))
    return out.reshape(B, SQ, 2 * D)
```
